```python
import jax
import jax.numpy as jnp

def _softmax(x, axis=-1):
    return jax.nn.softmax(x, axis=axis)

def _gelu(x):
    return jax.nn.gelu(x, approximate=True)

def _silu(x):
    return jax.nn.silu(x)

def _sigmoid(x):
    return jax.nn.sigmoid(x)

def _layernorm(x, axis=-1, eps=1e-05):
    m = jnp.mean(x, axis=axis, keepdims=True)
    v = jnp.var(x, axis=axis, keepdims=True)
    return (x - m) / jnp.sqrt(v + eps)

def _scatter_add(tgt, idx, src, axis=0):
    return tgt.at[idx].add(src)

def _segment_sum(src, seg, n):
    return jax.ops.segment_sum(src, seg, n)

class _Rng:

    def __init__(self, key):
        self._k = key

    def _next(self):
        self._k, sub = jax.random.split(self._k)
        return sub

    def normal(self, shape):
        return jax.random.normal(self._next(), shape, dtype=jnp.bfloat16)

    def randint(self, lo, hi, shape):
        return jax.random.randint(self._next(), shape, lo, hi, dtype=jnp.int32)

    def uniform(self, shape, lo=0.0, hi=1.0):
        return jax.random.uniform(self._next(), shape, jnp.bfloat16, lo, hi)

    def permutation(self, n):
        return jax.random.permutation(self._next(), n)
kernel_name = 'standalone__conformer_family_branchformer__speech'

def setup_inputs():
    _rng = _Rng(jax.random.key(int.from_bytes(__import__("os").urandom(4), "little")))
    _w = lambda a: (lambda t: t.astype(jnp.bfloat16) if jnp.issubdtype(t.dtype, jnp.floating) else t)(jnp.asarray(a))
    B, T, D, K = (2, 4000, 512, 31)
    s = float(D) ** (-0.5)
    return {'x': _w((lambda *s: _rng.normal(s) * 0.05)(B, T, D)), 'w_q': _w((lambda *s: _rng.normal(s) * 0.05)(D, D) * s), 'w_k': _w((lambda *s: _rng.normal(s) * 0.05)(D, D) * s), 'w_v': _w((lambda *s: _rng.normal(s) * 0.05)(D, D) * s), 'w_ao': _w((lambda *s: _rng.normal(s) * 0.05)(D, D) * s), 'w_up': _w((lambda *s: _rng.normal(s) * 0.05)(D, 2 * D) * s), 'dw': _w((lambda *s: _rng.normal(s) * 0.05)(K, D) * (1.0 / K)), 'w_dn': _w((lambda *s: _rng.normal(s) * 0.05)(D, D) * s), 'w_merge': _w((lambda *s: _rng.normal(s) * 0.05)(2 * D, D) * s)}

def reference(x, w_q, w_k, w_v, w_ao, w_up, dw, w_dn, w_merge):
    B, T, D = x.shape
    K = dw.shape[0]
    xa = _layernorm(x, axis=-1)
    q = jnp.einsum('btd,de->bte', xa, w_q)
    k = jnp.einsum('btd,de->bte', xa, w_k)
    v = jnp.einsum('btd,de->bte', xa, w_v)
    logits = jnp.einsum('btd,bsd->bts', q, k) * float(D) ** (-0.5)
    attn = _softmax(logits, axis=-1)
    ya = jnp.einsum('bts,bsd->btd', attn, v)
    ya = jnp.einsum('btd,de->bte', ya, w_ao)
    xc = _layernorm(x, axis=-1)
    h = _gelu(jnp.einsum('btd,de->bte', xc, w_up))
    u = h[..., :D].copy()
    g = _layernorm(h[..., D:], axis=-1)
    pad = K // 2
    gp = jnp.pad(g, ((0, 0), (pad, pad), (0, 0)))
    conv = jnp.zeros_like(g)
    for i in range(K):
        conv = conv + gp[:, i:i + T, :] * dw[i][None, None, :]
    yc = jnp.einsum('btd,de->bte', u * conv, w_dn)
    merged = jnp.concatenate([ya, yc], axis=-1)
    out = jnp.einsum('btf,fd->btd', merged, w_merge)
    return x + out
```

```python
import functools
import math
import jax
import jax.numpy as jnp
from jax import lax
from jax.experimental import pallas as pl
from jax.experimental.pallas import tpu as pltpu

F32 = jnp.float32
BF16 = jnp.bfloat16
U32 = jnp.uint32
EPS = 1e-5
LANES = 128
HALO = 16
PAD = 8


def _ln(x):
    d = x.shape[-1]
    m = jnp.sum(x, axis=-1, keepdims=True) * (1.0 / d)
    c = x - m
    v = jnp.sum(c * c, axis=-1, keepdims=True) * (1.0 / d)
    return c * lax.rsqrt(v + EPS)


def _gelu(x):
    c1 = math.sqrt(2.0 / math.pi)
    c2 = c1 * 0.044715
    t = jnp.tanh(x * (c1 + c2 * (x * x)))
    hx = 0.5 * x
    return hx + hx * t


def _dot(a, b):
    return jnp.dot(a, b, preferred_element_type=F32)


def _dot_nt(a, b):
    return lax.dot_general(a, b, (((1,), (1,)), ((), ())), preferred_element_type=F32)


def _pack(v):
    return pltpu.bitcast(v.astype(BF16), U32)


def _unpack(w):
    return pltpu.bitcast(w, BF16)


def _kernel(x_hbm, wq_hbm, wk_hbm, wv_hbm, wao_hbm, wup_hbm, dw_hbm, wdn_hbm, wm_hbm,
            o_hbm,
            x_buf, xa0, xa1, wq, wk, wv, wao, wup_in, dw_in, wdn, wm,
            wqk, wu, wg, wva, wdc, g_first, u_first, cb,
            s_e, s_o, za_buf, q_buf, o_buf,
            x_sem, w_sem, o_sem, *, B, T, D, KW, BQ, BK, TP, CR, LR, DL, XG):
    NQ = T // BQ
    NB = B * NQ
    NL = D // LANES
    NC = TP // BK
    HQ = BQ // 2
    xas = (xa0, xa1)
    G, H, U, W, Z = (NL * j for j in range(5))

    def x_copy(n):
        b, i = n // NQ, n % NQ
        r = pl.ds(pl.multiple_of(i * BQ, BQ), BQ)
        return pltpu.make_async_copy(x_hbm.at[b, r, :], x_buf.at[b, r, :], x_sem.at[n])

    def o_copy(n, slot):
        b, i = n // NQ, n % NQ
        r = pl.ds(pl.multiple_of(i * BQ, BQ), BQ)
        return pltpu.make_async_copy(o_buf.at[slot], o_hbm.at[b, r, :], o_sem.at[slot])

    w_pairs = [(wq_hbm, wq), (wk_hbm, wk), (wv_hbm, wv), (wao_hbm, wao), (wm_hbm, wm),
               (wdn_hbm, wdn), (wup_hbm, wup_in), (dw_hbm, dw_in)]
    w_copies = [pltpu.make_async_copy(s, d, w_sem.at[j]) for j, (s, d) in enumerate(w_pairs)]
    def ln_rows(b, r0, nrows):
        return _pack(_ln(x_buf[b, r0:r0 + nrows, :].astype(F32)))

    cq, ck, cv, cao, cm, cdn, cup, cdw = w_copies
    for c in (cq, ck, cv, cao):
        c.start()
    for b in range(B):
        xas[b][T // 2:TP // 2, :] = jnp.zeros(((TP - T) // 2, D), U32)
    cb[G:G + NL, BQ:BQ + 2 * HALO, :] = jnp.zeros((NL, 2 * HALO, LANES), F32)
    cb[U:U + NL, BQ:BQ + HALO, :] = jnp.zeros((NL, HALO, LANES), F32)
    cq.wait()
    ck.wait()
    for c in (cm, cdn):
        c.start()
    wqk[...] = _pack(_dot_nt(wq[...], wk[...]) * (math.log2(math.e) / math.sqrt(D)))
    cv.wait()
    cao.wait()
    for c in (cup, cdw, x_copy(NQ)):
        c.start()
    for n in range(0, XG):
        x_copy(n).start()
    w1 = _dot(wv[...], wao[...]).astype(BF16)
    cm.wait()
    cdn.wait()
    for n in range(XG, 2 * XG):
        x_copy(n).start()
    wva[0:D // 2, :] = _pack(_dot(w1, wm[0:D, :]))
    wdc[0:D // 2, :] = _pack(_dot(wdn[...], wm[D:2 * D, :]))
    cup.wait()
    cdw.wait()
    x_copy(NQ).wait()
    for n in range(2 * XG, NQ):
        x_copy(n).start()
    wu[...] = _pack(wup_in[:, 0:D])
    wg[...] = _pack(wup_in[:, D:2 * D])
    dwf = dw_in[...].astype(F32)
    for k in range(KW):
        for l in range(NL):
            cb[W + l, 8 * k:8 * k + 8, :] = jnp.broadcast_to(dwf[k:k + 1, l * LANES:(l + 1) * LANES], (8, LANES))

    def ln_body(n, c):
        x_copy(n).wait()
        xa0[pl.ds(pl.multiple_of(n * HQ, HQ), HQ), :] = _pack(
            _ln(x_buf[0, pl.ds(pl.multiple_of(n * BQ, BQ), BQ), :].astype(F32)))
        return c
    lax.fori_loop(0, NQ, ln_body, 0)

    xf = jnp.concatenate([_ln(x_buf[b, 0:HALO, :].astype(F32)) for b in range(B)], axis=0).astype(BF16)
    uf = _dot(xf, _unpack(wu[...]))
    gf = _ln(_gelu(_dot(xf, _unpack(wg[...]))))
    for b in range(B):
        u_first[b] = uf[b * HALO:(b + 1) * HALO]
        g_first[b] = gf[b * HALO:(b + 1) * HALO]

    s_par = (s_e, s_o)
    A0 = TP // 2
    W0 = BQ

    def body(i, carry, b):
        n = b * NQ + i
        xa = xas[b]
        slot = i % 2
        r0 = pl.multiple_of(i * BQ, BQ)
        h0 = pl.multiple_of(i * HQ, HQ)

        if b + 1 < B:
            @pl.when(i >= 1)
            def _():
                x_copy(n + NQ).wait()

            @pl.when(i + 1 < NQ)
            def _():
                x_copy(n + NQ + 1).start()

        @pl.when(n >= 2)
        def _():
            o_copy(n - 2, slot).wait()

        first = i == 0
        z8 = pl.multiple_of((i // NQ) * 16, 16)
        zf = pl.multiple_of((i // (NQ + 1)) * 16, 16)

        def fence(src, dst):
            lead_s = (0,) * (len(src.shape) - 2)
            lead_d = (0,) * (len(dst.shape) - 2)
            rows_d = 8 * (4 // jnp.dtype(dst.dtype).itemsize)
            v = src[lead_s + (pl.ds(zf, 8), slice(0, LANES))]
            v = pltpu.bitcast(v, dst.dtype)
            dst[lead_d + (pl.ds(dst.shape[-2] - rows_d + zf, rows_d), slice(0, LANES))] = v

        for l in range(NL):
            ls = slice(l * LANES, (l + 1) * LANES)
            cb[G + l, 0:HALO, :] = jnp.where(first, 0.0, cb[G + l, BQ:BQ + HALO, :])
            cb[G + l, HALO:2 * HALO, :] = jnp.where(first, g_first[b, :, ls],
                                                    cb[G + l, BQ + HALO:BQ + 2 * HALO, :])
            cb[U + l, 0:HALO, :] = jnp.where(first, u_first[b, :, ls], cb[U + l, BQ:BQ + HALO, :])

        ru = pl.ds(pl.multiple_of(h0 + HALO // 2, HALO // 2), HQ)
        hg = _dot(_unpack(xa[ru, :]), _unpack(wg[...]))
        hu = _dot(_unpack(xa[ru, :]), _unpack(wu[...]))
        for l in range(NL):
            cb[H + l, 0:BQ, :] = hg[:, l * LANES:(l + 1) * LANES]
        for l in range(NL):
            cb[U + l, HALO:HALO + BQ, :] = hu[:, l * LANES:(l + 1) * LANES]
        q_buf[0:HQ, :] = _pack(_dot(_unpack(xa[pl.ds(h0, HQ), :]), _unpack(wqk[...])))
        cb[Z, pl.ds(HQ + zf, 8), :] = cb[W, 0:8, :]

        def gate_rows(t0, nrows):
            h = jnp.concatenate([cb[H + l, t0:t0 + nrows, :] for l in range(NL)], axis=1)
            g = _ln(_gelu(h))
            for l in range(NL):
                cb[G + l, 2 * HALO + t0:2 * HALO + t0 + nrows, :] = g[:, l * LANES:(l + 1) * LANES]

        def conv_piece(l, t0, nr):
            acc = [None] * nr
            off = HALO - KW // 2
            for s in range(8):
                taps = [(a, 8 * a + s - off) for a in range((KW + off + 7) // 8)
                        if 0 <= 8 * a + s - off < KW]
                w = {a: cb[W + l, 8 * k:8 * k + 8, :] for a, k in taps}
                for j in range(nr + max(a for a, _ in taps)):
                    use = [a for a, _ in taps if 0 <= j - a < nr]
                    if not use:
                        continue
                    gv = cb[G + l, t0 + 8 * j + s:t0 + 8 * j + s + 8, :]
                    for a in use:
                        t = gv * w[a]
                        acc[j - a] = t if acc[j - a] is None else acc[j - a] + t
            cv = jnp.concatenate(acc, axis=0)
            u = _gelu(cb[U + l, t0:t0 + 8 * nr, :])
            cb[Z + l, pl.ds(zf + t0 // 2, 4 * nr), :] = pltpu.bitcast(_pack(cv * u), F32)

        blocks = [(t0, min(CR, BQ - t0)) for t0 in range(0, BQ, CR)]
        gate_rows(*blocks[0])
        for k, (t0, nrows) in enumerate(blocks):
            if k + 1 < len(blocks):
                gate_rows(*blocks[k + 1])
            for l in range(NL):
                conv_piece(l, t0, nrows // 8)

        def kv(c):
            return _unpack(xa[c * BK // 2:(c + 1) * BK // 2, :])

        m = None
        for c in range(NC):
            s = _dot_nt(_unpack(q_buf[pl.ds(z8, HQ), :]), kv(c))
            if (c + 1) * BK > T:
                col = lax.broadcasted_iota(jnp.int32, (BQ, BK), 1)
                s = jnp.where(col < T - c * BK, s, -jnp.inf)
            s_par[c % 2][0:BQ, (c // 2) * BK:(c // 2 + 1) * BK] = s
            for l in range(BK // LANES):
                t = s[:, l * LANES:(l + 1) * LANES]
                m = t if m is None else jnp.maximum(m, t)
        m = jnp.max(m, axis=-1, keepdims=True)

        def probs(c, lsum):
            p = jnp.exp2(s_par[c % 2][pl.ds(z8, BQ), (c // 2) * BK:(c // 2 + 1) * BK] - m)
            for l in range(BK // LANES):
                t = p[:, l * LANES:(l + 1) * LANES]
                lsum = t if lsum is None else lsum + t
            return p.astype(BF16), lsum

        p, lsum = probs(0, None)
        for c in range(NC):
            pn = None
            if c + 1 < NC:
                pn, lsum = probs(c + 1, lsum)
            if c == DL:
                fence(cb, xa)
            d = _dot(p, kv(c))
            if c > 0:
                d = d + s_par[(c - 1) % 2][pl.ds(z8, BQ), A0:A0 + D]
            if c + 1 < NC:
                s_par[c % 2][0:BQ, A0:A0 + D] = d
            p = pn
        lsum = jnp.sum(lsum, axis=-1, keepdims=True)
        za_buf[0:HQ, :] = _pack(d * (1.0 / lsum))

        if b + 1 < B:
            for t0 in range(0, BQ, LR):
                xas[b + 1][pl.ds(h0 + t0 // 2, LR // 2), :] = _pack(
                    _ln(x_buf[b + 1, pl.ds(r0 + t0, LR), :].astype(F32)))
                fence(xas[b + 1], x_buf)
            fence(xas[b + 1], wva)

        zc = jnp.concatenate([cb[Z + l, pl.ds(z8, HQ), :] for l in range(NL)], axis=1)
        out = _dot(pltpu.bitcast(zc, BF16), _unpack(wdc[0:D // 2, :]))
        out = out + x_buf[b, pl.ds(r0, BQ), :].astype(F32)
        out = out + _dot(_unpack(za_buf[pl.ds(z8, HQ), :]), _unpack(wva[0:D // 2, :]))
        o_buf[slot] = out.astype(o_buf.dtype)
        o_copy(n, slot).start()
        return carry

    for b in range(B):
        lax.fori_loop(0, NQ, functools.partial(body, b=b), 0)
    o_copy(NB - 2, (NB - 2) % 2).wait()
    o_copy(NB - 1, (NB - 1) % 2).wait()


def make(BQ=400, BK=512, CR=16, LR=16, DL=0, XG=3, flags=None):
    def fn(x, w_q, w_k, w_v, w_ao, w_up, dw, w_dn, w_merge):
        B, T, D = x.shape
        KW = dw.shape[0]
        TP = -(-(T + HALO) // BK) * BK
        NL = D // LANES
        kern = functools.partial(_kernel, B=B, T=T, D=D, KW=KW, BQ=BQ, BK=BK, TP=TP, CR=CR, LR=LR, DL=DL, XG=XG)
        any_spec = pl.BlockSpec(memory_space=pl.ANY)
        V = pltpu.VMEM
        E = 2 * PAD
        scratch = [
            V((B, T + 2 * E, D), BF16), V((TP // 2 + E, D), U32), V((TP // 2 + E, D), U32),
            V((D, D), BF16), V((D, D), BF16), V((D, D), BF16), V((D, D), BF16),
            V((D, 2 * D), BF16), V((KW, D), BF16), V((D, D), BF16), V((2 * D, D), BF16),
            V((D // 2, D), U32), V((D // 2, D), U32), V((D // 2, D), U32), V((D // 2 + E, D), U32),
            V((D // 2 + E, D), U32),
            V((B, HALO, D), F32), V((B, HALO, D), F32),
            V((5 * NL, BQ + 2 * HALO, LANES), F32),
            V((BQ + E, TP // 2 + D), F32), V((BQ + E, TP // 2 + D), F32),
            V((BQ // 2 + E, D), U32), V((BQ // 2 + E, D), U32),
            V((2, BQ, D), BF16),
            pltpu.SemaphoreType.DMA((B * (T // BQ),)), pltpu.SemaphoreType.DMA((8,)),
            pltpu.SemaphoreType.DMA((2,)),
        ]
        return pl.pallas_call(
            kern,
            out_shape=jax.ShapeDtypeStruct((B, T, D), x.dtype),
            in_specs=[any_spec] * 9,
            out_specs=any_spec,
            scratch_shapes=scratch,
            compiler_params=pltpu.CompilerParams(vmem_limit_bytes=100 * 1024 * 1024, flags=flags),
        )(x, w_q, w_k, w_v, w_ao, w_up, dw, w_dn, w_merge)
    return fn


_branchformer = make()


@jax.jit
def pallas_standalone__conformer_family_branchformer__speech_kernel(
    x: jax.Array,
    w_q: jax.Array,
    w_k: jax.Array,
    w_v: jax.Array,
    w_ao: jax.Array,
    w_up: jax.Array,
    dw: jax.Array,
    w_dn: jax.Array,
    w_merge: jax.Array,
):
    return _branchformer(x, w_q, w_k, w_v, w_ao, w_up, dw, w_dn, w_merge)
```

```python
import functools
import math
import jax
import jax.numpy as jnp
from jax import lax
from jax.experimental import pallas as pl
from jax.experimental.pallas import tpu as pltpu

F32 = jnp.float32
BF16 = jnp.bfloat16
U32 = jnp.uint32
EPS = 1e-5
LANES = 128
HALO = 16
PAD = 16


def _ln(x):
    d = x.shape[-1]
    m = jnp.sum(x, axis=-1, keepdims=True) * (1.0 / d)
    c = x - m
    v = jnp.sum(c * c, axis=-1, keepdims=True) * (1.0 / d)
    return c * lax.rsqrt(v + EPS)


def _gelu(x):
    c1 = math.sqrt(2.0 / math.pi)
    c2 = c1 * 0.044715
    t = jnp.tanh(x * (c1 + c2 * (x * x)))
    hx = 0.5 * x
    return hx + hx * t


def _dot(a, b):
    return jnp.dot(a, b, preferred_element_type=F32)


def _dot_nt(a, b):
    return lax.dot_general(a, b, (((1,), (1,)), ((), ())), preferred_element_type=F32)


def _pack(v):
    return pltpu.bitcast(v.astype(BF16), U32)


def _unpack(w):
    return pltpu.bitcast(w, BF16)


def _combos(a11, a12, a21, a22):
    return [a11 + a22, a11, a22, a21 - a22, a12 - a11, a11 + a21, a12 + a22]


PAIRS = ((0, 0), (1, 6), (3, 1), (4, 2), (2, 5), (5, 4), (6, 3))


def _combine(n):
    return (n[0] + n[3] - n[4] + n[6], n[1] + n[3], n[2] + n[4], n[0] - n[1] + n[2] + n[5])


def _kernel(x_hbm, wq_hbm, wk_hbm, wv_hbm, wao_hbm, wup_hbm, dw_hbm, wdn_hbm, wm_hbm,
            o_hbm,
            x_buf, xh_buf, xs_all, wst, dw_in, wf32, wc, g_first, cb, xn_buf,
            s_e, s_o, a_e, a_o, y_buf, q_buf, o_buf,
            x_sem, h_sem, w_sem, o_sem, *, B, T, D, KW, BQ, BK, TP, CR, LR, ORDER, MORDER, PK, MC, XC):
    NQ = T // BQ
    NB = B * NQ
    NL = D // LANES
    NC = TP // BK
    HB = BQ // 2
    HD = D // 2
    G, H, U, W, Z = (NL * j for j in range(5))

    def x_copy(n):
        b, i = n // NQ, n % NQ
        r = pl.ds(pl.multiple_of(i * BQ, BQ), BQ)
        return pltpu.make_async_copy(x_hbm.at[b, r, :], x_buf.at[b, r, :], x_sem.at[n])

    def o_copy(n, slot):
        b, i = n // NQ, n % NQ
        r = pl.ds(pl.multiple_of(i * BQ, BQ), BQ)
        return pltpu.make_async_copy(o_buf.at[slot], o_hbm.at[b, r, :], o_sem.at[slot])

    heads = [(b, i) for b in range(B) for i in range(1, NQ)]
    h_copies = [pltpu.make_async_copy(x_hbm.at[b, i * BQ:i * BQ + HALO, :],
                                      xh_buf.at[j * HALO:(j + 1) * HALO, :], h_sem)
                for j, (b, i) in enumerate(heads)]
    WQ, WK, WV, WAO, WMA, WDN, WMC, WU, WG, W1, XH = range(11)
    w_src = [wq_hbm, wk_hbm, wv_hbm, wao_hbm, wm_hbm.at[0:D], wdn_hbm, wm_hbm.at[D:2 * D],
             wup_hbm.at[:, 0:D], wup_hbm.at[:, D:2 * D]]
    w_copies = [pltpu.make_async_copy(src, wst.at[j], w_sem.at[j]) for j, src in enumerate(w_src)]
    dw_copy = pltpu.make_async_copy(dw_hbm, dw_in, w_sem.at[len(w_src)])
    QK, VA, DC, UU, GG = range(5)
    RB = HALO * len(heads)
    NRB = D // RB

    def ln_rows(b, r0, t0, nrows):
        top = _ln(x_buf[b, pl.ds(r0 + t0, nrows), :].astype(F32))
        bot = _ln(x_buf[b, pl.ds(r0 + HB + t0, nrows), :].astype(F32))
        return [_pack(v) for v in _combos(top[:, :HD], top[:, HD:], bot[:, :HD], bot[:, HD:])]

    for j in (WQ, WK, WV, WAO):
        w_copies[j].start()
    for b in range(B):
        xs_all[b, :, T // 4:TP // 2, :] = jnp.zeros((7, TP // 2 - T // 4, HD), U32)
    cb[G:G + NL, BQ:BQ + HALO, :] = jnp.zeros((NL, HALO, LANES), F32)
    w_copies[WQ].wait()
    w_copies[WK].wait()
    for j in (WMA, WDN, WMC):
        w_copies[j].start()

    def fold_qk(t, c):
        r = pl.ds(pl.multiple_of(t * RB, RB), RB)
        wf32[QK, r, :] = _dot_nt(wst[WQ, r, :], wst[WK]) * (math.log2(math.e) / math.sqrt(D))
        return c
    lax.fori_loop(0, NRB, fold_qk, 0)

    w_copies[WV].wait()
    w_copies[WAO].wait()
    for c in [w_copies[WU], w_copies[WG], dw_copy, x_copy(0)] + h_copies:
        c.start()

    def fold(t, c):
        j = t // NRB

        @pl.when(t == NRB)
        def _():
            for k in (WMA, WDN, WMC):
                w_copies[k].wait()
            x_copy(1).start()
            x_copy(2).start()

        @pl.when(t == 3 * NRB)
        def _():
            for cp in [w_copies[WU], w_copies[WG], dw_copy] + h_copies:
                cp.wait()
            for n in range(3, NQ):
                x_copy(n).start()
            wst[XH, 0:RB, :] = _ln(xh_buf[...].astype(F32)).astype(BF16)

        left = jnp.where(j == 0, WV, jnp.where(j == 1, W1, jnp.where(j == 2, WDN, XH)))
        right = jnp.where(j == 0, WAO, jnp.where(j == 1, WMA, jnp.where(j == 2, WMC, WG)))
        r = pl.ds(pl.multiple_of((t % NRB) * RB, RB), RB)
        v = _dot(wst[left, r, :], wst[right])
        wf32[jnp.where(j == 1, VA, jnp.where(j == 2, DC, UU)), r, :] = v
        wst[jnp.where(j == 0, W1, WQ), r, :] = v.astype(BF16)
        return c
    lax.fori_loop(0, 3 * NRB + 1, fold, 0)

    gf = _ln(_gelu(wf32[UU, 0:RB, :]))
    for j, (b, i) in enumerate(heads):
        g_first[b * NQ + i - 1] = gf[j * HALO:(j + 1) * HALO]
    for b in range(B):
        g_first[b * NQ + NQ - 1] = jnp.zeros((HALO, D), F32)

    def widen(t, c):
        j, r = t // NRB, pl.ds(pl.multiple_of((t % NRB) * RB, RB), RB)
        wf32[UU + j, r, :] = wst[WU + j, r, :].astype(F32)
        return c
    lax.fori_loop(0, 2 * NRB, widen, 0)

    def split(t, c):
        j, t0 = t // 2, pl.multiple_of((t % 2) * (HD // 2), HD // 2)
        top, bot = pl.ds(t0, HD // 2), pl.ds(HD + t0, HD // 2)
        quads = wf32[j, top, 0:HD], wf32[j, top, HD:D], wf32[j, bot, 0:HD], wf32[j, bot, HD:D]
        for k, v in enumerate(_combos(*quads)):
            wc[j, k, pl.ds(pl.multiple_of(t0 // 2, HD // 4), HD // 4), :] = _pack(v)
        return c
    lax.fori_loop(0, 10, split, 0)

    for l in range(NL):
        cb[Z + l, 0:KW, :] = dw_in[:, l * LANES:(l + 1) * LANES].astype(F32)

    def taps(k, c):
        for l in range(NL):
            cb[W + l, pl.ds(pl.multiple_of(8 * k, 8), 8), :] = jnp.broadcast_to(
                cb[Z + l, pl.ds(k, 1), :], (8, LANES))
        return c
    lax.fori_loop(0, KW, taps, 0)

    def ln_body(n, c):
        x_copy(n).wait()
        for j, v in enumerate(ln_rows(0, pl.multiple_of(n * BQ, BQ), 0, HB)):
            xs_all[0, j, pl.ds(pl.multiple_of(n * (HB // 2), HB // 2), HB // 2), :] = v
        return c
    lax.fori_loop(0, NQ, ln_body, 0)
    x_copy(NQ).start()
    wqk, wva, wdc, wu, wg = (wc.at[j] for j in (QK, VA, DC, UU, GG))

    s_par = (s_e, s_o)
    a_par = (a_e, a_o)
    SW = TP // 2

    def body(n, carry):
        b, i = n // NQ, n % NQ
        xs = xs_all.at[b]
        slot = n % 2
        r0 = pl.multiple_of(i * BQ, BQ)
        h0 = pl.multiple_of(i * (HB // 2), HB // 2)

        @pl.when(n + NQ < NB)
        def _():
            x_copy(n + NQ).wait()

        @pl.when(n + NQ + 1 < NB)
        def _():
            x_copy(n + NQ + 1).start()

        @pl.when(n >= 2)
        def _():
            o_copy(n - 2, slot).wait()

        first = i == 0
        z8 = pl.multiple_of((n // NB) * 16, 16)
        zf = pl.multiple_of((n // (NB + 1)) * 16, 16)

        def pin(dst, v):
            lead = (0,) * (len(dst.shape) - 2)
            rows = 8 * (4 // jnp.dtype(dst.dtype).itemsize)
            v = pltpu.bitcast(v[v.shape[0] - 8:, :LANES], dst.dtype)
            dst[lead + (pl.ds(dst.shape[-2] - rows + zf, rows), slice(0, LANES))] = v

        def project(w):
            return _combine([_dot(_unpack(xs[l, pl.ds(h0, HB // 2), :]), _unpack(w[r, 0:HD // 2, :]))
                             for l, r in PAIRS])

        def put_quads(base, row0, quads):
            for q, v in enumerate(quads):
                for l in range(NL // 2):
                    cb[base + (q % 2) * (NL // 2) + l, row0 + (q // 2) * HB:row0 + (q // 2 + 1) * HB, :] = (
                        v[:, l * LANES:(l + 1) * LANES])

        for l in range(NL):
            ls = slice(l * LANES, (l + 1) * LANES)
            cb[G + l, 0:HALO, :] = jnp.where(first, 0.0, cb[G + l, BQ:BQ + HALO, :])
            cb[G + l, BQ + HALO:BQ + 2 * HALO, :] = g_first[n, :, ls]

        bn = (b + 1) % B
        for t0 in range(0, HB, LR):
            nrows = min(LR, HB - t0)
            for j, v in enumerate(ln_rows(bn, r0, t0, nrows)):
                xn_buf[j, t0 // 2:(t0 + nrows) // 2, :] = v
            pin(x_buf, xn_buf[0, pl.ds(z8, 8), :])

        put_quads(U, 0, [_gelu(v) for v in project(wu)])
        put_quads(H, 0, [_gelu(v) for v in project(wg)])
        pin(cb, xn_buf[0, pl.ds(z8, 8), :])
        a11, a12, a21, a22 = project(wqk)
        for j, v in enumerate([a11 + a22, a21 + a22, a11, a22, a11 + a12, a21 - a11, a12 - a22]):
            q_buf[j, 0:HB // 2, :] = _pack(v)

        def gate_rows(t0, nrows):
            g = _ln(jnp.concatenate([cb[H + l, t0:t0 + nrows, :] for l in range(NL)], axis=1))
            for l in range(NL):
                cb[G + l, HALO + t0:HALO + t0 + nrows, :] = g[:, l * LANES:(l + 1) * LANES]

        def conv_rows(l, t0, nr):
            acc = [None] * nr
            off = HALO - KW // 2
            for s in range(8):
                taps = [(a, 8 * a + s - off) for a in range((KW + off + 7) // 8)
                        if 0 <= 8 * a + s - off < KW]
                w = {a: cb[W + l, 8 * k:8 * k + 8, :] for a, k in taps}
                for j in range(nr + max(a for a, _ in taps)):
                    use = [a for a, _ in taps if 0 <= j - a < nr]
                    if not use:
                        continue
                    gv = cb[G + l, t0 + 8 * j + s:t0 + 8 * j + s + 8, :]
                    for a in use:
                        t = gv * w[a]
                        acc[j - a] = t if acc[j - a] is None else acc[j - a] + t
            return acc * 1

        def conv_piece(l, t0, nrows):
            cv = jnp.concatenate(conv_rows(l, t0, nrows // 8), axis=0)
            cb[Z + l, pl.ds(zf + t0, nrows), :] = cv * cb[U + l, t0:t0 + nrows, :]

        blocks = [(t0, min(CR, BQ - t0)) for t0 in range(0, BQ, CR)]
        gate_rows(*blocks[0])
        gate_rows(*blocks[1])
        for k, (t0, nrows) in enumerate(blocks):
            if k + 2 < len(blocks):
                gate_rows(*blocks[k + 2])
            for l in range(NL):
                conv_piece(l, t0, nrows)

        def kv(j, c):
            return _unpack(xs[j, c * BK // 2:(c + 1) * BK // 2, :])

        m = [None, None]
        for c in range(NC):
            M = []
            for j, r in enumerate((0, 1, 3, 4, 2, 5, 6)):
                M.append(_dot_nt(_unpack(q_buf[j, pl.ds(z8, HB // 2), :]), kv(r, c)))
            quads = (M[0] + M[3] - M[4] + M[6], M[2] + M[4], M[1] + M[3], M[0] - M[1] + M[2] + M[5])
            for q, s in enumerate(quads):
                if (c + 1) * BK > T // 2:
                    col = lax.broadcasted_iota(jnp.int32, (HB, BK), 1)
                    s = jnp.where(col < T // 2 - c * BK, s, -jnp.inf)
                c0 = (q % 2) * SW + (c // 2) * BK
                s_par[c % 2][(q // 2) * HB:(q // 2 + 1) * HB, c0:c0 + BK] = s
                for l in range(BK // LANES):
                    t = s[:, l * LANES:(l + 1) * LANES]
                    m[q // 2] = t if m[q // 2] is None else jnp.maximum(m[q // 2], t)
        for h in range(2):
            mx = jnp.max(m[h], axis=-1, keepdims=True)
            m[h] = mx + jnp.log2(jnp.sum(jnp.exp2(m[h] - mx), axis=-1, keepdims=True))

        def merge(quads, w):
            left = _combos(*quads)
            out = [None] * 7
            for k in MORDER:
                l, r = PAIRS[k]
                out[k] = _dot(left[l].astype(BF16), _unpack(w[r, 0:HD // 2, :]))
            return _combine(out)

        def merge_conv():
            zq = [jnp.concatenate([cb[Z + (q % 2) * (NL // 2) + l, pl.ds(z8 + (q // 2) * HB, HB), :]
                                   for l in range(NL // 2)], axis=1) for q in range(4)]
            for q, v in enumerate(merge(zq, wdc)):
                y_buf[q, 0:HB, :] = v

        def probs(c):
            p, part = [], [None, None]
            for q in range(4):
                c0 = (q % 2) * SW + (c // 2) * BK
                e = jnp.exp2(s_par[c % 2][pl.ds(z8 + (q // 2) * HB, HB), c0:c0 + BK] - m[q // 2])
                for l in range(BK // LANES):
                    t = e[:, l * LANES:(l + 1) * LANES]
                    part[q // 2] = t if part[q // 2] is None else part[q // 2] + t
                p.append(e)
            return [v.astype(BF16) for v in _combos(*p)], jnp.concatenate(part, axis=1)

        def accumulate(c, k, d):
            if c > 0:
                d = d + a_par[(c - 1) % 2][k, pl.ds(z8, HB), :]
            if c + 1 < NC:
                a_par[c % 2][k, 0:HB, :] = d
            return d

        nxt = probs(0)
        for c in range(NC):
            if c == MC:
                merge_conv()
            p, part = nxt
            acc = [None] * 7
            for kk, k in enumerate(ORDER):
                l, r = PAIRS[k]
                d = _dot(p[l], kv(r, c))
                if kk == PK and c + 1 < NC:
                    pin(s_par[(c + 1) % 2], d)
                    nxt = probs(c + 1)
                acc[k] = accumulate(c, k, d)
            lsum = accumulate(c, 7, part)
        lsum = [lsum[:, :LANES], lsum[:, LANES:]]
        o11, o12, o21, o22 = _combine(acc)
        inv = [1.0 / jnp.sum(v, axis=-1, keepdims=True) for v in lsum]
        pin(xn_buf, acc[ORDER[XC]])
        for j in range(7):
            xs_all[bn, j, pl.ds(h0, HB // 2), :] = xn_buf[j, pl.ds(z8, HB // 2), :]
        for q, v in enumerate(merge((o11 * inv[0], o12 * inv[0], o21 * inv[1], o22 * inv[1]), wva)):
            rows, cols = (q // 2) * HB, slice((q % 2) * HD, (q % 2 + 1) * HD)
            res = x_buf[b, pl.ds(r0 + rows, HB), cols].astype(F32) + y_buf[q, pl.ds(z8, HB), :]
            o_buf[slot, rows:rows + HB, cols] = (v + res).astype(o_buf.dtype)
        o_copy(n, slot).start()
        return carry

    lax.fori_loop(0, NB, body, 0)
    o_copy(NB - 2, (NB - 2) % 2).wait()
    o_copy(NB - 1, (NB - 1) % 2).wait()


def make(BQ=800, BK=256, CR=16, LR=32, PK=0, MC=0, XC=6, MORDER=(4, 2, 1, 0, 3, 5, 6), ORDER=(1, 4, 0, 3, 2, 5, 6), flags=None):
    def fn(x, w_q, w_k, w_v, w_ao, w_up, dw, w_dn, w_merge):
        B, T, D = x.shape
        KW = dw.shape[0]
        TP = -(-(T // 2) // BK) * BK
        NL = D // LANES
        NQ = T // BQ
        HB, HD = BQ // 2, D // 2
        kern = functools.partial(_kernel, B=B, T=T, D=D, KW=KW, BQ=BQ, BK=BK, TP=TP, CR=CR, LR=LR, ORDER=ORDER, MORDER=MORDER, PK=PK, MC=MC, XC=XC)
        any_spec = pl.BlockSpec(memory_space=pl.ANY)
        V = pltpu.VMEM
        E = PAD
        scratch = [
            V((B, T + E, D), BF16), V((B * (NQ - 1) * HALO, D), BF16),
            V((B, 7, TP // 2 + E, HD), U32),
            V((11, D, D), BF16), V((KW, D), BF16), V((5, D, D), F32), V((5, 7, HD // 2, HD), U32),
            V((B * NQ, HALO, D), F32),
            V((5 * NL, BQ + 2 * HALO + E, LANES), F32), V((7, HB // 2 + E, HD), U32),
            V((BQ + E, TP), F32), V((BQ + E, TP), F32),
            V((8, HB + E, HD), F32), V((8, HB + E, HD), F32),
            V((4, HB + E, HD), F32), V((7, HB // 2 + E, HD), U32),
            V((2, BQ, D), BF16),
            pltpu.SemaphoreType.DMA((B * NQ,)), pltpu.SemaphoreType.DMA(()),
            pltpu.SemaphoreType.DMA((10,)), pltpu.SemaphoreType.DMA((2,)),
        ]
        return pl.pallas_call(
            kern,
            out_shape=jax.ShapeDtypeStruct((B, T, D), x.dtype),
            in_specs=[any_spec] * 9,
            out_specs=any_spec,
            scratch_shapes=scratch,
            compiler_params=pltpu.CompilerParams(vmem_limit_bytes=110 * 1024 * 1024, flags=flags),
        )(x, w_q, w_k, w_v, w_ao, w_up, dw, w_dn, w_merge)
    return fn


_branchformer = make()


@jax.jit
def pallas_standalone__conformer_family_branchformer__speech_kernel(
    x: jax.Array,
    w_q: jax.Array,
    w_k: jax.Array,
    w_v: jax.Array,
    w_ao: jax.Array,
    w_up: jax.Array,
    dw: jax.Array,
    w_dn: jax.Array,
    w_merge: jax.Array,
):
    return _branchformer(x, w_q, w_k, w_v, w_ao, w_up, dw, w_dn, w_merge)
```

```python
import functools
import math
import jax
import jax.numpy as jnp
from jax import lax
from jax.experimental import pallas as pl
from jax.experimental.pallas import tpu as pltpu

F32 = jnp.float32
BF16 = jnp.bfloat16
U32 = jnp.uint32
EPS = 1e-5
LANES = 128
HALO = 16
PAD = 16


def _ln(x):
    d = x.shape[-1]
    m = jnp.sum(x, axis=-1, keepdims=True) * (1.0 / d)
    c = x - m
    v = jnp.sum(c * c, axis=-1, keepdims=True) * (1.0 / d)
    return c * lax.rsqrt(v + EPS)


def _gelu(x):
    c1 = math.sqrt(2.0 / math.pi)
    c2 = c1 * 0.044715
    t = jnp.tanh(x * (c1 + c2 * (x * x)))
    hx = 0.5 * x
    return hx + hx * t


def _dot(a, b):
    return jnp.dot(a, b, preferred_element_type=F32)


def _dot_nt(a, b):
    return lax.dot_general(a, b, (((1,), (1,)), ((), ())), preferred_element_type=F32)


def _pack(v):
    return pltpu.bitcast(v.astype(BF16), U32)


def _unpack(w):
    return pltpu.bitcast(w, BF16)


def _combos(a11, a12, a21, a22):
    return [a11 + a22, a11, a22, a21 - a22, a12 - a11, a11 + a21, a12 + a22]


PAIRS = ((0, 0), (1, 6), (3, 1), (4, 2), (2, 5), (5, 4), (6, 3))


def _combine(n):
    return (n[0] - n[4] + n[3] + n[6], n[1] + n[3], n[4] + n[2], n[0] - n[1] + n[2] + n[5])


def _kernel(x_hbm, wq_hbm, wk_hbm, wv_hbm, wao_hbm, wup_hbm, dw_hbm, wdn_hbm, wm_hbm,
            o_hbm,
            x_buf, xh_buf, xs_all, wst, dw_in, wf32, wc, g_first, cb, xn_buf,
            s_e, s_o, a_e, a_o, y_buf, q_buf, o_buf,
            x_sem, h_sem, w_sem, o_sem, *, B, T, D, KW, BQ, BK, TP, CR, LR, ORDER, MORDER, PK, MC, XC, SKIP, QSSA, LC, GU, SORDER):
    NQ = T // BQ
    NB = B * NQ
    NL = D // LANES
    NC = TP // BK
    HB = BQ // 2
    HD = D // 2
    G, U, W, Z = (NL * j for j in range(4))

    def x_copy(n):
        b, i = n // NQ, n % NQ
        r = pl.ds(pl.multiple_of(i * BQ, BQ), BQ)
        return pltpu.make_async_copy(x_hbm.at[b, r, :], x_buf.at[b, r, :], x_sem.at[n])

    def o_copy(n, slot):
        b, i = n // NQ, n % NQ
        r = pl.ds(pl.multiple_of(i * BQ, BQ), BQ)
        return pltpu.make_async_copy(o_buf.at[slot], o_hbm.at[b, r, :], o_sem.at[slot])

    heads = [(b, i) for b in range(B) for i in range(1, NQ)]
    h_copies = [pltpu.make_async_copy(x_hbm.at[b, i * BQ:i * BQ + HALO, :],
                                      xh_buf.at[j * HALO:(j + 1) * HALO, :], h_sem)
                for j, (b, i) in enumerate(heads)]
    WQ, WK, WV, WAO, WMA, WDN, WMC, WU, WG, W1, XH = range(11)
    w_src = [wq_hbm, wk_hbm, wv_hbm, wao_hbm, wm_hbm.at[0:D], wdn_hbm, wm_hbm.at[D:2 * D],
             wup_hbm.at[:, 0:D], wup_hbm.at[:, D:2 * D]]
    w_copies = [pltpu.make_async_copy(src, wst.at[j], w_sem.at[j]) for j, src in enumerate(w_src)]
    dw_copy = pltpu.make_async_copy(dw_hbm, dw_in, w_sem.at[len(w_src)])
    QK, VA, DC, UU, GG = range(5)
    RB = HALO * len(heads)
    NRB = D // RB

    def ln_rows(b, r0, t0, nrows):
        top = _ln(x_buf[b, pl.ds(r0 + t0, nrows), :].astype(F32))
        bot = _ln(x_buf[b, pl.ds(r0 + HB + t0, nrows), :].astype(F32))
        return [_pack(v) for v in _combos(top[:, :HD], top[:, HD:], bot[:, :HD], bot[:, HD:])]

    for j in (WQ, WK, WV, WAO):
        w_copies[j].start()
    for b in range(B):
        xs_all[b, :, T // 4:TP // 2, :] = jnp.zeros((7, TP // 2 - T // 4, HD), U32)
    cb[G:G + NL, BQ:BQ + HALO, :] = jnp.zeros((NL, HALO, LANES), F32)
    w_copies[WQ].wait()
    w_copies[WK].wait()
    for j in (WMA, WDN, WMC):
        w_copies[j].start()

    def fold_qk(t, c):
        r = pl.ds(pl.multiple_of(t * RB, RB), RB)
        wf32[QK, r, :] = _dot_nt(wst[WQ, r, :], wst[WK]) * (math.log2(math.e) / math.sqrt(D))
        return c
    lax.fori_loop(0, NRB, fold_qk, 0)

    w_copies[WV].wait()
    w_copies[WAO].wait()
    for c in [w_copies[WU], w_copies[WG], dw_copy, x_copy(0)] + h_copies:
        c.start()

    def fold(t, c):
        j = t // NRB

        @pl.when(t == NRB)
        def _():
            for k in (WMA, WDN, WMC):
                w_copies[k].wait()
            x_copy(1).start()
            x_copy(2).start()

        @pl.when(t == 3 * NRB)
        def _():
            for cp in [w_copies[WU], w_copies[WG], dw_copy] + h_copies:
                cp.wait()
            for n in range(3, NQ):
                x_copy(n).start()
            wst[XH, 0:RB, :] = _ln(xh_buf[...].astype(F32)).astype(BF16)

        left = jnp.where(j == 0, WV, jnp.where(j == 1, W1, jnp.where(j == 2, WDN, XH)))
        right = jnp.where(j == 0, WAO, jnp.where(j == 1, WMA, jnp.where(j == 2, WMC, WG)))
        r = pl.ds(pl.multiple_of((t % NRB) * RB, RB), RB)
        v = _dot(wst[left, r, :], wst[right])
        wf32[jnp.where(j == 1, VA, jnp.where(j == 2, DC, UU)), r, :] = v
        wst[jnp.where(j == 0, W1, WQ), r, :] = v.astype(BF16)
        return c
    lax.fori_loop(0, 3 * NRB + 1, fold, 0)

    gf = _ln(_gelu(wf32[UU, 0:RB, :]))
    for j, (b, i) in enumerate(heads):
        g_first[b * NQ + i - 1] = gf[j * HALO:(j + 1) * HALO]
    for b in range(B):
        g_first[b * NQ + NQ - 1] = jnp.zeros((HALO, D), F32)

    def widen(t, c):
        j, r = t // NRB, pl.ds(pl.multiple_of((t % NRB) * RB, RB), RB)
        wf32[UU + j, r, :] = wst[WU + j, r, :].astype(F32)
        return c
    lax.fori_loop(0, 2 * NRB, widen, 0)

    def split(t, c):
        j, t0 = t // 2, pl.multiple_of((t % 2) * (HD // 2), HD // 2)
        top, bot = pl.ds(t0, HD // 2), pl.ds(HD + t0, HD // 2)
        quads = wf32[j, top, 0:HD], wf32[j, top, HD:D], wf32[j, bot, 0:HD], wf32[j, bot, HD:D]
        for k, v in enumerate(_combos(*quads)):
            wc[j, k, pl.ds(pl.multiple_of(t0 // 2, HD // 4), HD // 4), :] = _pack(v)
        return c
    lax.fori_loop(0, 10, split, 0)

    for l in range(NL):
        cb[Z + l, 0:KW, :] = dw_in[:, l * LANES:(l + 1) * LANES].astype(F32)

    def taps(k, c):
        for l in range(NL):
            cb[W + l, pl.ds(pl.multiple_of(8 * k, 8), 8), :] = jnp.broadcast_to(
                cb[Z + l, pl.ds(k, 1), :], (8, LANES))
        return c
    lax.fori_loop(0, KW, taps, 0)

    def ln_body(n, c):
        x_copy(n).wait()
        for j, v in enumerate(ln_rows(0, pl.multiple_of(n * BQ, BQ), 0, HB)):
            xs_all[0, j, pl.ds(pl.multiple_of(n * (HB // 2), HB // 2), HB // 2), :] = v
        return c
    lax.fori_loop(0, NQ, ln_body, 0)
    x_copy(NQ).start()
    wqk, wva, wdc, wu, wg = (wc.at[j] for j in (QK, VA, DC, UU, GG))

    s_par = (s_e, s_o)
    a_par = (a_e, a_o)
    SW = TP // 2

    def body(n, carry):
        b, i = n // NQ, n % NQ
        xs = xs_all.at[b]
        slot = n % 2
        r0 = pl.multiple_of(i * BQ, BQ)
        h0 = pl.multiple_of(i * (HB // 2), HB // 2)

        @pl.when(n + NQ < NB)
        def _():
            x_copy(n + NQ).wait()

        @pl.when(n + NQ + 1 < NB)
        def _():
            x_copy(n + NQ + 1).start()

        @pl.when(n >= 2)
        def _():
            o_copy(n - 2, slot).wait()

        first = i == 0
        z8 = pl.multiple_of((n // NB) * 16, 16)
        zf = pl.multiple_of((n // (NB + 1)) * 16, 16)

        def pin(dst, v):
            lead = (0,) * (len(dst.shape) - 2)
            rows = 8 * (4 // jnp.dtype(dst.dtype).itemsize)
            v = pltpu.bitcast(v[v.shape[0] - 8:, :LANES], dst.dtype)
            dst[lead + (pl.ds(dst.shape[-2] - rows + zf, rows), slice(0, LANES))] = v

        def project(w):
            out = [None] * 7
            for k in ORDER:
                l, r = PAIRS[k]
                out[k] = _dot(_unpack(xs[l, pl.ds(h0, HB // 2), :]), _unpack(w[r]))
            return _combine(out)

        def put_quads(base, row0, quads):
            for q, v in enumerate(quads):
                for l in range(NL // 2):
                    cb[base + (q % 2) * (NL // 2) + l, row0 + (q // 2) * HB:row0 + (q // 2 + 1) * HB, :] = (
                        v[:, l * LANES:(l + 1) * LANES])

        for l in range(NL):
            ls = slice(l * LANES, (l + 1) * LANES)
            cb[G + l, 0:HALO, :] = jnp.where(first, 0.0, cb[G + l, BQ:BQ + HALO, :])
            cb[G + l, BQ + HALO:BQ + 2 * HALO, :] = g_first[n, :, ls]

        put_quads(U, 0, [v if GU else _gelu(v) for v in project(wu)])
        g11, g12, g21, g22 = (_gelu(v) for v in project(wg))
        for h, halves in ((1, (g21, g22)), (0, (g11, g12))):
            g = _ln(jnp.concatenate(halves, axis=1))
            for l in range(NL):
                cb[G + l, HALO + h * HB:HALO + (h + 1) * HB, :] = g[:, l * LANES:(l + 1) * LANES]
        pin(cb, g)
        a11, a12, a21, a22 = project(wqk)
        qs = [a11 + a22, a21 + a22, a11, a22, a11 + a12, a21 - a11, a12 - a22]
        if QSSA:
            qs = [v.astype(BF16) for v in qs]
        else:
            for j, v in enumerate(qs):
                q_buf[j, 0:HB // 2, :] = _pack(v)

        def conv_rows(l, t0, nr):
            acc = [None] * nr
            off = HALO - KW // 2
            for s in range(8):
                taps = [(a, 8 * a + s - off) for a in range((KW + off + 7) // 8)
                        if 0 <= 8 * a + s - off < KW]
                w = {a: cb[W + l, 8 * k:8 * k + 8, :] for a, k in taps}
                for j in range(nr + max(a for a, _ in taps)):
                    use = [a for a, _ in taps if 0 <= j - a < nr]
                    if not use:
                        continue
                    gv = cb[G + l, t0 + 8 * j + s:t0 + 8 * j + s + 8, :]
                    for a in use:
                        t = gv * w[a]
                        acc[j - a] = t if acc[j - a] is None else acc[j - a] + t
            return acc * 1

        def conv_piece(l, t0, nrows):
            cv = jnp.concatenate(conv_rows(l, t0, nrows // 8), axis=0)
            cb[Z + l, pl.ds(zf + t0, nrows), :] = cv * (_gelu if GU else (lambda v: v))(cb[U + l, t0:t0 + nrows, :])

        for t0 in range(0, BQ, CR):
            for l in range(NL if 'conv' not in SKIP else 0):
                conv_piece(l, t0, min(CR, BQ - t0))

        bn = (b + 1) % B

        def ln_next():
            for t0 in range(0, HB, LR):
                nrows = min(LR, HB - t0)
                for j, v in enumerate(ln_rows(bn, r0, t0, nrows)):
                    xn_buf[j, t0 // 2:(t0 + nrows) // 2, :] = v
                pin(x_buf if t0 + LR < HB else xs, xn_buf[0, pl.ds(z8, 8), :])

        def kv(j, c):
            return _unpack(xs[j, c * BK // 2:(c + 1) * BK // 2, :])

        m = [None, None]
        for c in range(NC):
            if c == LC:
                ln_next()
            M = [None] * 7
            for j in SORDER:
                lhs = qs[j] if QSSA else _unpack(q_buf[j, pl.ds(z8, HB // 2), :])
                M[j] = _dot_nt(lhs, kv((0, 1, 3, 4, 2, 5, 6)[j], c))
            quads = (M[0] - M[4] + M[3] + M[6], M[4] + M[2], M[1] + M[3], M[0] - M[1] + M[2] + M[5])
            for q, s in enumerate(quads):
                if (c + 1) * BK > T // 2:
                    col = lax.broadcasted_iota(jnp.int32, (HB, BK), 1)
                    s = jnp.where(col < T // 2 - c * BK, s, -jnp.inf)
                c0 = (q % 2) * SW + (c // 2) * BK
                s_par[c % 2][(q // 2) * HB:(q // 2 + 1) * HB, c0:c0 + BK] = s
                for l in range(BK // LANES):
                    t = s[:, l * LANES:(l + 1) * LANES]
                    m[q // 2] = t if m[q // 2] is None else jnp.maximum(m[q // 2], t)
        for h in range(2):
            mx = jnp.max(m[h], axis=-1, keepdims=True)
            m[h] = mx + jnp.log2(jnp.sum(jnp.exp2(m[h] - mx), axis=-1, keepdims=True))

        def merge(quads, w):
            left = _combos(*quads)
            out = [None] * 7
            for k in MORDER:
                l, r = PAIRS[k]
                out[k] = _dot(left[l].astype(BF16), _unpack(w[r, 0:HD // 2, :]))
            return _combine(out)

        def merge_conv():
            zq = [jnp.concatenate([cb[Z + (q % 2) * (NL // 2) + l, pl.ds(z8 + (q // 2) * HB, HB), :]
                                   for l in range(NL // 2)], axis=1) for q in range(4)]
            for q, v in enumerate(merge(zq, wdc)):
                rows, cols = (q // 2) * HB, slice((q % 2) * HD, (q % 2 + 1) * HD)
                y_buf[q, 0:HB, :] = v + x_buf[b, pl.ds(r0 + rows, HB), cols].astype(F32)

        def probs(c):
            p, part = [], [None, None]
            for q in range(4):
                c0 = (q % 2) * SW + (c // 2) * BK
                e = jnp.exp2(s_par[c % 2][pl.ds(z8 + (q // 2) * HB, HB), c0:c0 + BK] - m[q // 2])
                for l in range(BK // LANES):
                    t = e[:, l * LANES:(l + 1) * LANES]
                    part[q // 2] = t if part[q // 2] is None else part[q // 2] + t
                p.append(e)
            return [v.astype(BF16) for v in _combos(*p)], jnp.concatenate(part, axis=1)

        def accumulate(c, k, d):
            if c > 0:
                d = d + a_par[(c - 1) % 2][k, pl.ds(z8, HB), :]
            if c + 1 < NC:
                a_par[c % 2][k, 0:HB, :] = d
            return d

        nxt = probs(0)
        for c in range(NC):
            if c == MC:
                merge_conv()
            if c + NC == LC:
                ln_next()
            p, part = nxt
            acc = [None] * 7
            for kk, k in enumerate(ORDER):
                l, r = PAIRS[k]
                d = _dot(p[l], kv(r, c))
                if kk == PK and c + 1 < NC:
                    pin(s_par[(c + 1) % 2], d)
                    nxt = probs(c + 1)
                acc[k] = accumulate(c, k, d)
            lsum = accumulate(c, 7, part)
        lsum = [lsum[:, :LANES], lsum[:, LANES:]]
        o11, o12, o21, o22 = _combine(acc)
        inv = [1.0 / jnp.sum(v, axis=-1, keepdims=True) for v in lsum]
        pin(xn_buf, acc[ORDER[XC]])
        for j in range(7):
            xs_all[bn, j, pl.ds(h0, HB // 2), :] = xn_buf[j, pl.ds(z8, HB // 2), :]
        for q, v in enumerate(merge((o11 * inv[0], o12 * inv[0], o21 * inv[1], o22 * inv[1]), wva)):
            rows, cols = (q // 2) * HB, slice((q % 2) * HD, (q % 2 + 1) * HD)
            o_buf[slot, rows:rows + HB, cols] = (v + y_buf[q, pl.ds(z8, HB), :]).astype(o_buf.dtype)
        o_copy(n, slot).start()
        return carry

    lax.fori_loop(0, NB, body, 0)
    o_copy(NB - 2, (NB - 2) % 2).wait()
    o_copy(NB - 1, (NB - 1) % 2).wait()


def make(BQ=800, BK=256, CR=24, LR=32, SP=0, AP=0, SKIP=(), QSSA=1, LC=12, GU=0, SORDER=(1, 4, 0, 3, 2, 5, 6), PK=0, MC=0, XC=6, MORDER=(4, 2, 1, 0, 3, 5, 6), ORDER=(1, 4, 0, 3, 2, 5, 6), flags=None):
    def fn(x, w_q, w_k, w_v, w_ao, w_up, dw, w_dn, w_merge):
        B, T, D = x.shape
        KW = dw.shape[0]
        TP = -(-(T // 2) // BK) * BK
        NL = D // LANES
        NQ = T // BQ
        HB, HD = BQ // 2, D // 2
        kern = functools.partial(_kernel, B=B, T=T, D=D, KW=KW, BQ=BQ, BK=BK, TP=TP, CR=CR, LR=LR, ORDER=ORDER, MORDER=MORDER, PK=PK, MC=MC, XC=XC, SKIP=SKIP, QSSA=QSSA, LC=LC, GU=GU, SORDER=SORDER)
        any_spec = pl.BlockSpec(memory_space=pl.ANY)
        V = pltpu.VMEM
        E = PAD
        scratch = [
            V((B, T + E, D), BF16), V((B * (NQ - 1) * HALO, D), BF16),
            V((B, 7, TP // 2 + E, HD), U32),
            V((11, D, D), BF16), V((KW, D), BF16), V((5, D, D), F32), V((5, 7, HD // 2, HD), U32),
            V((B * NQ, HALO, D), F32),
            V((4 * NL, BQ + 2 * HALO + E, LANES), F32), V((7, HB // 2 + E, HD), U32),
            V((BQ + E, TP + SP), F32), V((BQ + E, TP + SP), F32),
            V((8, HB + E + AP, HD), F32), V((8, HB + E + AP, HD), F32),
            V((4, HB + E, HD), F32), V((7, HB // 2 + E, HD), U32),
            V((2, BQ, D), BF16),
            pltpu.SemaphoreType.DMA((B * NQ,)), pltpu.SemaphoreType.DMA(()),
            pltpu.SemaphoreType.DMA((10,)), pltpu.SemaphoreType.DMA((2,)),
        ]
        return pl.pallas_call(
            kern,
            out_shape=jax.ShapeDtypeStruct((B, T, D), x.dtype),
            in_specs=[any_spec] * 9,
            out_specs=any_spec,
            scratch_shapes=scratch,
            compiler_params=pltpu.CompilerParams(vmem_limit_bytes=110 * 1024 * 1024, flags=flags),
        )(x, w_q, w_k, w_v, w_ao, w_up, dw, w_dn, w_merge)
    return fn


_branchformer = make(CR=24, GU=1)


@jax.jit
def pallas_standalone__conformer_family_branchformer__speech_kernel(
    x: jax.Array,
    w_q: jax.Array,
    w_k: jax.Array,
    w_v: jax.Array,
    w_ao: jax.Array,
    w_up: jax.Array,
    dw: jax.Array,
    w_dn: jax.Array,
    w_merge: jax.Array,
):
    return _branchformer(x, w_q, w_k, w_v, w_ao, w_up, dw, w_dn, w_merge)
```

```python
import functools
import math
import jax
import jax.numpy as jnp
from jax import lax
from jax.experimental import pallas as pl
from jax.experimental.pallas import tpu as pltpu

F32 = jnp.float32
BF16 = jnp.bfloat16
U32 = jnp.uint32
EPS = 1e-5
LANES = 128
HALO = 16
PAD = 16


def _ln(x):
    d = x.shape[-1]
    m = jnp.sum(x, axis=-1, keepdims=True) * (1.0 / d)
    c = x - m
    v = jnp.sum(c * c, axis=-1, keepdims=True) * (1.0 / d)
    return c * lax.rsqrt(v + EPS)


def _gelu(x):
    c1 = math.sqrt(2.0 / math.pi)
    c2 = c1 * 0.044715
    t = jnp.tanh(x * (c1 + c2 * (x * x)))
    hx = 0.5 * x
    return hx + hx * t


def _dot(a, b):
    return jnp.dot(a, b, preferred_element_type=F32)


def _dot_nt(a, b):
    return lax.dot_general(a, b, (((1,), (1,)), ((), ())), preferred_element_type=F32)


def _pack(v):
    return pltpu.bitcast(v.astype(BF16), U32)


def _unpack(w):
    return pltpu.bitcast(w, BF16)


def _pack_rows(pair):
    return pltpu.bitcast(pltpu.pack_elementwise(pair, packed_dtype=BF16), U32)


def _unpack_rows(w, parity):
    return pltpu.unpack_elementwise(w, index=parity, packed_dtype=BF16, unpacked_dtype=F32)


def _combos(a11, a12, a21, a22):
    return [a11 + a22, a11, a22, a21 - a22, a12 - a11, a11 + a21, a12 + a22]


PAIRS = ((0, 0), (1, 6), (3, 1), (4, 2), (2, 5), (5, 4), (6, 3))


def _combine(n):
    return (n[0] - n[4] + n[3] + n[6], n[1] + n[3], n[4] + n[2], n[0] - n[1] + n[2] + n[5])


def _pin(dst, v, zero):
    lead = (0,) * (len(dst.shape) - 2)
    rows = 8 * (4 // jnp.dtype(dst.dtype).itemsize)
    v = pltpu.bitcast(v[v.shape[0] - 8:, :LANES], dst.dtype)
    dst[lead + (pl.ds(dst.shape[-2] - rows + zero, rows), slice(0, LANES))] = v


def _kernel(x_hbm, wq_hbm, wk_hbm, wv_hbm, wao_hbm, wup_hbm, dw_hbm, wdn_hbm, wm_hbm,
            o_hbm,
            x_buf, xh_buf, xs_all, wst, dw_in, wf32, wc, g_first, cb, xn_buf,
            s_e, s_o, a_e, a_o, y_buf, q_buf, o_buf,
            x_sem, h_sem, w_sem, o_sem, *, B, T, D, KW, BQ, BK, TP, CR, LR, ORDER, MORDER, PK, MC, XC, GP, GB, SKIP, QSSA, LC, GU, SORDER):
    NQ = T // BQ
    NB = B * NQ
    NL = D // LANES
    NC = TP // BK
    HB = BQ // 2
    HD = D // 2
    G, U, W, Z = (NL * j for j in range(4))

    def x_copy(n):
        b, i = n // NQ, n % NQ
        r = pl.ds(pl.multiple_of(i * BQ, BQ), BQ)
        return pltpu.make_async_copy(x_hbm.at[b, r, :], x_buf.at[b, r, :], x_sem.at[n])

    def o_copy(n, slot):
        b, i = n // NQ, n % NQ
        r = pl.ds(pl.multiple_of(i * BQ, BQ), BQ)
        return pltpu.make_async_copy(o_buf.at[slot], o_hbm.at[b, r, :], o_sem.at[slot])

    heads = [(b, i) for b in range(B) for i in range(1, NQ)]
    h_copies = [pltpu.make_async_copy(x_hbm.at[b, i * BQ:i * BQ + HALO, :],
                                      xh_buf.at[j * HALO:(j + 1) * HALO, :], h_sem)
                for j, (b, i) in enumerate(heads)]
    WQ, WK, WV, WAO, WMA, WDN, WMC, WU, WG, W1, XH = range(11)
    w_src = [wq_hbm, wk_hbm, wv_hbm, wao_hbm, wm_hbm.at[0:D], wdn_hbm, wm_hbm.at[D:2 * D],
             wup_hbm.at[:, 0:D], wup_hbm.at[:, D:2 * D]]
    w_copies = [pltpu.make_async_copy(src, wst.at[j], w_sem.at[j]) for j, src in enumerate(w_src)]
    dw_copy = pltpu.make_async_copy(dw_hbm, dw_in, w_sem.at[len(w_src)])
    QK, VA, DC, UU, GG = range(5)
    RB = HALO * len(heads)
    NRB = D // RB

    def ln_rows(b, r0, t0, nrows):
        words = [pltpu.bitcast(x_buf[b, pl.ds(r0 + h * HB + t0, nrows), :], U32) for h in range(2)]
        ops = []
        for parity in range(2):
            top, bot = (_ln(_unpack_rows(w, parity)) for w in words)
            ops.append(_combos(top[:, :HD], top[:, HD:], bot[:, :HD], bot[:, HD:]))
        return [_pack_rows(pair) for pair in zip(*ops)]

    for c in (w_copies[WQ], w_copies[WK], dw_copy, w_copies[WV], w_copies[WAO]):
        c.start()
    for b in range(B):
        xs_all[b, :, T // 4:TP // 2, :] = jnp.zeros((7, TP // 2 - T // 4, HD), U32)
    cb[G:G + NL, BQ:BQ + HALO, :] = jnp.zeros((NL, HALO, LANES), F32)
    for b in range(B):
        g_first[b * NQ + NQ - 1] = jnp.zeros((HALO, D), F32)
    w_copies[WQ].wait()
    w_copies[WK].wait()
    x_copy(0).start()
    x_copy(1).start()

    def put_folded(j, r, v):
        for l in range(NL):
            wf32[j, l, r, :] = v[:, l * LANES:(l + 1) * LANES]

    def fold_qk(t, c):
        r = pl.ds(pl.multiple_of(t * RB, RB), RB)
        put_folded(QK, r, _dot_nt(wst[WQ, r, :], wst[WK]) * (math.log2(math.e) / math.sqrt(D)))
        return c
    lax.fori_loop(0, NRB, fold_qk, 0)

    def put_operands(j, t0, parts):
        ops = [_combos(top[:, :HD], top[:, HD:], bot[:, :HD], bot[:, HD:]) for top, bot in parts]
        for k, pair in enumerate(zip(*ops)):
            wc[j, k, pl.ds(pl.multiple_of(t0 // 2, HD // 4), HD // 4), :] = _pack_rows(pair)

    def split_folded(t, c):
        j, t0 = t // 2, (t % 2) * (HD // 2)
        put_operands(j, t0, [[jnp.concatenate(
            [wf32[j, l, pl.ds(h * HD + t0 + parity, HD // 4, stride=2), :] for l in range(NL)], axis=1)
            for h in range(2)] for parity in range(2)])
        return c
    lax.fori_loop(0, 2, split_folded, 0)

    dw_copy.wait()
    for l in range(NL):
        cb[Z + l, 0:KW, :] = dw_in[:, l * LANES:(l + 1) * LANES].astype(F32)

    def taps(k, c):
        for l in range(NL):
            cb[W + l, pl.ds(pl.multiple_of(8 * k, 8), 8), :] = jnp.broadcast_to(
                cb[Z + l, pl.ds(k, 1), :], (8, LANES))
        return c
    lax.fori_loop(0, KW, taps, 0)

    PB = HB // HALO

    def ln_first(u0, count, last):
        for u in (jnp.minimum(u0 + k, last) for k in range(count)):
            r0 = pl.multiple_of((u // PB) * BQ + (u % PB) * HALO, HALO)
            for k, v in enumerate(ln_rows(0, r0, 0, HALO)):
                xs_all[0, k, pl.ds(pl.multiple_of(u * (HALO // 2), HALO // 2), HALO // 2), :] = v

    NF = 3 * NRB + 1
    PF = -(-(NQ - 1) * PB // NF)
    assert NQ == 5 and (PB // PF, 2 * PB // PF, 3 * PB // PF) == (3, 6, 9) and NRB == 4
    arrivals = {
        0: ([w_copies[WV], w_copies[WAO], x_copy(0)], [w_copies[WMA], x_copy(2)]),
        3: ([x_copy(1)], [w_copies[WDN], w_copies[WMC]]),
        4: ([w_copies[WMA]], [x_copy(3)]),
        6: ([x_copy(2)], [w_copies[WG]] + h_copies),
        8: ([w_copies[WDN], w_copies[WMC]], [w_copies[WU], x_copy(4)]),
        9: ([x_copy(3)], []),
    }

    def fold(t, c):
        for step, (done, new) in arrivals.items():
            @pl.when(t == step)
            def _():
                for cp in done:
                    cp.wait()
                for cp in new:
                    cp.start()

        @pl.when(t == NF - 1)
        def _():
            for cp in [w_copies[WG]] + h_copies:
                cp.wait()
            x_copy(NQ).start()
            wst[XH, 0:RB, :] = _ln(xh_buf[...].astype(F32)).astype(BF16)

        j = t // NRB
        left = jnp.where(j == 0, WV, jnp.where(j == 1, W1, jnp.where(j == 2, WDN, XH)))
        right = jnp.where(j == 0, WAO, jnp.where(j == 1, WMA, jnp.where(j == 2, WMC, WG)))
        r = pl.ds(pl.multiple_of((t % NRB) * RB, RB), RB)
        v = _dot(wst[left, r, :], wst[right])
        put_folded(jnp.where(j == 1, VA, jnp.where(j == 2, DC, QK)), r, v)
        wst[jnp.where(j == 0, W1, WQ), r, :] = v.astype(BF16)
        ln_first(PF * t, PF, (NQ - 1) * PB - 1)
        return c
    lax.fori_loop(0, NF, fold, 0)

    gf = _ln(_gelu(jnp.concatenate([wf32[QK, l, 0:RB, :] for l in range(NL)], axis=1)))
    for j, (b, i) in enumerate(heads):
        g_first[b * NQ + i - 1] = gf[j * HALO:(j + 1) * HALO]
    lax.fori_loop(2, 6, split_folded, 0)
    w_copies[WU].wait()

    def split_plain(t, c):
        j, t0 = t // 2, (t % 2) * (HD // 2)
        words = [pltpu.bitcast(wst[WU + j, pl.ds(pl.multiple_of(h * HD + t0, HD // 2), HD // 2), :], U32)
                 for h in range(2)]
        put_operands(UU + j, t0, [[_unpack_rows(w, parity) for w in words] for parity in range(2)])
        return c
    lax.fori_loop(0, 4, split_plain, 0)

    x_copy(NQ - 1).wait()

    def ln_last(t, c):
        ln_first((NQ - 1) * PB + 5 * t, 5, NQ * PB - 1)
        return c
    lax.fori_loop(0, PB // 5, ln_last, 0)
    wqk, wva, wdc, wu, wg = (wc.at[j] for j in (QK, VA, DC, UU, GG))

    s_par = (s_e, s_o)
    a_par = (a_e, a_o)
    SW = TP // 2

    def body(n, carry):
        b, i = n // NQ, n % NQ
        xs = xs_all.at[b]
        slot = n % 2
        r0 = pl.multiple_of(i * BQ, BQ)
        h0 = pl.multiple_of(i * (HB // 2), HB // 2)

        @pl.when(n + NQ < NB)
        def _():
            x_copy(n + NQ).wait()

        @pl.when(n + NQ + 1 < NB)
        def _():
            x_copy(n + NQ + 1).start()

        @pl.when(n >= 2)
        def _():
            o_copy(n - 2, slot).wait()

        first = i == 0
        z8 = pl.multiple_of((n // NB) * 16, 16)
        zf = pl.multiple_of((n // (NB + 1)) * 16, 16)

        pin = functools.partial(_pin, zero=zf)

        def project(w, order=ORDER):
            out = [None] * 7
            for k in order:
                l, r = PAIRS[k]
                out[k] = _dot(_unpack(xs[l, pl.ds(h0, HB // 2), :]), _unpack(w[r]))
            return _combine(out)

        def put_quads(base, row0, quads):
            for q, v in enumerate(quads):
                for l in range(NL // 2):
                    cb[base + (q % 2) * (NL // 2) + l, row0 + (q // 2) * HB:row0 + (q // 2 + 1) * HB, :] = (
                        v[:, l * LANES:(l + 1) * LANES])

        for l in range(NL):
            ls = slice(l * LANES, (l + 1) * LANES)
            cb[G + l, 0:HALO, :] = jnp.where(first, 0.0, cb[G + l, BQ:BQ + HALO, :])
            cb[G + l, BQ + HALO:BQ + 2 * HALO, :] = g_first[n, :, ls]

        put_quads(U, 0, [v if GU else _gelu(v) for v in project(wu)])
        g11, g12, g21, g22 = (_gelu(v) for v in project(wg, (3, 1, 4, 0, 6, 2, 5)))

        def put_gate(t0, h):
            g = _ln(h)
            for l in range(NL):
                cb[G + l, HALO + t0:HALO + t0 + h.shape[0], :] = g[:, l * LANES:(l + 1) * LANES]
            return g

        g = put_gate(0, jnp.concatenate([g11, g12], axis=1))
        g2 = jnp.concatenate([g21, g22], axis=1)
        if GP == 0:
            g = put_gate(HB, g2)
        pin(cb, g)
        a11, a12, a21, a22 = project(wqk)
        qs = [a11 + a22, a21 + a22, a11, a22, a11 + a12, a21 - a11, a12 - a22]
        if QSSA:
            qs = [v.astype(BF16) for v in qs]
        else:
            for j, v in enumerate(qs):
                q_buf[j, 0:HB // 2, :] = _pack(v)

        def conv_rows(l, t0, nr):
            acc = [None] * nr
            off = HALO - KW // 2
            for s in range(8):
                taps = [(a, 8 * a + s - off) for a in range((KW + off + 7) // 8)
                        if 0 <= 8 * a + s - off < KW]
                w = {a: cb[W + l, 8 * k:8 * k + 8, :] for a, k in taps}
                for j in range(nr + max(a for a, _ in taps)):
                    use = [a for a, _ in taps if 0 <= j - a < nr]
                    if not use:
                        continue
                    gv = cb[G + l, t0 + 8 * j + s:t0 + 8 * j + s + 8, :]
                    for a in use:
                        t = gv * w[a]
                        acc[j - a] = t if acc[j - a] is None else acc[j - a] + t
            return acc * 1

        def conv_piece(l, t0, nrows):
            cv = jnp.concatenate(conv_rows(l, t0, nrows // 8), axis=0)
            cb[Z + l, pl.ds(zf + t0, nrows), :] = cv * (_gelu if GU else (lambda v: v))(cb[U + l, t0:t0 + nrows, :])

        for t0 in range(0, BQ, CR):
            k = t0 // CR - GB
            if GP and 0 <= k < HB // GP:
                put_gate(HB + k * GP, g2[k * GP:(k + 1) * GP])
            for l in range(NL if 'conv' not in SKIP else 0):
                conv_piece(l, t0, min(CR, BQ - t0))

        bn = (b + 1) % B

        def ln_next():
            for t0 in range(0, HB, LR):
                nrows = min(LR, HB - t0)
                for j, v in enumerate(ln_rows(bn, r0, t0, nrows)):
                    xn_buf[j, t0 // 2:(t0 + nrows) // 2, :] = v
                pin(x_buf if t0 + LR < HB else xs, xn_buf[0, pl.ds(z8, 8), :])

        def kv(j, c):
            return _unpack(xs[j, c * BK // 2:(c + 1) * BK // 2, :])

        m = [None, None]
        for c in range(NC):
            if c == LC:
                ln_next()
            M = [None] * 7
            for j in SORDER:
                lhs = qs[j] if QSSA else _unpack(q_buf[j, pl.ds(z8, HB // 2), :])
                M[j] = _dot_nt(lhs, kv((0, 1, 3, 4, 2, 5, 6)[j], c))
            quads = (M[0] - M[4] + M[3] + M[6], M[4] + M[2], M[1] + M[3], M[0] - M[1] + M[2] + M[5])
            for q, s in enumerate(quads):
                if (c + 1) * BK > T // 2:
                    col = lax.broadcasted_iota(jnp.int32, (HB, BK), 1)
                    s = jnp.where(col < T // 2 - c * BK, s, -jnp.inf)
                c0 = (q % 2) * SW + (c // 2) * BK
                s_par[c % 2][(q // 2) * HB:(q // 2 + 1) * HB, c0:c0 + BK] = s
                for l in range(BK // LANES):
                    t = s[:, l * LANES:(l + 1) * LANES]
                    m[q // 2] = t if m[q // 2] is None else jnp.maximum(m[q // 2], t)
        for h in range(2):
            mx = jnp.max(m[h], axis=-1, keepdims=True)
            m[h] = mx + jnp.log2(jnp.sum(jnp.exp2(m[h] - mx), axis=-1, keepdims=True))

        def merge(quads, w, after=None):
            left = _combos(*quads)
            out = [None] * 7
            for step, k in enumerate(MORDER):
                l, r = PAIRS[k]
                out[k] = _dot(left[l].astype(BF16), _unpack(w[r]))
                if after:
                    after(step + 1, out[k])
            return _combine(out)

        def merge_conv():
            zq = [jnp.concatenate([cb[Z + (q % 2) * (NL // 2) + l, pl.ds(z8 + (q // 2) * HB, HB), :]
                                   for l in range(NL // 2)], axis=1) for q in range(4)]
            for q, v in enumerate(merge(zq, wdc)):
                rows, cols = (q // 2) * HB, slice((q % 2) * HD, (q % 2 + 1) * HD)
                y_buf[q, 0:HB, :] = v + x_buf[b, pl.ds(r0 + rows, HB), cols].astype(F32)

        def probs(c):
            p, part = [], [None, None]
            for q in range(4):
                c0 = (q % 2) * SW + (c // 2) * BK
                e = jnp.exp2(s_par[c % 2][pl.ds(z8 + (q // 2) * HB, HB), c0:c0 + BK] - m[q // 2])
                for l in range(BK // LANES):
                    t = e[:, l * LANES:(l + 1) * LANES]
                    part[q // 2] = t if part[q // 2] is None else part[q // 2] + t
                p.append(e)
            return [v.astype(BF16) for v in _combos(*p)], jnp.concatenate(part, axis=1)

        def accumulate(c, k, d):
            if c > 0:
                d = d + a_par[(c - 1) % 2][k, pl.ds(z8, HB), :]
            if c + 1 < NC:
                a_par[c % 2][k, 0:HB, :] = d
            return d

        nxt = probs(0)
        for c in range(NC):
            if c == MC:
                merge_conv()
            if c + NC == LC:
                ln_next()
            p, part = nxt
            acc = [None] * 7
            for kk, k in enumerate(ORDER):
                l, r = PAIRS[k]
                d = _dot(p[l], kv(r, c))
                if kk == PK and c + 1 < NC:
                    pin(s_par[(c + 1) % 2], d)
                    nxt = probs(c + 1)
                acc[k] = accumulate(c, k, d)
            lsum = accumulate(c, 7, part)
        lsum = [lsum[:, :LANES], lsum[:, LANES:]]
        o11, o12, o21, o22 = _combine(acc)
        inv = [1.0 / jnp.sum(v, axis=-1, keepdims=True) for v in lsum]
        def publish(step, v):
            js = XC[step] if step < len(XC) else ()
            if js:
                pin(xn_buf, v)
            for j in js:
                xs_all[bn, j, pl.ds(h0, HB // 2), :] = xn_buf[j, pl.ds(z8, HB // 2), :]

        publish(0, acc[ORDER[6]])
        for q, v in enumerate(merge((o11 * inv[0], o12 * inv[0], o21 * inv[1], o22 * inv[1]), wva, publish)):
            rows, cols = (q // 2) * HB, slice((q % 2) * HD, (q % 2 + 1) * HD)
            o_buf[slot, rows:rows + HB, cols] = (v + y_buf[q, pl.ds(z8, HB), :]).astype(o_buf.dtype)
        o_copy(n, slot).start()
        return carry

    lax.fori_loop(0, NB, body, 0)
    o_copy(NB - 2, (NB - 2) % 2).wait()
    o_copy(NB - 1, (NB - 1) % 2).wait()


def make(BQ=800, BK=256, CR=24, LR=32, SP=0, AP=0, SKIP=(), QSSA=1, LC=12, GU=1, SORDER=(1, 4, 0, 3, 2, 5, 6), PK=0, MC=0, XC=((0,), (1,), (2, 3), (4,), (5,), (6,)), GP=0, GB=2, MORDER=(4, 2, 1, 0, 3, 5, 6), ORDER=(4, 1, 0, 2, 3, 5, 6), flags=None):
    def fn(x, w_q, w_k, w_v, w_ao, w_up, dw, w_dn, w_merge):
        B, T, D = x.shape
        KW = dw.shape[0]
        TP = -(-(T // 2) // BK) * BK
        NL = D // LANES
        NQ = T // BQ
        HB, HD = BQ // 2, D // 2
        kern = functools.partial(_kernel, B=B, T=T, D=D, KW=KW, BQ=BQ, BK=BK, TP=TP, CR=CR, LR=LR, ORDER=ORDER, MORDER=MORDER, PK=PK, MC=MC, XC=XC, GP=GP, GB=GB, SKIP=SKIP, QSSA=QSSA, LC=LC, GU=GU, SORDER=SORDER)
        any_spec = pl.BlockSpec(memory_space=pl.ANY)
        V = pltpu.VMEM
        E = PAD
        scratch = [
            V((B, T + E, D), BF16), V((B * (NQ - 1) * HALO, D), BF16),
            V((B, 7, TP // 2 + E, HD), U32),
            V((11, D, D), BF16), V((KW, D), BF16), V((3, NL, D, LANES), F32), V((5, 7, HD // 2, HD), U32),
            V((B * NQ, HALO, D), F32),
            V((4 * NL, BQ + 2 * HALO + E, LANES), F32), V((7, HB // 2 + E, HD), U32),
            V((BQ + E, TP + SP), F32), V((BQ + E, TP + SP), F32),
            V((8, HB + E + AP, HD), F32), V((8, HB + E + AP, HD), F32),
            V((4, HB + E, HD), F32), V((7, HB // 2 + E, HD), U32),
            V((2, BQ, D), BF16),
            pltpu.SemaphoreType.DMA((B * NQ,)), pltpu.SemaphoreType.DMA(()),
            pltpu.SemaphoreType.DMA((10,)), pltpu.SemaphoreType.DMA((2,)),
        ]
        return pl.pallas_call(
            kern,
            out_shape=jax.ShapeDtypeStruct((B, T, D), x.dtype),
            in_specs=[any_spec] * 9,
            out_specs=any_spec,
            scratch_shapes=scratch,
            compiler_params=pltpu.CompilerParams(vmem_limit_bytes=110 * 1024 * 1024, flags=flags),
        )(x, w_q, w_k, w_v, w_ao, w_up, dw, w_dn, w_merge)
    return fn


_branchformer = make()


@jax.jit
def pallas_standalone__conformer_family_branchformer__speech_kernel(
    x: jax.Array,
    w_q: jax.Array,
    w_k: jax.Array,
    w_v: jax.Array,
    w_ao: jax.Array,
    w_up: jax.Array,
    dw: jax.Array,
    w_dn: jax.Array,
    w_merge: jax.Array,
):
    return _branchformer(x, w_q, w_k, w_v, w_ao, w_up, dw, w_dn, w_merge)
```

```python
import functools
import math
import jax
import jax.numpy as jnp
from jax import lax
from jax.experimental import pallas as pl
from jax.experimental.pallas import tpu as pltpu

F32 = jnp.float32
BF16 = jnp.bfloat16
U32 = jnp.uint32
EPS = 1e-5
LANES = 128
HALO = 16
PAD = 16


def _ln(x, eps=EPS):
    d = x.shape[-1]
    m = jnp.sum(x, axis=-1, keepdims=True) * (1.0 / d)
    c = x - m
    v = jnp.sum(c * c, axis=-1, keepdims=True) * (1.0 / d)
    return c * lax.rsqrt(v + eps)


def _gelu2(x):
    c1 = math.sqrt(2.0 / math.pi)
    c2 = c1 * 0.044715
    return x + x * jnp.tanh(x * (c1 + c2 * (x * x)))


def _gate(h2):
    return _ln(h2, 4.0 * EPS)


def _dot(a, b):
    return jnp.dot(a, b, preferred_element_type=F32)


def _dot_nt(a, b):
    return lax.dot_general(a, b, (((1,), (1,)), ((), ())), preferred_element_type=F32)


def _pack(v):
    return pltpu.bitcast(v.astype(BF16), U32)


def _unpack(w):
    return pltpu.bitcast(w, BF16)


def _pack_rows(pair):
    return pltpu.bitcast(pltpu.pack_elementwise(pair, packed_dtype=BF16), U32)


def _unpack_rows(w, parity):
    return pltpu.unpack_elementwise(w, index=parity, packed_dtype=BF16, unpacked_dtype=F32)


def _combos(a11, a12, a21, a22):
    return [a11 + a22, a11, a22, a21 - a22, a12 - a11, a11 + a21, a12 + a22]


PAIRS = ((0, 0), (1, 6), (3, 1), (4, 2), (2, 5), (5, 4), (6, 3))


def _combine(n):
    return (n[0] - n[4] + n[3] + n[6], n[1] + n[3], n[4] + n[2], n[0] - n[1] + n[2] + n[5])


def _pin(dst, v, zero):
    lead = (0,) * (len(dst.shape) - 2)
    rows = 8 * (4 // jnp.dtype(dst.dtype).itemsize)
    v = pltpu.bitcast(v[v.shape[0] - 8:, :LANES], dst.dtype)
    dst[lead + (pl.ds(dst.shape[-2] - rows + zero, rows), slice(0, LANES))] = v


def _kernel(x_hbm, wq_hbm, wk_hbm, wv_hbm, wao_hbm, wup_hbm, dw_hbm, wdn_hbm, wm_hbm,
            o_hbm,
            x_buf, xh_buf, xs_all, wst, dw_in, wf32, wc, g_first, cb, xn_buf,
            s_e, s_o, a_e, a_o, y_buf, q_buf, o_buf,
            x_sem, h_sem, w_sem, o_sem, *, B, T, D, KW, BQ, BK, TP, CR, LR, ORDER, MORDER, PK, MC, XC, AO, ST, AT, ZT, YT, GP, GB, SKIP, QSSA, LC, GU, SORDER):
    NQ = T // BQ
    NB = B * NQ
    NL = D // LANES
    NC = TP // BK
    HB = BQ // 2
    HD = D // 2
    G, U, W, Z = (NL * j for j in range(4))

    def x_copy(n):
        b, i = n // NQ, n % NQ
        r = pl.ds(pl.multiple_of(i * BQ, BQ), BQ)
        return pltpu.make_async_copy(x_hbm.at[b, r, :], x_buf.at[b, r, :], x_sem.at[n])

    def o_copy(n, slot):
        b, i = n // NQ, n % NQ
        r = pl.ds(pl.multiple_of(i * BQ, BQ), BQ)
        return pltpu.make_async_copy(o_buf.at[slot], o_hbm.at[b, r, :], o_sem.at[slot])

    heads = [(b, i) for b in range(B) for i in range(1, NQ)]
    h_copies = [pltpu.make_async_copy(x_hbm.at[b, i * BQ:i * BQ + HALO, :],
                                      xh_buf.at[j * HALO:(j + 1) * HALO, :], h_sem)
                for j, (b, i) in enumerate(heads)]
    WQ, WK, WV, WAO, WMA, WDN, WMC, WU, WG, W1, XH = range(11)
    w_src = [wq_hbm, wk_hbm, wv_hbm, wao_hbm, wm_hbm.at[0:D], wdn_hbm, wm_hbm.at[D:2 * D],
             wup_hbm.at[:, 0:D], wup_hbm.at[:, D:2 * D]]
    w_copies = [pltpu.make_async_copy(src, wst.at[j], w_sem.at[j]) for j, src in enumerate(w_src)]
    dw_copy = pltpu.make_async_copy(dw_hbm, dw_in, w_sem.at[len(w_src)])
    QK, VA, DC, UU, GG = range(5)
    RB = HALO * len(heads)
    NRB = D // RB

    def ln_rows(b, r0, t0, nrows):
        words = [pltpu.bitcast(x_buf[b, pl.ds(r0 + h * HB + t0, nrows), :], U32) for h in range(2)]
        ops = []
        for parity in range(2):
            top, bot = (_ln(_unpack_rows(w, parity)) for w in words)
            ops.append(_combos(top[:, :HD], top[:, HD:], bot[:, :HD], bot[:, HD:]))
        return [_pack_rows(pair) for pair in zip(*ops)]

    for c in (w_copies[WQ], w_copies[WK], dw_copy, w_copies[WV], w_copies[WAO]):
        c.start()
    for b in range(B):
        xs_all[b, :, T // 4:TP // 2, :] = jnp.zeros((7, TP // 2 - T // 4, HD), U32)
    cb[G:G + NL, BQ:BQ + HALO, :] = jnp.zeros((NL, HALO, LANES), F32)
    for b in range(B):
        g_first[b * NQ + NQ - 1] = jnp.zeros((HALO, D), F32)
    w_copies[WQ].wait()
    w_copies[WK].wait()
    x_copy(0).start()
    x_copy(1).start()

    def put_folded(j, r, v):
        for l in range(NL):
            wf32[j, l, r, :] = v[:, l * LANES:(l + 1) * LANES]

    def fold_qk(t, c):
        r = pl.ds(pl.multiple_of(t * RB, RB), RB)
        put_folded(QK, r, _dot_nt(wst[WQ, r, :], wst[WK]) * (math.log2(math.e) / math.sqrt(D)))
        return c
    lax.fori_loop(0, NRB, fold_qk, 0)

    def put_operands(j, t0, parts):
        ops = [_combos(top[:, :HD], top[:, HD:], bot[:, :HD], bot[:, HD:]) for top, bot in parts]
        for k, pair in enumerate(zip(*ops)):
            wc[j, k, pl.ds(pl.multiple_of(t0 // 2, HD // 4), HD // 4), :] = _pack_rows(pair)

    def split_folded(t, c):
        j, t0 = t // 2, (t % 2) * (HD // 2)
        put_operands(j, t0, [[jnp.concatenate(
            [wf32[j, l, pl.ds(h * HD + t0 + parity, HD // 4, stride=2), :] for l in range(NL)], axis=1)
            for h in range(2)] for parity in range(2)])
        return c
    lax.fori_loop(0, 2, split_folded, 0)

    dw_copy.wait()
    for l in range(NL):
        cb[Z + l, 0:KW, :] = 0.5 * dw_in[:, l * LANES:(l + 1) * LANES].astype(F32)

    def taps(k, c):
        for l in range(NL):
            cb[W + l, pl.ds(pl.multiple_of(8 * k, 8), 8), :] = jnp.broadcast_to(
                cb[Z + l, pl.ds(k, 1), :], (8, LANES))
        return c
    lax.fori_loop(0, KW, taps, 0)

    PB = HB // HALO

    def ln_first(u0, count, last):
        for u in (jnp.minimum(u0 + k, last) for k in range(count)):
            r0 = pl.multiple_of((u // PB) * BQ + (u % PB) * HALO, HALO)
            for k, v in enumerate(ln_rows(0, r0, 0, HALO)):
                xs_all[0, k, pl.ds(pl.multiple_of(u * (HALO // 2), HALO // 2), HALO // 2), :] = v

    NF = 3 * NRB + 1
    PF = -(-(NQ - 1) * PB // NF)
    assert NQ == 5 and (PB // PF, 2 * PB // PF, 3 * PB // PF) == (3, 6, 9) and NRB == 4
    arrivals = {
        0: ([w_copies[WV], w_copies[WAO], x_copy(0)], [w_copies[WMA], x_copy(2)]),
        3: ([x_copy(1)], [w_copies[WDN], w_copies[WMC]]),
        4: ([w_copies[WMA]], [x_copy(3)]),
        6: ([x_copy(2)], [w_copies[WG]] + h_copies),
        8: ([w_copies[WDN], w_copies[WMC]], [w_copies[WU], x_copy(4)]),
        9: ([x_copy(3)], []),
    }

    def fold(t, c):
        for step, (done, new) in arrivals.items():
            @pl.when(t == step)
            def _():
                for cp in done:
                    cp.wait()
                for cp in new:
                    cp.start()

        @pl.when(t == NF - 1)
        def _():
            for cp in [w_copies[WG]] + h_copies:
                cp.wait()
            wst[XH, 0:RB, :] = _ln(xh_buf[...].astype(F32)).astype(BF16)

        j = t // NRB
        left = jnp.where(j == 0, WV, jnp.where(j == 1, W1, jnp.where(j == 2, WDN, XH)))
        right = jnp.where(j == 0, WAO, jnp.where(j == 1, WMA, jnp.where(j == 2, WMC, WG)))
        r = pl.ds(pl.multiple_of((t % NRB) * RB, RB), RB)
        v = _dot(wst[left, r, :], wst[right])
        put_folded(jnp.where(j == 1, VA, jnp.where(j == 2, DC, QK)), r, v)
        wst[jnp.where(j == 0, W1, WQ), r, :] = v.astype(BF16)
        ln_first(PF * t, PF, (NQ - 1) * PB - 1)
        return c
    lax.fori_loop(0, NF, fold, 0)

    gf = _gate(_gelu2(jnp.concatenate([wf32[QK, l, 0:RB, :] for l in range(NL)], axis=1)))
    for j, (b, i) in enumerate(heads):
        g_first[b * NQ + i - 1] = gf[j * HALO:(j + 1) * HALO]
    lax.fori_loop(2, 6, split_folded, 0)
    w_copies[WU].wait()

    def split_plain(t, c):
        j, t0 = t // 2, (t % 2) * (HD // 2)
        words = [pltpu.bitcast(wst[WU + j, pl.ds(pl.multiple_of(h * HD + t0, HD // 2), HD // 2), :], U32)
                 for h in range(2)]
        put_operands(UU + j, t0, [[_unpack_rows(w, parity) for w in words] for parity in range(2)])
        return c
    lax.fori_loop(0, 4, split_plain, 0)

    x_copy(NQ - 1).wait()
    x_copy(NQ).start()

    def ln_last(t, c):
        ln_first((NQ - 1) * PB + 5 * t, 5, NQ * PB - 1)
        return c
    lax.fori_loop(0, PB // 5, ln_last, 0)
    wqk, wva, wdc, wu, wg = (wc.at[j] for j in (QK, VA, DC, UU, GG))

    s_par = (s_e, s_o)
    a_par = (a_e, a_o)
    SW = TP // 2

    def body(n, carry):
        b, i = n // NQ, n % NQ
        xs = xs_all.at[b]
        slot = n % 2
        r0 = pl.multiple_of(i * BQ, BQ)
        h0 = pl.multiple_of(i * (HB // 2), HB // 2)

        @pl.when(n + NQ < NB)
        def _():
            x_copy(n + NQ).wait()

        @pl.when(n + NQ + 1 < NB)
        def _():
            x_copy(n + NQ + 1).start()

        @pl.when(n >= 2)
        def _():
            o_copy(n - 2, slot).wait()

        first = i == 0
        z8 = pl.multiple_of((n // NB) * 16, 16)
        zf = pl.multiple_of((n // (NB + 1)) * 16, 16)

        pin = functools.partial(_pin, zero=zf)

        def project(w, order=ORDER):
            out = [None] * 7
            for k in order:
                l, r = PAIRS[k]
                out[k] = _dot(_unpack(xs[l, pl.ds(h0, HB // 2), :]), _unpack(w[r]))
            return _combine(out)

        def put_quads(base, row0, quads):
            for q, v in enumerate(quads):
                for l in range(NL // 2):
                    cb[base + (q % 2) * (NL // 2) + l, row0 + (q // 2) * HB:row0 + (q // 2 + 1) * HB, :] = (
                        v[:, l * LANES:(l + 1) * LANES])

        for l in range(NL):
            ls = slice(l * LANES, (l + 1) * LANES)
            cb[G + l, 0:HALO, :] = jnp.where(first, 0.0, cb[G + l, BQ:BQ + HALO, :])
            cb[G + l, BQ + HALO:BQ + 2 * HALO, :] = g_first[n, :, ls]

        put_quads(U, 0, [v if GU else _gelu2(v) for v in project(wu)])
        g11, g12, g21, g22 = (_gelu2(v) for v in project(wg, (3, 1, 4, 0, 6, 2, 5)))

        def put_gate(t0, h):
            g = _gate(h)
            for l in range(NL):
                cb[G + l, HALO + t0:HALO + t0 + h.shape[0], :] = g[:, l * LANES:(l + 1) * LANES]
            return g

        g = put_gate(0, jnp.concatenate([g11, g12], axis=1))
        g2 = jnp.concatenate([g21, g22], axis=1)
        if GP == 0:
            g = put_gate(HB, g2)
        pin(cb, g)
        a11, a12, a21, a22 = project(wqk)
        qs = [a11 + a22, a21 + a22, a11, a22, a11 + a12, a21 - a11, a12 - a22]
        if QSSA:
            qs = [v.astype(BF16) for v in qs]
        else:
            for j, v in enumerate(qs):
                q_buf[j, 0:HB // 2, :] = _pack(v)

        def conv_rows(l, t0, nr):
            acc = [None] * nr
            off = HALO - KW // 2
            for s in range(8):
                taps = [(a, 8 * a + s - off) for a in range((KW + off + 7) // 8)
                        if 0 <= 8 * a + s - off < KW]
                w = {a: cb[W + l, 8 * k:8 * k + 8, :] for a, k in taps}
                for j in range(nr + max(a for a, _ in taps)):
                    use = [a for a, _ in taps if 0 <= j - a < nr]
                    if not use:
                        continue
                    gv = cb[G + l, t0 + 8 * j + s:t0 + 8 * j + s + 8, :]
                    for a in use:
                        t = gv * w[a]
                        acc[j - a] = t if acc[j - a] is None else acc[j - a] + t
            return acc * 1

        def conv_piece(l, t0, nrows):
            cv = jnp.concatenate(conv_rows(l, t0, nrows // 8), axis=0)
            cb[Z + l, pl.ds(zf + t0, nrows), :] = cv * (_gelu2 if GU else (lambda v: v))(cb[U + l, t0:t0 + nrows, :])

        for t0 in range(0, BQ, CR):
            k = t0 // CR - GB
            if GP and 0 <= k < HB // GP:
                put_gate(HB + k * GP, g2[k * GP:(k + 1) * GP])
            for l in range(NL if 'conv' not in SKIP else 0):
                conv_piece(l, t0, min(CR, BQ - t0))

        bn = (b + 1) % B

        def ln_next():
            for t0 in range(0, HB, LR):
                nrows = min(LR, HB - t0)
                for j, v in enumerate(ln_rows(bn, r0, t0, nrows)):
                    xn_buf[j, t0 // 2:(t0 + nrows) // 2, :] = v
                pin(x_buf if t0 + LR < HB else xs, xn_buf[0, pl.ds(z8, 8), :])

        def kv(j, c):
            return _unpack(xs[j, c * BK // 2:(c + 1) * BK // 2, :])

        m = [None, None]
        for c in range(NC):
            if c == LC:
                ln_next()
            M = [None] * 7
            for j in SORDER:
                lhs = qs[j] if QSSA else _unpack(q_buf[j, pl.ds(z8, HB // 2), :])
                M[j] = _dot_nt(lhs, kv((0, 1, 3, 4, 2, 5, 6)[j], c))
            quads = (M[0] - M[4] + M[3] + M[6], M[4] + M[2], M[1] + M[3], M[0] - M[1] + M[2] + M[5])
            for q, s in enumerate(quads):
                if (c + 1) * BK > T // 2:
                    col = lax.broadcasted_iota(jnp.int32, (HB, BK), 1)
                    s = jnp.where(col < T // 2 - c * BK, s, -jnp.inf)
                c0 = (q % 2) * SW + (c // 2) * BK
                s_par[c % 2][(q // 2) * HB:(q // 2 + 1) * HB, c0:c0 + BK] = s
                for l in range(BK // LANES):
                    t = s[:, l * LANES:(l + 1) * LANES]
                    m[q // 2] = t if m[q // 2] is None else jnp.maximum(m[q // 2], t)
        for h in range(2):
            mx = jnp.max(m[h], axis=-1, keepdims=True)
            m[h] = mx + jnp.log2(jnp.sum(jnp.exp2(m[h] - mx), axis=-1, keepdims=True))

        def merge(quads, w, after=None):
            left = _combos(*quads)
            out = [None] * 7
            for step, k in enumerate(MORDER):
                l, r = PAIRS[k]
                out[k] = _dot(left[l].astype(BF16), _unpack(w[r]))
                if after:
                    after(step + 1, out[k])
            return _combine(out)

        def merge_conv():
            zq = [jnp.concatenate([cb[Z + (q % 2) * (NL // 2) + l, pl.ds((0 if ZT else z8) + (q // 2) * HB, HB), :]
                                   for l in range(NL // 2)], axis=1) for q in range(4)]
            for q, v in enumerate(merge(zq, wdc)):
                rows, cols = (q // 2) * HB, slice((q % 2) * HD, (q % 2 + 1) * HD)
                y_buf[q, 0:HB, :] = v + x_buf[b, pl.ds(r0 + rows, HB), cols].astype(F32)

        def probs(c):
            p, part = [], [None, None]
            for q in range(4):
                c0 = (q % 2) * SW + (c // 2) * BK
                e = jnp.exp2(s_par[c % 2][pl.ds((0 if ST == 1 or (ST == 2 and c > 0) else z8) + (q // 2) * HB, HB), c0:c0 + BK] - m[q // 2])
                for l in range(BK // LANES):
                    t = e[:, l * LANES:(l + 1) * LANES]
                    part[q // 2] = t if part[q // 2] is None else part[q // 2] + t
                p.append(e)
            return [v.astype(BF16) for v in _combos(*p)], jnp.concatenate(part, axis=1)

        def accumulate(c, k, d):
            if c > 0:
                d = d + a_par[(c - 1) % 2][k, pl.ds((0 if AT else z8) + AO * ((c - 1) % 2), HB), :]
            if c + 1 < NC:
                a_par[c % 2][k, AO * (c % 2):AO * (c % 2) + HB, :] = d
            return d

        if ST == 1:
            pin(s_par[0], M[SORDER[0]])
        nxt = probs(0)
        for c in range(NC):
            if c == MC:
                merge_conv()
            if c + NC == LC:
                ln_next()
            p, part = nxt
            acc = [None] * 7
            for kk, k in enumerate(ORDER):
                l, r = PAIRS[k]
                d = _dot(p[l], kv(r, c))
                if kk == PK and c + 1 < NC:
                    pin(s_par[(c + 1) % 2], d)
                    nxt = probs(c + 1)
                acc[k] = accumulate(c, k, d)
            lsum = accumulate(c, 7, part)
            if AT and c + 1 < NC:
                pin(a_par[c % 2], lsum if AT == 1 else acc[ORDER[0]])
        lsum = [lsum[:, :LANES], lsum[:, LANES:]]
        o11, o12, o21, o22 = _combine(acc)
        inv = [1.0 / jnp.sum(v, axis=-1, keepdims=True) for v in lsum]
        def publish(step, v):
            js = XC[step] if step < len(XC) else ()
            if js:
                pin(xn_buf, v)
            for j in js:
                xs_all[bn, j, pl.ds(h0, HB // 2), :] = xn_buf[j, pl.ds(0 if YT else z8, HB // 2), :]

        if YT:
            pin(y_buf, acc[ORDER[0]])
        publish(0, acc[ORDER[6]])
        for q, v in enumerate(merge((o11 * inv[0], o12 * inv[0], o21 * inv[1], o22 * inv[1]), wva, publish)):
            rows, cols = (q // 2) * HB, slice((q % 2) * HD, (q % 2 + 1) * HD)
            o_buf[slot, rows:rows + HB, cols] = (v + y_buf[q, pl.ds(0 if YT else z8, HB), :]).astype(o_buf.dtype)
        o_copy(n, slot).start()
        return carry

    lax.fori_loop(0, NB, body, 0)
    o_copy(NB - 2, (NB - 2) % 2).wait()
    o_copy(NB - 1, (NB - 1) % 2).wait()


def make(BQ=800, BK=256, CR=24, LR=32, SP=0, AP=64, AO=0, ST=2, AT=1, ZT=1, YT=1, SKIP=(), QSSA=1, LC=12, GU=1, SORDER=(1, 4, 0, 3, 2, 5, 6), PK=0, MC=0, XC=((0,), (1,), (2, 3), (4,), (5,), (6,)), GP=0, GB=2, MORDER=(4, 2, 1, 0, 3, 5, 6), ORDER=(4, 1, 0, 2, 3, 5, 6), flags=None):
    def fn(x, w_q, w_k, w_v, w_ao, w_up, dw, w_dn, w_merge):
        B, T, D = x.shape
        KW = dw.shape[0]
        TP = -(-(T // 2) // BK) * BK
        NL = D // LANES
        NQ = T // BQ
        HB, HD = BQ // 2, D // 2
        kern = functools.partial(_kernel, B=B, T=T, D=D, KW=KW, BQ=BQ, BK=BK, TP=TP, CR=CR, LR=LR, ORDER=ORDER, MORDER=MORDER, PK=PK, MC=MC, XC=XC, AO=AO, ST=ST, AT=AT, ZT=ZT, YT=YT, GP=GP, GB=GB, SKIP=SKIP, QSSA=QSSA, LC=LC, GU=GU, SORDER=SORDER)
        any_spec = pl.BlockSpec(memory_space=pl.ANY)
        V = pltpu.VMEM
        E = PAD
        scratch = [
            V((B, T + E, D), BF16), V((B * (NQ - 1) * HALO, D), BF16),
            V((B, 7, TP // 2 + E, HD), U32),
            V((11, D, D), BF16), V((KW, D), BF16), V((3, NL, D + 8, LANES), F32), V((5, 7, HD // 2, HD), U32),
            V((B * NQ, HALO, D), F32),
            V((4 * NL, BQ + 2 * HALO + E, LANES), F32), V((7, HB // 2 + E, HD), U32),
            V((BQ + E, TP + SP), F32), V((BQ + E, TP + SP), F32),
            V((8, HB + E + AP, HD), F32), V((8, HB + E + AP, HD), F32),
            V((4, HB + E, HD), F32), V((7, HB // 2 + E, HD), U32),
            V((2, BQ, D), BF16),
            pltpu.SemaphoreType.DMA((B * NQ,)), pltpu.SemaphoreType.DMA(()),
            pltpu.SemaphoreType.DMA((10,)), pltpu.SemaphoreType.DMA((2,)),
        ]
        return pl.pallas_call(
            kern,
            out_shape=jax.ShapeDtypeStruct((B, T, D), x.dtype),
            in_specs=[any_spec] * 9,
            out_specs=any_spec,
            scratch_shapes=scratch,
            compiler_params=pltpu.CompilerParams(vmem_limit_bytes=110 * 1024 * 1024, flags=flags),
        )(x, w_q, w_k, w_v, w_ao, w_up, dw, w_dn, w_merge)
    return fn


_branchformer = make()


@jax.jit
def pallas_standalone__conformer_family_branchformer__speech_kernel(
    x: jax.Array,
    w_q: jax.Array,
    w_k: jax.Array,
    w_v: jax.Array,
    w_ao: jax.Array,
    w_up: jax.Array,
    dw: jax.Array,
    w_dn: jax.Array,
    w_merge: jax.Array,
):
    return _branchformer(x, w_q, w_k, w_v, w_ao, w_up, dw, w_dn, w_merge)
```

```python
import functools
import math

import jax
import jax.numpy as jnp
from jax import lax
from jax.experimental import pallas as pl
from jax.experimental.pallas import tpu as pltpu

F32 = jnp.float32
BF16 = jnp.bfloat16
U32 = jnp.uint32
EPS = 1e-5
LANES = 128
HALO = 16
SPARE = 16

BQ = 800
BK = 256
CONV_ROWS = 24
LN_ROWS = 32
LN_CHUNK = 4

PAIRS = ((0, 0), (1, 6), (3, 1), (4, 2), (2, 5), (5, 4), (6, 3))
KEY_OPERAND = (0, 1, 3, 4, 2, 5, 6)
ORDER = (4, 1, 0, 2, 3, 5, 6)
GATE_ORDER = (3, 1, 4, 0, 6, 2, 5)
SCORE_ORDER = (0, 1, 4, 3, 2, 5, 6)
MERGE_ORDER = (4, 2, 1, 0, 3, 5, 6)
PUBLISH = ((0,), (1,), (2, 3), (4,), (5,), (6,))


def _ln(x, eps=EPS):
    d = x.shape[-1]
    m = jnp.sum(x, axis=-1, keepdims=True) * (1.0 / d)
    c = x - m
    v = jnp.sum(c * c, axis=-1, keepdims=True) * (1.0 / d)
    return c * lax.rsqrt(v + eps)


def _gelu2(x):
    c1 = math.sqrt(2.0 / math.pi)
    c2 = c1 * 0.044715
    return x + x * jnp.tanh(x * (c1 + c2 * (x * x)))


def _gate(h2):
    return _ln(h2, 4.0 * EPS)


def _dot(a, b):
    return jnp.dot(a, b, preferred_element_type=F32)


def _dot_nt(a, b):
    return lax.dot_general(a, b, (((1,), (1,)), ((), ())), preferred_element_type=F32)


def _as_bf16(words):
    return pltpu.bitcast(words, BF16)


def _pack_rows(pair):
    return pltpu.bitcast(pltpu.pack_elementwise(pair, packed_dtype=BF16), U32)


def _unpack_rows(words, parity):
    return pltpu.unpack_elementwise(words, index=parity, packed_dtype=BF16, unpacked_dtype=F32)


def _combos(a11, a12, a21, a22):
    return [a11 + a22, a11, a22, a21 - a22, a12 - a11, a11 + a21, a12 + a22]


def _combine(n):
    return (n[0] - n[4] + n[3] + n[6], n[1] + n[3], n[4] + n[2], n[0] - n[1] + n[2] + n[5])


def _operands(parts):
    h = parts[0][0].shape[1] // 2
    ops = [_combos(top[:, :h], top[:, h:], bot[:, :h], bot[:, h:]) for top, bot in parts]
    return [_pack_rows(pair) for pair in zip(*ops)]


def _pin(dst, v, zero):
    lead = (0,) * (len(dst.shape) - 2)
    rows = 8 * (4 // jnp.dtype(dst.dtype).itemsize)
    v = pltpu.bitcast(v[v.shape[0] - 8:, :LANES], dst.dtype)
    dst[lead + (pl.ds(dst.shape[-2] - rows + zero, rows), slice(0, LANES))] = v


def _kernel(x_hbm, wq_hbm, wk_hbm, wv_hbm, wao_hbm, wup_hbm, dw_hbm, wdn_hbm, wm_hbm,
            o_hbm,
            x_buf, xh_buf, xs_all, wst, dw_in, wf32, wc, g_next, cb, xn_buf,
            s_even, s_odd, a_even, a_odd, y_buf, o_buf,
            x_sem, h_sem, w_sem, o_sem):
    B, T, D = x_hbm.shape
    KW = dw_hbm.shape[0]
    TP = s_even.shape[1]
    NQ = T // BQ
    NB = B * NQ
    NL = D // LANES
    NC = TP // BK
    HB = BQ // 2
    HD = D // 2
    G, U, W, Z = (NL * j for j in range(4))

    def x_copy(n):
        b, i = n // NQ, n % NQ
        r = pl.ds(pl.multiple_of(i * BQ, BQ), BQ)
        return pltpu.make_async_copy(x_hbm.at[b, r, :], x_buf.at[b, r, :], x_sem.at[n])

    def o_copy(n, slot):
        b, i = n // NQ, n % NQ
        r = pl.ds(pl.multiple_of(i * BQ, BQ), BQ)
        return pltpu.make_async_copy(o_buf.at[slot], o_hbm.at[b, r, :], o_sem.at[slot])

    heads = [(b, i) for b in range(B) for i in range(1, NQ)]
    h_copies = [pltpu.make_async_copy(x_hbm.at[b, i * BQ:i * BQ + HALO, :],
                                      xh_buf.at[j * HALO:(j + 1) * HALO, :], h_sem)
                for j, (b, i) in enumerate(heads)]
    WQ, WK, WV, WAO, WMA, WDN, WMC, WU, WG, W1, XH = range(11)
    w_src = [wq_hbm, wk_hbm, wv_hbm, wao_hbm, wm_hbm.at[0:D], wdn_hbm, wm_hbm.at[D:2 * D],
             wup_hbm.at[:, 0:D], wup_hbm.at[:, D:2 * D]]
    w_copies = [pltpu.make_async_copy(src, wst.at[j], w_sem.at[j]) for j, src in enumerate(w_src)]
    dw_copy = pltpu.make_async_copy(dw_hbm, dw_in, w_sem.at[len(w_src)])
    QK, VA, DC, UU, GG = range(5)
    RB = HALO * len(heads)
    NRB = D // RB

    def ln_rows(b, r0, t0, nrows):
        words = [pltpu.bitcast(x_buf[b, pl.ds(r0 + h * HB + t0, nrows), :], U32) for h in range(2)]
        return _operands([[_ln(_unpack_rows(w, parity)) for w in words] for parity in range(2)])

    for c in (w_copies[WQ], w_copies[WK], dw_copy, w_copies[WV], w_copies[WAO]):
        c.start()
    for b in range(B):
        xs_all[b, :, T // 4:TP // 2, :] = jnp.zeros((7, TP // 2 - T // 4, HD), U32)
    cb[G:G + NL, BQ:BQ + HALO, :] = jnp.zeros((NL, HALO, LANES), F32)
    for b in range(B):
        g_next[b * NQ + NQ - 1] = jnp.zeros((HALO, D), F32)
    w_copies[WQ].wait()
    w_copies[WK].wait()
    x_copy(0).start()
    x_copy(1).start()

    def put_folded(j, r, v):
        for l in range(NL):
            wf32[j, l, r, :] = v[:, l * LANES:(l + 1) * LANES]

    def fold_qk(t, c):
        r = pl.ds(pl.multiple_of(t * RB, RB), RB)
        put_folded(QK, r, _dot_nt(wst[WQ, r, :], wst[WK]) * (math.log2(math.e) / math.sqrt(D)))
        return c
    lax.fori_loop(0, NRB, fold_qk, 0)

    def put_operands(j, t0, parts):
        for k, v in enumerate(_operands(parts)):
            wc[j, k, pl.ds(pl.multiple_of(t0 // 2, HD // 4), HD // 4), :] = v

    def split_folded(t, c):
        j, t0 = t // 2, (t % 2) * (HD // 2)
        put_operands(j, t0, [[jnp.concatenate(
            [wf32[j, l, pl.ds(h * HD + t0 + parity, HD // 4, stride=2), :] for l in range(NL)], axis=1)
            for h in range(2)] for parity in range(2)])
        return c
    lax.fori_loop(0, 2, split_folded, 0)

    dw_copy.wait()
    for l in range(NL):
        cb[Z + l, 0:KW, :] = 0.5 * dw_in[:, l * LANES:(l + 1) * LANES].astype(F32)

    def spread_taps(k, c):
        for l in range(NL):
            cb[W + l, pl.ds(pl.multiple_of(8 * k, 8), 8), :] = jnp.broadcast_to(
                cb[Z + l, pl.ds(k, 1), :], (8, LANES))
        return c
    lax.fori_loop(0, KW, spread_taps, 0)

    PB = HB // HALO

    def ln_first(u0, count, last):
        for u in (jnp.minimum(u0 + k, last) for k in range(count)):
            r0 = pl.multiple_of((u // PB) * BQ + (u % PB) * HALO, HALO)
            for k, v in enumerate(ln_rows(0, r0, 0, HALO)):
                xs_all[0, k, pl.ds(pl.multiple_of(u * (HALO // 2), HALO // 2), HALO // 2), :] = v

    NF = 3 * NRB + 1
    PF = -(-(NQ - 1) * PB // NF)
    assert NQ == 5 and NRB == 4 and (PB // PF, 2 * PB // PF, 3 * PB // PF) == (3, 6, 9)
    arrivals = {
        0: ([w_copies[WV], w_copies[WAO], x_copy(0)], [w_copies[WMA], x_copy(2)]),
        3: ([x_copy(1)], [w_copies[WDN], w_copies[WMC]]),
        4: ([w_copies[WMA]], [x_copy(3)]),
        6: ([x_copy(2)], [w_copies[WG]] + h_copies),
        8: ([w_copies[WDN], w_copies[WMC]], [w_copies[WU], x_copy(4)]),
        9: ([x_copy(3)], []),
    }

    def fold(t, c):
        for step, (done, new) in arrivals.items():
            @pl.when(t == step)
            def _():
                for cp in done:
                    cp.wait()
                for cp in new:
                    cp.start()

        @pl.when(t == NF - 1)
        def _():
            for cp in [w_copies[WG]] + h_copies:
                cp.wait()
            wst[XH, 0:RB, :] = _ln(xh_buf[...].astype(F32)).astype(BF16)

        j = t // NRB
        left = jnp.where(j == 0, WV, jnp.where(j == 1, W1, jnp.where(j == 2, WDN, XH)))
        right = jnp.where(j == 0, WAO, jnp.where(j == 1, WMA, jnp.where(j == 2, WMC, WG)))
        r = pl.ds(pl.multiple_of((t % NRB) * RB, RB), RB)
        v = _dot(wst[left, r, :], wst[right])
        put_folded(jnp.where(j == 1, VA, jnp.where(j == 2, DC, QK)), r, v)
        wst[jnp.where(j == 0, W1, WQ), r, :] = v.astype(BF16)
        ln_first(PF * t, PF, (NQ - 1) * PB - 1)
        return c
    lax.fori_loop(0, NF, fold, 0)

    gate_heads = _gate(_gelu2(jnp.concatenate([wf32[QK, l, 0:RB, :] for l in range(NL)], axis=1)))
    for j, (b, i) in enumerate(heads):
        g_next[b * NQ + i - 1] = gate_heads[j * HALO:(j + 1) * HALO]
    lax.fori_loop(2, 6, split_folded, 0)
    w_copies[WU].wait()

    def split_plain(t, c):
        j, t0 = t // 2, (t % 2) * (HD // 2)
        words = [pltpu.bitcast(wst[WU + j, pl.ds(pl.multiple_of(h * HD + t0, HD // 2), HD // 2), :], U32)
                 for h in range(2)]
        put_operands(UU + j, t0, [[_unpack_rows(w, parity) for w in words] for parity in range(2)])
        return c
    lax.fori_loop(0, 4, split_plain, 0)

    x_copy(NQ - 1).wait()
    x_copy(NQ).start()

    def ln_last(t, c):
        ln_first((NQ - 1) * PB + 5 * t, 5, NQ * PB - 1)
        return c
    lax.fori_loop(0, PB // 5, ln_last, 0)

    wqk, wva, wdc, wu, wg = (wc.at[j] for j in (QK, VA, DC, UU, GG))
    s_par = (s_even, s_odd)
    a_par = (a_even, a_odd)
    SW = TP // 2

    def block(q):
        return (q // 2) * HB, slice((q % 2) * HD, (q % 2 + 1) * HD)

    def body(n, carry):
        b, i = n // NQ, n % NQ
        b_next = (b + 1) % B
        xs = xs_all.at[b]
        slot = n % 2
        r0 = pl.multiple_of(i * BQ, BQ)
        h0 = pl.multiple_of(i * (HB // 2), HB // 2)

        @pl.when(n + NQ < NB)
        def _():
            x_copy(n + NQ).wait()

        @pl.when(n + NQ + 1 < NB)
        def _():
            x_copy(n + NQ + 1).start()

        @pl.when(n >= 2)
        def _():
            o_copy(n - 2, slot).wait()

        zero_ld = pl.multiple_of((n // NB) * 16, 16)
        zero_st = pl.multiple_of((n // (NB + 1)) * 16, 16)
        pin = functools.partial(_pin, zero=zero_st)

        def project(w, order):
            out = [None] * 7
            for k in order:
                l, r = PAIRS[k]
                out[k] = _dot(_as_bf16(xs[l, pl.ds(h0, HB // 2), :]), _as_bf16(w[r]))
            return _combine(out)

        for l in range(NL):
            cb[G + l, 0:HALO, :] = jnp.where(i == 0, 0.0, cb[G + l, BQ:BQ + HALO, :])
            cb[G + l, BQ + HALO:BQ + 2 * HALO, :] = g_next[n, :, l * LANES:(l + 1) * LANES]

        for q, v in enumerate(project(wu, ORDER)):
            for l in range(NL // 2):
                cb[U + (q % 2) * (NL // 2) + l, (q // 2) * HB:(q // 2 + 1) * HB, :] = (
                    v[:, l * LANES:(l + 1) * LANES])
        gate = [_gelu2(v) for v in project(wg, GATE_ORDER)]
        for h in range(2):
            g = _gate(jnp.concatenate(gate[2 * h:2 * h + 2], axis=1))
            for l in range(NL):
                cb[G + l, HALO + h * HB:HALO + (h + 1) * HB, :] = g[:, l * LANES:(l + 1) * LANES]
        pin(cb, g)
        q11, q12, q21, q22 = project(wqk, ORDER)
        queries = [v.astype(BF16) for v in
                   (q11 + q22, q21 + q22, q11, q22, q11 + q12, q21 - q11, q12 - q22)]

        def conv_step(l, t0, nrows):
            acc = [None] * (nrows // 8)
            off = HALO - KW // 2
            for s in range(8):
                taps = [(a, 8 * a + s - off) for a in range((KW + off + 7) // 8)
                        if 0 <= 8 * a + s - off < KW]
                w = {a: cb[W + l, 8 * k:8 * k + 8, :] for a, k in taps}
                for j in range(len(acc) + max(a for a, _ in taps)):
                    use = [a for a, _ in taps if 0 <= j - a < len(acc)]
                    if not use:
                        continue
                    gv = cb[G + l, t0 + 8 * j + s:t0 + 8 * j + s + 8, :]
                    for a in use:
                        t = gv * w[a]
                        acc[j - a] = t if acc[j - a] is None else acc[j - a] + t
            cb[Z + l, pl.ds(zero_st + t0, nrows), :] = (
                jnp.concatenate(acc, axis=0) * _gelu2(cb[U + l, t0:t0 + nrows, :]))

        for t0 in range(0, BQ, CONV_ROWS):
            for l in range(NL):
                conv_step(l, t0, min(CONV_ROWS, BQ - t0))

        def keys(j, c):
            return _as_bf16(xs[j, c * BK // 2:(c + 1) * BK // 2, :])

        m = [None, None]
        for c in range(NC):
            prod = [None] * 7
            for k in SCORE_ORDER:
                prod[k] = _dot_nt(queries[k], keys(KEY_OPERAND[k], c))
            s11, s21, s12, s22 = _combine(prod)
            for q, s in enumerate((s11, s12, s21, s22)):
                if (c + 1) * BK > T // 2:
                    col = lax.broadcasted_iota(jnp.int32, (HB, BK), 1)
                    s = jnp.where(col < T // 2 - c * BK, s, -jnp.inf)
                c0 = (q % 2) * SW + (c // 2) * BK
                s_par[c % 2][(q // 2) * HB:(q // 2 + 1) * HB, c0:c0 + BK] = s
                for l in range(BK // LANES):
                    t = s[:, l * LANES:(l + 1) * LANES]
                    m[q // 2] = t if m[q // 2] is None else jnp.maximum(m[q // 2], t)
        for h in range(2):
            row_max = jnp.max(m[h], axis=-1, keepdims=True)
            m[h] = row_max + jnp.log2(jnp.sum(jnp.exp2(m[h] - row_max), axis=-1, keepdims=True))

        def weights(c):
            p, part = [], [None, None]
            for q in range(4):
                c0 = (q % 2) * SW + (c // 2) * BK
                rows = pl.ds((zero_ld if c == 0 else 0) + (q // 2) * HB, HB)
                e = jnp.exp2(s_par[c % 2][rows, c0:c0 + BK] - m[q // 2])
                for l in range(BK // LANES):
                    t = e[:, l * LANES:(l + 1) * LANES]
                    part[q // 2] = t if part[q // 2] is None else part[q // 2] + t
                p.append(e)
            return [v.astype(BF16) for v in _combos(*p)], jnp.concatenate(part, axis=1)

        def accumulate(c, k, d):
            if c > 0:
                d = d + a_par[(c - 1) % 2][k, 0:HB, :]
            if c + 1 < NC:
                a_par[c % 2][k, 0:HB, :] = d
            return d

        def merge(quads, w, after=None):
            left = _combos(*quads)
            out = [None] * 7
            for step, k in enumerate(MERGE_ORDER):
                l, r = PAIRS[k]
                out[k] = _dot(left[l].astype(BF16), _as_bf16(w[r]))
                if after:
                    after(step + 1, out[k])
            return _combine(out)

        def ln_next():
            for t0 in range(0, HB, LN_ROWS):
                nrows = min(LN_ROWS, HB - t0)
                for j, v in enumerate(ln_rows(b_next, r0, t0, nrows)):
                    xn_buf[j, t0 // 2:(t0 + nrows) // 2, :] = v
                pin(x_buf if t0 + LN_ROWS < HB else xs, xn_buf[0, pl.ds(zero_ld, 8), :])

        def publish(step, v):
            if step < len(PUBLISH):
                pin(xn_buf, v)
                for j in PUBLISH[step]:
                    xs_all[b_next, j, pl.ds(h0, HB // 2), :] = xn_buf[j, 0:HB // 2, :]

        nxt = weights(0)

        z = [jnp.concatenate([cb[Z + (q % 2) * (NL // 2) + l, (q // 2) * HB:(q // 2 + 1) * HB, :]
                              for l in range(NL // 2)], axis=1) for q in range(4)]
        for q, v in enumerate(merge(z, wdc)):
            rows, cols = block(q)
            y_buf[q, 0:HB, :] = v + x_buf[b, pl.ds(r0 + rows, HB), cols].astype(F32)

        for c in range(NC):
            p, part = nxt
            acc = [None] * 7
            for step, k in enumerate(ORDER):
                l, r = PAIRS[k]
                if c == LN_CHUNK and step == 0:
                    ln_next()
                d = _dot(p[l], keys(r, c))
                if step == 1 and c + 1 < NC:
                    pin(s_par[(c + 1) % 2], d)
                    nxt = weights(c + 1)
                acc[k] = accumulate(c, k, d)
            total = accumulate(c, 7, part)
            if c + 1 < NC:
                pin(a_par[c % 2], total)
        o11, o12, o21, o22 = _combine(acc)
        inv = [1.0 / jnp.sum(v, axis=-1, keepdims=True) for v in (total[:, :LANES], total[:, LANES:])]

        pin(y_buf, acc[ORDER[0]])
        publish(0, acc[ORDER[6]])
        for q, v in enumerate(merge((o11 * inv[0], o12 * inv[0], o21 * inv[1], o22 * inv[1]), wva, publish)):
            rows, cols = block(q)
            o_buf[slot, rows:rows + HB, cols] = (v + y_buf[q, 0:HB, :]).astype(o_buf.dtype)
        o_copy(n, slot).start()
        return carry

    lax.fori_loop(0, NB, body, 0)
    o_copy(NB - 2, (NB - 2) % 2).wait()
    o_copy(NB - 1, (NB - 1) % 2).wait()


@jax.jit
def pallas_standalone__conformer_family_branchformer__speech_kernel(
    x: jax.Array,
    w_q: jax.Array,
    w_k: jax.Array,
    w_v: jax.Array,
    w_ao: jax.Array,
    w_up: jax.Array,
    dw: jax.Array,
    w_dn: jax.Array,
    w_merge: jax.Array,
):
    B, T, D = x.shape
    KW = dw.shape[0]
    TP = -(-(T // 2) // BK) * BK
    NL, NQ, HB, HD = D // LANES, T // BQ, BQ // 2, D // 2
    assert T % BQ == 0 and BK == HD == 2 * LANES and KW // 2 < HALO
    vmem, dma = pltpu.VMEM, pltpu.SemaphoreType.DMA
    scratch = [
        vmem((B, T + SPARE, D), BF16),
        vmem((B * (NQ - 1) * HALO, D), BF16),
        vmem((B, 7, TP // 2 + SPARE, HD), U32),
        vmem((11, D, D), BF16),
        vmem((KW, D), BF16),
        vmem((3, NL, D + 8, LANES), F32),
        vmem((5, 7, HD // 2, HD), U32),
        vmem((B * NQ, HALO, D), F32),
        vmem((4 * NL, BQ + 2 * HALO + SPARE, LANES), F32),
        vmem((7, HB // 2 + SPARE, HD), U32),
        vmem((BQ + SPARE, TP), F32),
        vmem((BQ + SPARE, TP), F32),
        vmem((8, HB + SPARE, HD), F32),
        vmem((8, HB + SPARE, HD), F32),
        vmem((4, HB + SPARE, HD), F32),
        vmem((2, BQ, D), x.dtype),
        dma((B * NQ,)), dma(()), dma((10,)), dma((2,)),
    ]
    in_hbm = pl.BlockSpec(memory_space=pl.ANY)
    return pl.pallas_call(
        _kernel,
        out_shape=jax.ShapeDtypeStruct((B, T, D), x.dtype),
        in_specs=[in_hbm] * 9,
        out_specs=in_hbm,
        scratch_shapes=scratch,
        compiler_params=pltpu.CompilerParams(vmem_limit_bytes=110 * 1024 * 1024),
    )(x, w_q, w_k, w_v, w_ao, w_up, dw, w_dn, w_merge)
```

```python
import functools
import math

import jax
import jax.numpy as jnp
from jax import lax
from jax.experimental import pallas as pl
from jax.experimental.pallas import tpu as pltpu

F32 = jnp.float32
BF16 = jnp.bfloat16
U32 = jnp.uint32
EPS = 1e-5
LANES = 128
HALO = 16
SPARE = 16

BQ = 800
BK = 256
CONV_ROWS = 24
LN_ROWS = 32
LN_CHUNK = 4

PAIRS = ((0, 0), (1, 6), (3, 1), (4, 2), (2, 5), (5, 4), (6, 3))
KEY_OPERAND = (0, 1, 3, 4, 2, 5, 6)
ORDER = (4, 1, 0, 2, 3, 5, 6)
GATE_ORDER = (3, 1, 4, 0, 6, 2, 5)
SCORE_ORDER = (0, 1, 4, 3, 2, 5, 6)
MERGE_ORDER = (4, 2, 1, 0, 3, 5, 6)
PUBLISH = ((0,), (1,), (2, 3), (4,), (5,), (6,))


def _ln(x, eps=EPS):
    d = x.shape[-1]
    m = jnp.sum(x, axis=-1, keepdims=True) * (1.0 / d)
    c = x - m
    v = jnp.sum(c * c, axis=-1, keepdims=True) * (1.0 / d)
    return c * lax.rsqrt(v + eps)


def _gelu2(x):
    c1 = math.sqrt(2.0 / math.pi)
    c2 = c1 * 0.044715
    return x + x * jnp.tanh(x * (c1 + c2 * (x * x)))


def _gate(h2):
    return _ln(h2, 4.0 * EPS)


def _dot(a, b):
    return jnp.dot(a, b, preferred_element_type=F32)


def _dot_nt(a, b):
    return lax.dot_general(a, b, (((1,), (1,)), ((), ())), preferred_element_type=F32)


def _as_bf16(words):
    return pltpu.bitcast(words, BF16)


def _pack_rows(pair):
    return pltpu.bitcast(pltpu.pack_elementwise(pair, packed_dtype=BF16), U32)


def _unpack_rows(words, parity):
    return pltpu.unpack_elementwise(words, index=parity, packed_dtype=BF16, unpacked_dtype=F32)


def _combos(a11, a12, a21, a22):
    return [a11 + a22, a11, a22, a21 - a22, a12 - a11, a11 + a21, a12 + a22]


def _combine(n):
    return (n[0] - n[4] + n[3] + n[6], n[1] + n[3], n[4] + n[2], n[0] - n[1] + n[2] + n[5])


def _operands(parts):
    h = parts[0][0].shape[1] // 2
    ops = [_combos(top[:, :h], top[:, h:], bot[:, :h], bot[:, h:]) for top, bot in parts]
    return [_pack_rows(pair) for pair in zip(*ops)]


def _pin(dst, v, zero):
    lead = (0,) * (len(dst.shape) - 2)
    rows = 8 * (4 // jnp.dtype(dst.dtype).itemsize)
    v = pltpu.bitcast(v[v.shape[0] - 8:, :LANES], dst.dtype)
    dst[lead + (pl.ds(dst.shape[-2] - rows + zero, rows), slice(0, LANES))] = v


def _kernel(x_hbm, wq_hbm, wk_hbm, wv_hbm, wao_hbm, wup_hbm, dw_hbm, wdn_hbm, wm_hbm,
            o_hbm,
            x_buf, xh_buf, xs_all, wst, dw_in, wf32, wc, g_next, cb, xn_buf,
            s_even, s_odd, a_even, a_odd, y_buf, o_buf,
            x_sem, h_sem, w_sem, o_sem):
    B, D = xs_all.shape[0], x_hbm.shape[1]
    T = x_hbm.shape[0] // B
    KW = dw_hbm.shape[0]
    TP = s_even.shape[1]
    NQ = T // BQ
    NB = B * NQ
    NL = D // LANES
    NC = TP // BK
    HB = BQ // 2
    HD = D // 2
    G, U, W, Z = (NL * j for j in range(4))

    def x_copy(n):
        r = pl.ds(pl.multiple_of(n * BQ, BQ), BQ)
        return pltpu.make_async_copy(x_hbm.at[r, :], x_buf.at[r, :], x_sem.at[n])

    def o_copy(n, slot):
        r = pl.ds(pl.multiple_of(n * BQ, BQ), BQ)
        return pltpu.make_async_copy(o_buf.at[slot], o_hbm.at[r, :], o_sem.at[slot])

    heads = [(b, i) for b in range(B) for i in range(1, NQ)]
    h_copies = [pltpu.make_async_copy(x_hbm.at[b * T + i * BQ:b * T + i * BQ + HALO, :],
                                      xh_buf.at[j * HALO:(j + 1) * HALO, :], h_sem)
                for j, (b, i) in enumerate(heads)]
    WQ, WK, WV, WAO, WMA, WDN, WMC, WU, WG, W1, XH = range(11)
    w_src = [wq_hbm, wk_hbm, wv_hbm, wao_hbm, wm_hbm.at[0:D], wdn_hbm, wm_hbm.at[D:2 * D],
             wup_hbm.at[:, 0:D], wup_hbm.at[:, D:2 * D]]
    w_copies = [pltpu.make_async_copy(src, wst.at[j], w_sem.at[j]) for j, src in enumerate(w_src)]
    dw_copy = pltpu.make_async_copy(dw_hbm, dw_in, w_sem.at[len(w_src)])
    QK, VA, DC, UU, GG = range(5)
    RB = HALO * len(heads)
    NRB = D // RB

    def ln_rows(r0, t0, nrows):
        words = [pltpu.bitcast(x_buf[pl.ds(r0 + h * HB + t0, nrows), :], U32) for h in range(2)]
        return _operands([[_ln(_unpack_rows(w, parity)) for w in words] for parity in range(2)])

    for c in (w_copies[WQ], w_copies[WK], dw_copy, w_copies[WV], w_copies[WAO]):
        c.start()
    for b in range(B):
        xs_all[b, :, T // 4:TP // 2, :] = jnp.zeros((7, TP // 2 - T // 4, HD), U32)
    cb[G:G + NL, BQ:BQ + HALO, :] = jnp.zeros((NL, HALO, LANES), F32)
    for b in range(B):
        g_next[b * NQ + NQ - 1] = jnp.zeros((HALO, D), F32)
    w_copies[WQ].wait()
    w_copies[WK].wait()
    x_copy(0).start()
    x_copy(1).start()

    def put_folded(j, r, v):
        for l in range(NL):
            wf32[j, l, r, :] = v[:, l * LANES:(l + 1) * LANES]

    def fold_qk(t, c):
        r = pl.ds(pl.multiple_of(t * RB, RB), RB)
        put_folded(QK, r, _dot_nt(wst[WQ, r, :], wst[WK]) * (math.log2(math.e) / math.sqrt(D)))
        return c
    lax.fori_loop(0, NRB, fold_qk, 0)

    def put_operands(j, t0, parts):
        for k, v in enumerate(_operands(parts)):
            wc[j, k, pl.ds(pl.multiple_of(t0 // 2, HD // 4), HD // 4), :] = v

    def split_folded(t, c):
        j, t0 = t // 2, (t % 2) * (HD // 2)
        put_operands(j, t0, [[jnp.concatenate(
            [wf32[j, l, pl.ds(h * HD + t0 + parity, HD // 4, stride=2), :] for l in range(NL)], axis=1)
            for h in range(2)] for parity in range(2)])
        return c
    lax.fori_loop(0, 2, split_folded, 0)

    dw_copy.wait()
    for l in range(NL):
        cb[Z + l, 0:KW, :] = 0.5 * dw_in[:, l * LANES:(l + 1) * LANES].astype(F32)

    def spread_taps(k, c):
        for l in range(NL):
            cb[W + l, pl.ds(pl.multiple_of(8 * k, 8), 8), :] = jnp.broadcast_to(
                cb[Z + l, pl.ds(k, 1), :], (8, LANES))
        return c
    lax.fori_loop(0, KW, spread_taps, 0)

    PB = HB // HALO

    def ln_first(u0, count, last):
        for u in (jnp.minimum(u0 + k, last) for k in range(count)):
            r0 = pl.multiple_of((u // PB) * BQ + (u % PB) * HALO, HALO)
            for k, v in enumerate(ln_rows(r0, 0, HALO)):
                xs_all[0, k, pl.ds(pl.multiple_of(u * (HALO // 2), HALO // 2), HALO // 2), :] = v

    NF = 3 * NRB + 1
    PF = -(-(NQ - 1) * PB // NF)
    assert NQ == 5 and NRB == 4 and (PB // PF, 2 * PB // PF, 3 * PB // PF) == (3, 6, 9)
    arrivals = {
        0: ([w_copies[WV], w_copies[WAO], x_copy(0)], [w_copies[WMA], x_copy(2)]),
        3: ([x_copy(1)], [w_copies[WDN], w_copies[WMC]]),
        4: ([w_copies[WMA]], [x_copy(3)]),
        6: ([x_copy(2)], [w_copies[WG]] + h_copies),
        8: ([w_copies[WDN], w_copies[WMC]], [w_copies[WU], x_copy(4)]),
        9: ([x_copy(3)], []),
    }

    def fold(t, c):
        for step, (done, new) in arrivals.items():
            @pl.when(t == step)
            def _():
                for cp in done:
                    cp.wait()
                for cp in new:
                    cp.start()

        @pl.when(t == NF - 1)
        def _():
            for cp in [w_copies[WG]] + h_copies:
                cp.wait()
            wst[XH, 0:RB, :] = _ln(xh_buf[...].astype(F32)).astype(BF16)

        j = t // NRB
        left = jnp.where(j == 0, WV, jnp.where(j == 1, W1, jnp.where(j == 2, WDN, XH)))
        right = jnp.where(j == 0, WAO, jnp.where(j == 1, WMA, jnp.where(j == 2, WMC, WG)))
        r = pl.ds(pl.multiple_of((t % NRB) * RB, RB), RB)
        v = _dot(wst[left, r, :], wst[right])
        put_folded(jnp.where(j == 1, VA, jnp.where(j == 2, DC, QK)), r, v)
        wst[jnp.where(j == 0, W1, WQ), r, :] = v.astype(BF16)
        ln_first(PF * t, PF, (NQ - 1) * PB - 1)
        return c
    lax.fori_loop(0, NF, fold, 0)

    gate_heads = _gate(_gelu2(jnp.concatenate([wf32[QK, l, 0:RB, :] for l in range(NL)], axis=1)))
    for j, (b, i) in enumerate(heads):
        g_next[b * NQ + i - 1] = gate_heads[j * HALO:(j + 1) * HALO]
    lax.fori_loop(2, 6, split_folded, 0)
    w_copies[WU].wait()

    def split_plain(t, c):
        j, t0 = t // 2, (t % 2) * (HD // 2)
        words = [pltpu.bitcast(wst[WU + j, pl.ds(pl.multiple_of(h * HD + t0, HD // 2), HD // 2), :], U32)
                 for h in range(2)]
        put_operands(UU + j, t0, [[_unpack_rows(w, parity) for w in words] for parity in range(2)])
        return c
    lax.fori_loop(0, 4, split_plain, 0)

    x_copy(NQ - 1).wait()
    x_copy(NQ).start()

    def ln_last(t, c):
        ln_first((NQ - 1) * PB + 5 * t, 5, NQ * PB - 1)
        return c
    lax.fori_loop(0, PB // 5, ln_last, 0)

    wqk, wva, wdc, wu, wg = (wc.at[j] for j in (QK, VA, DC, UU, GG))
    s_par = (s_even, s_odd)
    a_par = (a_even, a_odd)
    SW = TP // 2

    def block(q):
        return (q // 2) * HB, slice((q % 2) * HD, (q % 2 + 1) * HD)

    def body(n, carry):
        b, i = carry
        b_next = jnp.where(b + 1 < B, b + 1, 0)
        xs = xs_all.at[b]
        slot = n & 1
        r0 = pl.multiple_of(n * BQ, BQ)
        r_next = pl.multiple_of((b_next * NQ + i) * BQ, BQ)
        h0 = pl.multiple_of(i * (HB // 2), HB // 2)

        @pl.when(n + NQ < NB)
        def _():
            x_copy(n + NQ).wait()

        @pl.when(n + NQ + 1 < NB)
        def _():
            x_copy(n + NQ + 1).start()

        @pl.when(n >= 2)
        def _():
            o_copy(n - 2, slot).wait()

        zero_ld = pl.multiple_of((n // NB) * 16, 16)
        zero_st = pl.multiple_of((n // (NB + 1)) * 16, 16)
        pin = functools.partial(_pin, zero=zero_st)

        def project(w, order):
            out = [None] * 7
            for k in order:
                l, r = PAIRS[k]
                out[k] = _dot(_as_bf16(xs[l, pl.ds(h0, HB // 2), :]), _as_bf16(w[r]))
            return _combine(out)

        for l in range(NL):
            cb[G + l, 0:HALO, :] = jnp.where(i == 0, 0.0, cb[G + l, BQ:BQ + HALO, :])
            cb[G + l, BQ + HALO:BQ + 2 * HALO, :] = g_next[n, :, l * LANES:(l + 1) * LANES]

        for q, v in enumerate(project(wu, ORDER)):
            for l in range(NL // 2):
                cb[U + (q % 2) * (NL // 2) + l, (q // 2) * HB:(q // 2 + 1) * HB, :] = (
                    v[:, l * LANES:(l + 1) * LANES])
        gate = [_gelu2(v) for v in project(wg, GATE_ORDER)]
        for h in range(2):
            g = _gate(jnp.concatenate(gate[2 * h:2 * h + 2], axis=1))
            for l in range(NL):
                cb[G + l, HALO + h * HB:HALO + (h + 1) * HB, :] = g[:, l * LANES:(l + 1) * LANES]
        pin(cb, g)
        q11, q12, q21, q22 = project(wqk, ORDER)
        queries = [v.astype(BF16) for v in
                   (q11 + q22, q21 + q22, q11, q22, q11 + q12, q21 - q11, q12 - q22)]

        def conv_step(l, t0, nrows):
            acc = [None] * (nrows // 8)
            off = HALO - KW // 2
            for s in range(8):
                taps = [(a, 8 * a + s - off) for a in range((KW + off + 7) // 8)
                        if 0 <= 8 * a + s - off < KW]
                w = {a: cb[W + l, 8 * k:8 * k + 8, :] for a, k in taps}
                for j in range(len(acc) + max(a for a, _ in taps)):
                    use = [a for a, _ in taps if 0 <= j - a < len(acc)]
                    if not use:
                        continue
                    gv = cb[G + l, t0 + 8 * j + s:t0 + 8 * j + s + 8, :]
                    for a in use:
                        t = gv * w[a]
                        acc[j - a] = t if acc[j - a] is None else acc[j - a] + t
            cb[Z + l, pl.ds(zero_st + t0, nrows), :] = (
                jnp.concatenate(acc, axis=0) * _gelu2(cb[U + l, t0:t0 + nrows, :]))

        for t0 in range(0, BQ, CONV_ROWS):
            for l in range(NL):
                conv_step(l, t0, min(CONV_ROWS, BQ - t0))

        def keys(j, c):
            return _as_bf16(xs[j, c * BK // 2:(c + 1) * BK // 2, :])

        m = [None, None]
        for c in range(NC):
            prod = [None] * 7
            for k in SCORE_ORDER:
                prod[k] = _dot_nt(queries[k], keys(KEY_OPERAND[k], c))
            s11, s21, s12, s22 = _combine(prod)
            for q, s in enumerate((s11, s12, s21, s22)):
                if (c + 1) * BK > T // 2:
                    col = lax.broadcasted_iota(jnp.int32, (HB, BK), 1)
                    s = jnp.where(col < T // 2 - c * BK, s, -jnp.inf)
                c0 = (q % 2) * SW + (c // 2) * BK
                s_par[c % 2][(q // 2) * HB:(q // 2 + 1) * HB, c0:c0 + BK] = s
                for l in range(BK // LANES):
                    t = s[:, l * LANES:(l + 1) * LANES]
                    m[q // 2] = t if m[q // 2] is None else jnp.maximum(m[q // 2], t)
        for h in range(2):
            row_max = jnp.max(m[h], axis=-1, keepdims=True)
            m[h] = row_max + jnp.log2(jnp.sum(jnp.exp2(m[h] - row_max), axis=-1, keepdims=True))

        def weights(c):
            p, part = [], [None, None]
            for q in range(4):
                c0 = (q % 2) * SW + (c // 2) * BK
                rows = pl.ds((zero_ld if c == 0 else 0) + (q // 2) * HB, HB)
                e = jnp.exp2(s_par[c % 2][rows, c0:c0 + BK] - m[q // 2])
                for l in range(BK // LANES):
                    t = e[:, l * LANES:(l + 1) * LANES]
                    part[q // 2] = t if part[q // 2] is None else part[q // 2] + t
                p.append(e)
            return [v.astype(BF16) for v in _combos(*p)], jnp.concatenate(part, axis=1)

        def accumulate(c, k, d):
            if c > 0:
                d = d + a_par[(c - 1) % 2][k, 0:HB, :]
            if c + 1 < NC:
                a_par[c % 2][k, 0:HB, :] = d
            return d

        def merge(quads, w, after=None):
            left = _combos(*quads)
            out = [None] * 7
            for step, k in enumerate(MERGE_ORDER):
                l, r = PAIRS[k]
                out[k] = _dot(left[l].astype(BF16), _as_bf16(w[r]))
                if after:
                    after(step + 1, out[k])
            return _combine(out)

        def ln_next():
            for t0 in range(0, HB, LN_ROWS):
                nrows = min(LN_ROWS, HB - t0)
                for j, v in enumerate(ln_rows(r_next, t0, nrows)):
                    xn_buf[j, t0 // 2:(t0 + nrows) // 2, :] = v
                pin(x_buf if t0 + LN_ROWS < HB else xs, xn_buf[0, pl.ds(zero_ld, 8), :])

        def publish(step, v):
            if step < len(PUBLISH):
                pin(xn_buf, v)
                for j in PUBLISH[step]:
                    xs_all[b_next, j, pl.ds(h0, HB // 2), :] = xn_buf[j, 0:HB // 2, :]

        nxt = weights(0)

        z = [jnp.concatenate([cb[Z + (q % 2) * (NL // 2) + l, (q // 2) * HB:(q // 2 + 1) * HB, :]
                              for l in range(NL // 2)], axis=1) for q in range(4)]
        for q, v in enumerate(merge(z, wdc)):
            rows, cols = block(q)
            y_buf[q, 0:HB, :] = v + x_buf[pl.ds(r0 + rows, HB), cols].astype(F32)

        for c in range(NC):
            p, part = nxt
            acc = [None] * 7
            for step, k in enumerate(ORDER):
                l, r = PAIRS[k]
                if c == LN_CHUNK and step == 0:
                    ln_next()
                d = _dot(p[l], keys(r, c))
                if step == 1 and c + 1 < NC:
                    pin(s_par[(c + 1) % 2], d)
                    nxt = weights(c + 1)
                acc[k] = accumulate(c, k, d)
            total = accumulate(c, 7, part)
            if c + 1 < NC:
                pin(a_par[c % 2], total)
        o11, o12, o21, o22 = _combine(acc)
        inv = [1.0 / jnp.sum(v, axis=-1, keepdims=True) for v in (total[:, :LANES], total[:, LANES:])]

        pin(y_buf, acc[ORDER[0]])
        publish(0, acc[ORDER[6]])
        for q, v in enumerate(merge((o11 * inv[0], o12 * inv[0], o21 * inv[1], o22 * inv[1]), wva, publish)):
            rows, cols = block(q)
            o_buf[slot, rows:rows + HB, cols] = (v + y_buf[q, 0:HB, :]).astype(o_buf.dtype)
        o_copy(n, slot).start()
        last = i + 1 == NQ
        return jnp.where(last, b + 1, b), jnp.where(last, 0, i + 1)

    lax.fori_loop(0, NB, body, (jnp.int32(0), jnp.int32(0)))
    o_copy(NB - 2, (NB - 2) % 2).wait()
    o_copy(NB - 1, (NB - 1) % 2).wait()


@jax.jit
def pallas_standalone__conformer_family_branchformer__speech_kernel(
    x: jax.Array,
    w_q: jax.Array,
    w_k: jax.Array,
    w_v: jax.Array,
    w_ao: jax.Array,
    w_up: jax.Array,
    dw: jax.Array,
    w_dn: jax.Array,
    w_merge: jax.Array,
):
    B, T, D = x.shape
    KW = dw.shape[0]
    TP = -(-(T // 2) // BK) * BK
    NL, NQ, HB, HD = D // LANES, T // BQ, BQ // 2, D // 2
    assert T % BQ == 0 and BK == HD == 2 * LANES and KW // 2 < HALO
    vmem, dma = pltpu.VMEM, pltpu.SemaphoreType.DMA
    scratch = [
        vmem((B * T + SPARE, D), BF16),
        vmem((B * (NQ - 1) * HALO, D), BF16),
        vmem((B, 7, TP // 2 + SPARE, HD), U32),
        vmem((11, D, D), BF16),
        vmem((KW, D), BF16),
        vmem((3, NL, D + 8, LANES), F32),
        vmem((5, 7, HD // 2, HD), U32),
        vmem((B * NQ, HALO, D), F32),
        vmem((4 * NL, BQ + 2 * HALO + SPARE, LANES), F32),
        vmem((7, HB // 2 + SPARE, HD), U32),
        vmem((BQ + SPARE, TP), F32),
        vmem((BQ + SPARE, TP), F32),
        vmem((8, HB + SPARE, HD), F32),
        vmem((8, HB + SPARE, HD), F32),
        vmem((4, HB + SPARE, HD), F32),
        vmem((2, BQ, D), x.dtype),
        dma((B * NQ,)), dma(()), dma((10,)), dma((2,)),
    ]
    in_hbm = pl.BlockSpec(memory_space=pl.ANY)
    return pl.pallas_call(
        _kernel,
        out_shape=jax.ShapeDtypeStruct((B * T, D), x.dtype),
        in_specs=[in_hbm] * 9,
        out_specs=in_hbm,
        scratch_shapes=scratch,
        compiler_params=pltpu.CompilerParams(vmem_limit_bytes=110 * 1024 * 1024),
    )(x.reshape(B * T, D), w_q, w_k, w_v, w_ao, w_up, dw, w_dn, w_merge).reshape(B, T, D)
```

```python
import functools
import math

import jax
import jax.numpy as jnp
from jax import lax
from jax.experimental import pallas as pl
from jax.experimental.pallas import tpu as pltpu

F32 = jnp.float32
BF16 = jnp.bfloat16
U32 = jnp.uint32
EPS = 1e-5
LANES = 128
HALO = 16
SPARE = 16

BQ = 800
BK = 256
CONV_ROWS = 24
LN_ROWS = 32
PIN_STEP = 1
LN_CHUNK = 4

PAIRS = ((0, 0), (1, 6), (3, 1), (4, 2), (2, 5), (5, 4), (6, 3))
KEY_OPERAND = (0, 1, 3, 4, 2, 5, 6)
ORDER = (4, 1, 0, 2, 3, 5, 6)
SCORE_ORDER = (0, 1, 4, 3, 2, 5, 6)
MERGE_ORDER = (4, 2, 1, 0, 3, 5, 6)
PUBLISH = ((0, 7), (1,), (2, 3), (4,), (5, 8), (6,))


def _ln(x, eps=EPS):
    d = x.shape[-1]
    m = jnp.sum(x, axis=-1, keepdims=True) * (1.0 / d)
    c = x - m
    v = jnp.sum(c * c, axis=-1, keepdims=True) * (1.0 / d)
    return c * lax.rsqrt(v + eps)


def _gelu2(x):
    c1 = math.sqrt(2.0 / math.pi)
    c2 = c1 * 0.044715
    return x + x * jnp.tanh(x * (c1 + c2 * (x * x)))


def _gate(h2):
    return _ln(h2, 4.0 * EPS)


def _dot(a, b):
    return jnp.dot(a, b, preferred_element_type=F32)


def _dot_nt(a, b):
    return lax.dot_general(a, b, (((1,), (1,)), ((), ())), preferred_element_type=F32)


def _as_bf16(words):
    return pltpu.bitcast(words, BF16)


def _pack_rows(pair):
    return pltpu.bitcast(pltpu.pack_elementwise(pair, packed_dtype=BF16), U32)


def _unpack_rows(words, parity):
    return pltpu.unpack_elementwise(words, index=parity, packed_dtype=BF16, unpacked_dtype=F32)


def _combos(a11, a12, a21, a22):
    return [a11 + a22, a11, a22, a21 - a22, a12 - a11, a11 + a21, a12 + a22]


def _combine(n):
    return (n[0] - n[4] + n[3] + n[6], n[1] + n[3], n[4] + n[2], n[0] - n[1] + n[2] + n[5])


def _operands(parts):
    h = parts[0][0].shape[1] // 2
    ops = [_combos(top[:, :h], top[:, h:], bot[:, :h], bot[:, h:]) + [top[:, h:], bot[:, :h]]
           for top, bot in parts]
    return [_pack_rows(pair) for pair in zip(*ops)]


def _pin(dst, v, zero):
    lead = (0,) * (len(dst.shape) - 2)
    rows = 8 * (4 // jnp.dtype(dst.dtype).itemsize)
    v = pltpu.bitcast(v[v.shape[0] - 8:, :LANES], dst.dtype)
    dst[lead + (pl.ds(dst.shape[-2] - rows + zero, rows), slice(0, LANES))] = v


def _kernel(x_hbm, wq_hbm, wk_hbm, wv_hbm, wao_hbm, wup_hbm, dw_hbm, wdn_hbm, wm_hbm,
            o_hbm,
            x_buf, xh_buf, xs_all, wst, dw_in, wf32, wc, wg, g_next, cb, xn_buf,
            s_even, s_odd, a_even, a_odd, y_buf, o_buf,
            x_sem, h_sem, w_sem, o_sem):
    B, D = xs_all.shape[0], x_hbm.shape[1]
    T = x_hbm.shape[0] // B
    KW = dw_hbm.shape[0]
    TP = s_even.shape[1]
    NQ = T // BQ
    NB = B * NQ
    NL = D // LANES
    NC = TP // BK
    HB = BQ // 2
    HD = D // 2
    G, U, W, Z = (NL * j for j in range(4))

    def x_copy(n):
        r = pl.ds(pl.multiple_of(n * BQ, BQ), BQ)
        return pltpu.make_async_copy(x_hbm.at[r, :], x_buf.at[r, :], x_sem.at[n])

    def o_copy(n, slot):
        r = pl.ds(pl.multiple_of(n * BQ, BQ), BQ)
        return pltpu.make_async_copy(o_buf.at[slot], o_hbm.at[r, :], o_sem.at[slot])

    heads = [(b, i) for b in range(B) for i in range(1, NQ)]
    h_copies = [pltpu.make_async_copy(x_hbm.at[b * T + i * BQ:b * T + i * BQ + HALO, :],
                                      xh_buf.at[j * HALO:(j + 1) * HALO, :], h_sem)
                for j, (b, i) in enumerate(heads)]
    WQ, WK, WV, WAO, WMA, WDN, WMC, WU, WG, W1, XH = range(11)
    w_src = [wq_hbm, wk_hbm, wv_hbm, wao_hbm, wm_hbm.at[0:D], wdn_hbm, wm_hbm.at[D:2 * D],
             wup_hbm.at[:, 0:D], wup_hbm.at[:, D:2 * D]]
    w_copies = [pltpu.make_async_copy(src, wst.at[j], w_sem.at[j]) for j, src in enumerate(w_src)]
    dw_copy = pltpu.make_async_copy(dw_hbm, dw_in, w_sem.at[len(w_src)])
    QK, VA, DC, UU = range(4)
    RB = HALO * len(heads)
    NRB = D // RB

    def ln_rows(r0, t0, nrows):
        words = [pltpu.bitcast(x_buf[pl.ds(r0 + h * HB + t0, nrows), :], U32) for h in range(2)]
        return _operands([[_ln(_unpack_rows(w, parity)) for w in words] for parity in range(2)])

    for c in (w_copies[WQ], w_copies[WK], dw_copy, w_copies[WV], w_copies[WAO]):
        c.start()
    for b in range(B):
        xs_all[b, :, T // 4:TP // 2, :] = jnp.zeros((9, TP // 2 - T // 4, HD), U32)
    cb[G:G + NL, BQ:BQ + HALO, :] = jnp.zeros((NL, HALO, LANES), F32)
    for b in range(B):
        g_next[b * NQ + NQ - 1] = jnp.zeros((HALO, D), F32)
    w_copies[WQ].wait()
    w_copies[WK].wait()
    x_copy(0).start()
    x_copy(1).start()

    def put_folded(j, r, v):
        for l in range(NL):
            wf32[j, l, r, :] = v[:, l * LANES:(l + 1) * LANES]

    def fold_qk(t, c):
        r = pl.ds(pl.multiple_of(t * RB, RB), RB)
        put_folded(QK, r, _dot_nt(wst[WQ, r, :], wst[WK]) * (math.log2(math.e) / math.sqrt(D)))
        return c
    lax.fori_loop(0, NRB, fold_qk, 0)

    def put_operands(j, t0, parts):
        for k, v in enumerate(_operands(parts)[:7]):
            wc[j, k, pl.ds(pl.multiple_of(t0 // 2, HD // 4), HD // 4), :] = v

    def split_folded(t, c):
        j, t0 = t // 2, (t % 2) * (HD // 2)
        put_operands(j, t0, [[jnp.concatenate(
            [wf32[j, l, pl.ds(h * HD + t0 + parity, HD // 4, stride=2), :] for l in range(NL)], axis=1)
            for h in range(2)] for parity in range(2)])
        return c
    lax.fori_loop(0, 2, split_folded, 0)

    dw_copy.wait()
    for l in range(NL):
        cb[Z + l, 0:KW, :] = 0.5 * dw_in[:, l * LANES:(l + 1) * LANES].astype(F32)

    def spread_taps(k, c):
        for l in range(NL):
            cb[W + l, pl.ds(pl.multiple_of(8 * k, 8), 8), :] = jnp.broadcast_to(
                cb[Z + l, pl.ds(k, 1), :], (8, LANES))
        return c
    lax.fori_loop(0, KW, spread_taps, 0)

    PB = HB // HALO

    def ln_first(u, nrows):
        r0 = pl.multiple_of((u // PB) * BQ + (u % PB) * HALO, HALO)
        for k, v in enumerate(ln_rows(r0, 0, nrows)):
            xs_all[0, k, pl.ds(pl.multiple_of(u * (HALO // 2), HALO // 2), nrows // 2), :] = v

    NF = 3 * NRB + 1
    PF = -(-(NQ - 1) * PB // NF)
    assert NQ == 5 and NRB == 4 and (PB // PF, 2 * PB // PF, 3 * PB // PF) == (3, 6, 9)
    arrivals = {
        0: ([w_copies[WV], w_copies[WAO], x_copy(0)], [w_copies[WMA], x_copy(2)]),
        3: ([x_copy(1)], [w_copies[WDN], w_copies[WMC]]),
        4: ([w_copies[WMA]], [x_copy(3)]),
        6: ([x_copy(2)], [w_copies[WG]] + h_copies),
        8: ([w_copies[WDN], w_copies[WMC]], [w_copies[WU], x_copy(4)]),
        9: ([x_copy(3)], []),
    }

    def fold(t, c):
        for step, (done, new) in arrivals.items():
            @pl.when(t == step)
            def _():
                for cp in done:
                    cp.wait()
                for cp in new:
                    cp.start()

        @pl.when(t == NF - 1)
        def _():
            for cp in [w_copies[WG]] + h_copies:
                cp.wait()
            wst[XH, 0:RB, :] = _ln(xh_buf[...].astype(F32)).astype(BF16)

        j = t // NRB
        left = jnp.where(j == 0, WV, jnp.where(j == 1, W1, jnp.where(j == 2, WDN, XH)))
        right = jnp.where(j == 0, WAO, jnp.where(j == 1, WMA, jnp.where(j == 2, WMC, WG)))
        r = pl.ds(pl.multiple_of((t % NRB) * RB, RB), RB)
        v = _dot(wst[left, r, :], wst[right])
        put_folded(jnp.where(j == 1, VA, jnp.where(j == 2, DC, QK)), r, v)
        wst[jnp.where(j == 0, W1, WQ), r, :] = v.astype(BF16)
        for k in range(PF):
            ln_first(jnp.minimum(PF * t + k, (NQ - 1) * PB - 1), HALO)
        return c
    lax.fori_loop(0, NF, fold, 0)

    gate_heads = _gate(_gelu2(jnp.concatenate([wf32[QK, l, 0:RB, :] for l in range(NL)], axis=1)))
    for j, (b, i) in enumerate(heads):
        g_next[b * NQ + i - 1] = gate_heads[j * HALO:(j + 1) * HALO]
    lax.fori_loop(2, 6, split_folded, 0)
    w_copies[WU].wait()

    def split_plain(t, c):
        t0 = t * (HD // 2)
        words = [pltpu.bitcast(wst[WU, pl.ds(pl.multiple_of(h * HD + t0, HD // 2), HD // 2), :], U32)
                 for h in range(2)]
        put_operands(UU, t0, [[_unpack_rows(w, parity) for w in words] for parity in range(2)])
        wg[pl.ds(pl.multiple_of(t0, HD // 2), HD // 2), :] = pltpu.bitcast(
            wst[WG, pl.ds(pl.multiple_of(2 * t0, HD), HD), :], U32)
        return c
    lax.fori_loop(0, 2, split_plain, 0)

    x_copy(NQ - 1).wait()
    x_copy(NQ).start()

    def ln_last(t, c):
        ln_first((NQ - 1) * PB + 5 * t, 5 * HALO)
        return c
    lax.fori_loop(0, PB // 5, ln_last, 0)

    wqk, wva, wdc, wu = (wc.at[j] for j in (QK, VA, DC, UU))
    s_par = (s_even, s_odd)
    a_par = (a_even, a_odd)
    SW = TP // 2

    def block(q):
        return (q // 2) * HB, slice((q % 2) * HD, (q % 2 + 1) * HD)

    def body(n, carry):
        b, i = carry
        b_next = jnp.where(b + 1 < B, b + 1, 0)
        xs = xs_all.at[b]
        slot = n & 1
        r0 = pl.multiple_of(n * BQ, BQ)
        r_next = pl.multiple_of((b_next * NQ + i) * BQ, BQ)
        h0 = pl.multiple_of(i * (HB // 2), HB // 2)

        @pl.when(n + NQ < NB)
        def _():
            x_copy(n + NQ).wait()

        @pl.when(n + NQ + 1 < NB)
        def _():
            x_copy(n + NQ + 1).start()

        @pl.when(n >= 2)
        def _():
            o_copy(n - 2, slot).wait()

        zero_ld = pl.multiple_of((n // NB) * 16, 16)
        zero_st = pl.multiple_of((n // (NB + 1)) * 16, 16)
        pin = functools.partial(_pin, zero=zero_st)

        def project(w, order):
            out = [None] * 7
            for k in order:
                l, r = PAIRS[k]
                out[k] = _dot(_as_bf16(xs[l, pl.ds(h0, HB // 2), :]), _as_bf16(w[r]))
            return _combine(out)

        for l in range(NL):
            cb[G + l, 0:HALO, :] = jnp.where(i == 0, 0.0, cb[G + l, BQ:BQ + HALO, :])
            cb[G + l, BQ + HALO:BQ + 2 * HALO, :] = g_next[n, :, l * LANES:(l + 1) * LANES]

        for h, planes in enumerate(((1, 7), (8, 2))):
            rows = jnp.concatenate([xs[l, pl.ds(h0, HB // 2), :] for l in planes], axis=1)
            g = _gate(_gelu2(_dot(_as_bf16(rows), _as_bf16(wg[...]))))
            for l in range(NL):
                cb[G + l, HALO + h * HB:HALO + (h + 1) * HB, :] = g[:, l * LANES:(l + 1) * LANES]
        for q, v in enumerate(project(wu, ORDER)):
            for l in range(NL // 2):
                cb[U + (q % 2) * (NL // 2) + l, (q // 2) * HB:(q // 2 + 1) * HB, :] = (
                    v[:, l * LANES:(l + 1) * LANES])
        pin(cb, v)
        q11, q12, q21, q22 = project(wqk, ORDER)
        queries = [v.astype(BF16) for v in
                   (q11 + q22, q21 + q22, q11, q22, q11 + q12, q21 - q11, q12 - q22)]

        def conv_step(l, t0, nrows):
            acc = [None] * (nrows // 8)
            off = HALO - KW // 2
            for s in range(8):
                taps = [(a, 8 * a + s - off) for a in range((KW + off + 7) // 8)
                        if 0 <= 8 * a + s - off < KW]
                w = {a: cb[W + l, 8 * k:8 * k + 8, :] for a, k in taps}
                for j in range(len(acc) + max(a for a, _ in taps)):
                    use = [a for a, _ in taps if 0 <= j - a < len(acc)]
                    if not use:
                        continue
                    gv = cb[G + l, t0 + 8 * j + s:t0 + 8 * j + s + 8, :]
                    for a in use:
                        t = gv * w[a]
                        acc[j - a] = t if acc[j - a] is None else acc[j - a] + t
            cb[Z + l, pl.ds(zero_st + t0, nrows), :] = (
                jnp.concatenate(acc, axis=0) * _gelu2(cb[U + l, t0:t0 + nrows, :]))

        for t0 in range(0, BQ, CONV_ROWS):
            for l in range(NL):
                conv_step(l, t0, min(CONV_ROWS, BQ - t0))

        def keys(j, c):
            return _as_bf16(xs[j, c * BK // 2:(c + 1) * BK // 2, :])

        m = [None, None]
        for c in range(NC):
            prod = [None] * 7
            for k in SCORE_ORDER:
                prod[k] = _dot_nt(queries[k], keys(KEY_OPERAND[k], c))
            s11, s21, s12, s22 = _combine(prod)
            for q, s in enumerate((s11, s12, s21, s22)):
                if (c + 1) * BK > T // 2:
                    col = lax.broadcasted_iota(jnp.int32, (HB, BK), 1)
                    s = jnp.where(col < T // 2 - c * BK, s, -jnp.inf)
                c0 = (q % 2) * SW + (c // 2) * BK
                s_par[c % 2][(q // 2) * HB:(q // 2 + 1) * HB, c0:c0 + BK] = s
                for l in range(BK // LANES):
                    t = s[:, l * LANES:(l + 1) * LANES]
                    m[q // 2] = t if m[q // 2] is None else jnp.maximum(m[q // 2], t)
        row_max = [jnp.max(v, axis=-1, keepdims=True) for v in m]
        scale = [1.0 / jnp.sum(jnp.exp2(v - top), axis=-1, keepdims=True) for v, top in zip(m, row_max)]

        def weights(c):
            p, part = [], [None, None]
            for q in range(4):
                c0 = (q % 2) * SW + (c // 2) * BK
                rows = pl.ds((zero_ld if c == 0 else 0) + (q // 2) * HB, HB)
                e = jnp.exp2(s_par[c % 2][rows, c0:c0 + BK] - row_max[q // 2]) * scale[q // 2]
                for l in range(BK // LANES):
                    t = e[:, l * LANES:(l + 1) * LANES]
                    part[q // 2] = t if part[q // 2] is None else part[q // 2] + t
                p.append(e)
            return [v.astype(BF16) for v in _combos(*p)], jnp.concatenate(part, axis=1)

        def accumulate(c, k, d):
            if c > 0:
                d = d + a_par[(c - 1) % 2][k, 0:HB, :]
            if c + 1 < NC:
                a_par[c % 2][k, 0:HB, :] = d
            return d

        def merge(quads, w, after=None):
            left = _combos(*quads)
            out = [None] * 7
            for step, k in enumerate(MERGE_ORDER):
                l, r = PAIRS[k]
                out[k] = _dot(left[l].astype(BF16), _as_bf16(w[r]))
                if after:
                    after(step + 1, out[k])
            return _combine(out)

        def ln_next():
            for t0 in range(0, HB, LN_ROWS):
                nrows = min(LN_ROWS, HB - t0)
                for j, v in enumerate(ln_rows(r_next, t0, nrows)):
                    xn_buf[j, t0 // 2:(t0 + nrows) // 2, :] = v
                pin(x_buf if t0 + LN_ROWS < HB else xs, xn_buf[0, pl.ds(zero_ld, 8), :])

        def publish(step, v):
            if step < len(PUBLISH) and PUBLISH[step]:
                pin(xn_buf, v)
                for j in PUBLISH[step]:
                    xs_all[b_next, j, pl.ds(h0, HB // 2), :] = xn_buf[j, 0:HB // 2, :]

        nxt = weights(0)

        z = [jnp.concatenate([cb[Z + (q % 2) * (NL // 2) + l, (q // 2) * HB:(q // 2 + 1) * HB, :]
                              for l in range(NL // 2)], axis=1) for q in range(4)]
        for q, v in enumerate(merge(z, wdc)):
            rows, cols = block(q)
            y_buf[q, 0:HB, :] = v + x_buf[pl.ds(r0 + rows, HB), cols].astype(F32)

        for c in range(NC):
            p, part = nxt
            acc = [None] * 7
            for step, k in enumerate(ORDER):
                l, r = PAIRS[k]
                if c == LN_CHUNK and step == 0:
                    ln_next()
                d = _dot(p[l], keys(r, c))
                if step == PIN_STEP and c + 1 < NC:
                    pin(s_par[(c + 1) % 2], d)
                    nxt = weights(c + 1)
                acc[k] = accumulate(c, k, d)
            total = accumulate(c, 7, part)
            if c + 1 < NC:
                pin(a_par[c % 2], total)
        o11, o12, o21, o22 = _combine(acc)
        inv = [1.0 / jnp.sum(v, axis=-1, keepdims=True) for v in (total[:, :LANES], total[:, LANES:])]

        pin(y_buf, acc[ORDER[0]])
        publish(0, acc[ORDER[6]])
        for q, v in enumerate(merge((o11 * inv[0], o12 * inv[0], o21 * inv[1], o22 * inv[1]), wva, publish)):
            rows, cols = block(q)
            o_buf[slot, rows:rows + HB, cols] = (v + y_buf[q, 0:HB, :]).astype(o_buf.dtype)
        o_copy(n, slot).start()
        last = i + 1 == NQ
        return jnp.where(last, b + 1, b), jnp.where(last, 0, i + 1)

    lax.fori_loop(0, NB, body, (jnp.int32(0), jnp.int32(0)))
    o_copy(NB - 2, (NB - 2) % 2).wait()
    o_copy(NB - 1, (NB - 1) % 2).wait()


@jax.jit
def pallas_standalone__conformer_family_branchformer__speech_kernel(
    x: jax.Array,
    w_q: jax.Array,
    w_k: jax.Array,
    w_v: jax.Array,
    w_ao: jax.Array,
    w_up: jax.Array,
    dw: jax.Array,
    w_dn: jax.Array,
    w_merge: jax.Array,
):
    B, T, D = x.shape
    KW = dw.shape[0]
    TP = -(-(T // 2) // BK) * BK
    NL, NQ, HB, HD = D // LANES, T // BQ, BQ // 2, D // 2
    assert T % BQ == 0 and BK == HD == 2 * LANES and KW // 2 < HALO
    vmem, dma = pltpu.VMEM, pltpu.SemaphoreType.DMA
    scratch = [
        vmem((B * T + SPARE, D), BF16),
        vmem((B * (NQ - 1) * HALO, D), BF16),
        vmem((B, 9, TP // 2 + SPARE, HD), U32),
        vmem((11, D, D), BF16),
        vmem((KW, D), BF16),
        vmem((3, NL, D + 8, LANES), F32),
        vmem((4, 7, HD // 2, HD), U32),
        vmem((HD, D), U32),
        vmem((B * NQ, HALO, D), F32),
        vmem((4 * NL, BQ + 2 * HALO + SPARE, LANES), F32),
        vmem((9, HB // 2 + SPARE, HD), U32),
        vmem((BQ + SPARE, TP), F32),
        vmem((BQ + SPARE, TP), F32),
        vmem((8, HB + SPARE, HD), F32),
        vmem((8, HB + SPARE, HD), F32),
        vmem((4, HB + SPARE, HD), F32),
        vmem((2, BQ, D), x.dtype),
        dma((B * NQ,)), dma(()), dma((10,)), dma((2,)),
    ]
    in_hbm = pl.BlockSpec(memory_space=pl.ANY)
    return pl.pallas_call(
        _kernel,
        out_shape=jax.ShapeDtypeStruct((B * T, D), x.dtype),
        in_specs=[in_hbm] * 9,
        out_specs=in_hbm,
        scratch_shapes=scratch,
        compiler_params=pltpu.CompilerParams(vmem_limit_bytes=110 * 1024 * 1024),
    )(x.reshape(B * T, D), w_q, w_k, w_v, w_ao, w_up, dw, w_dn, w_merge).reshape(B, T, D)
```

```python
import functools
import math

import jax
import jax.numpy as jnp
from jax import lax
from jax.experimental import pallas as pl
from jax.experimental.pallas import tpu as pltpu

F32 = jnp.float32
BF16 = jnp.bfloat16
U32 = jnp.uint32
EPS = 1e-5
LANES = 128
HALO = 16
SPARE = 16

BQ = 800
BK = 256
CONV_ROWS = 24
LN_ROWS = 32
PIN_STEP = 1
LN_CHUNK = 4

PAIRS = ((0, 0), (1, 6), (3, 1), (4, 2), (2, 5), (5, 4), (6, 3))
KEY_OPERAND = (0, 1, 3, 4, 2, 5, 6)
ORDER = (1, 4, 0, 3, 2, 5, 6)
SCORE_ORDER = (0, 1, 4, 3, 2, 5, 6)
MERGE_ORDER = (4, 2, 1, 0, 3, 5, 6)
PUBLISH = ((0, 7), (1,), (2, 3), (4,), (5, 8), (6,))


def _ln(x, eps=EPS):
    d = x.shape[-1]
    m = jnp.sum(x, axis=-1, keepdims=True) * (1.0 / d)
    c = x - m
    v = jnp.sum(c * c, axis=-1, keepdims=True) * (1.0 / d)
    return c * lax.rsqrt(v + eps)


def _gelu2(x):
    c1 = math.sqrt(2.0 / math.pi)
    c2 = c1 * 0.044715
    return x + x * jnp.tanh(x * (c1 + c2 * (x * x)))


def _gate(h2):
    return _ln(h2, 4.0 * EPS)


def _dot(a, b):
    return jnp.dot(a, b, preferred_element_type=F32)


def _dot_nt(a, b):
    return lax.dot_general(a, b, (((1,), (1,)), ((), ())), preferred_element_type=F32)


def _as_bf16(words):
    return pltpu.bitcast(words, BF16)


def _pack_rows(pair):
    return pltpu.bitcast(pltpu.pack_elementwise(pair, packed_dtype=BF16), U32)


def _unpack_rows(words, parity):
    return pltpu.unpack_elementwise(words, index=parity, packed_dtype=BF16, unpacked_dtype=F32)


def _combos(a11, a12, a21, a22):
    return [a11 + a22, a11, a22, a21 - a22, a12 - a11, a11 + a21, a12 + a22]


def _combine(n):
    return (n[0] - n[4] + n[3] + n[6], n[1] + n[3], n[4] + n[2], n[0] - n[1] + n[2] + n[5])


def _operands(parts):
    h = parts[0][0].shape[1] // 2
    ops = [_combos(top[:, :h], top[:, h:], bot[:, :h], bot[:, h:]) + [top[:, h:], bot[:, :h]]
           for top, bot in parts]
    return [_pack_rows(pair) for pair in zip(*ops)]


def _pin(dst, v, zero):
    lead = (0,) * (len(dst.shape) - 2)
    rows = 8 * (4 // jnp.dtype(dst.dtype).itemsize)
    v = pltpu.bitcast(v[v.shape[0] - 8:, :LANES], dst.dtype)
    dst[lead + (pl.ds(dst.shape[-2] - rows + zero, rows), slice(0, LANES))] = v


def _kernel(x_hbm, wq_hbm, wk_hbm, wv_hbm, wao_hbm, wup_hbm, dw_hbm, wdn_hbm, wm_hbm,
            o_hbm,
            x_buf, xs_all, wst, dw_in, wf32, wc, wg, cb, xn_buf,
            s_even, s_odd, a_even, a_odd, y_buf, o_buf,
            x_sem, w_sem, o_sem):
    B, D = xs_all.shape[0], x_hbm.shape[1]
    T = x_hbm.shape[0] // B
    KW = dw_hbm.shape[0]
    TP = s_even.shape[1]
    NQ = T // BQ
    NB = B * NQ
    NL = D // LANES
    NC = TP // BK
    HB = BQ // 2
    HD = D // 2
    G, U, W, Z = (NL * j for j in range(4))

    def x_copy(n):
        r = pl.ds(pl.multiple_of(n * BQ, BQ), BQ)
        return pltpu.make_async_copy(x_hbm.at[r, :], x_buf.at[r, :], x_sem.at[n])

    def o_copy(n, slot):
        r = pl.ds(pl.multiple_of(n * BQ, BQ), BQ)
        return pltpu.make_async_copy(o_buf.at[slot], o_hbm.at[r, :], o_sem.at[slot])

    WQ, WK, WV, WAO, WMA, WDN, WMC, WU, WG, W1 = range(10)
    w_src = [wq_hbm, wk_hbm, wv_hbm, wao_hbm, wm_hbm.at[0:D], wdn_hbm, wm_hbm.at[D:2 * D],
             wup_hbm.at[:, 0:D], wup_hbm.at[:, D:2 * D]]
    w_copies = [pltpu.make_async_copy(src, wst.at[j], w_sem.at[j]) for j, src in enumerate(w_src)]
    dw_copy = pltpu.make_async_copy(dw_hbm, dw_in, w_sem.at[len(w_src)])
    QK, VA, DC, UU = range(4)
    RB = 128
    NRB = D // RB

    def ln_rows(r0, t0, nrows):
        words = [pltpu.bitcast(x_buf[pl.ds(r0 + h * HB + t0, nrows), :], U32) for h in range(2)]
        return _operands([[_ln(_unpack_rows(w, parity)) for w in words] for parity in range(2)])

    for c in (w_copies[WQ], w_copies[WK], dw_copy, w_copies[WV], w_copies[WAO]):
        c.start()
    for b in range(B):
        xs_all[b, :, T // 4:TP // 2, :] = jnp.zeros((9, TP // 2 - T // 4, HD), U32)
    cb[G:G + NL, BQ:BQ + HALO, :] = jnp.zeros((NL, HALO, LANES), F32)
    w_copies[WQ].wait()
    w_copies[WK].wait()
    x_copy(0).start()
    x_copy(1).start()

    def put_folded(j, r, v):
        for l in range(NL):
            wf32[j, l, r, :] = v[:, l * LANES:(l + 1) * LANES]

    def fold_qk(t, c):
        r = pl.ds(pl.multiple_of(t * RB, RB), RB)
        put_folded(QK, r, _dot_nt(wst[WQ, r, :], wst[WK]) * (math.log2(math.e) / math.sqrt(D)))
        return c
    lax.fori_loop(0, NRB, fold_qk, 0)

    def put_operands(j, t0, parts):
        for k, v in enumerate(_operands(parts)[:7]):
            wc[j, k, pl.ds(pl.multiple_of(t0 // 2, HD // 4), HD // 4), :] = v

    def split_folded(t, c):
        j, t0 = t // 2, (t % 2) * (HD // 2)
        put_operands(j, t0, [[jnp.concatenate(
            [wf32[j, l, pl.ds(h * HD + t0 + parity, HD // 4, stride=2), :] for l in range(NL)], axis=1)
            for h in range(2)] for parity in range(2)])
        return c
    lax.fori_loop(0, 2, split_folded, 0)

    dw_copy.wait()
    for l in range(NL):
        cb[Z + l, 0:KW, :] = 0.5 * dw_in[:, l * LANES:(l + 1) * LANES].astype(F32)

    def spread_taps(k, c):
        for l in range(NL):
            cb[W + l, pl.ds(pl.multiple_of(8 * k, 8), 8), :] = jnp.broadcast_to(
                cb[Z + l, pl.ds(k, 1), :], (8, LANES))
        return c
    lax.fori_loop(0, KW, spread_taps, 0)

    PB = HB // HALO

    def ln_first(u, nrows):
        r0 = pl.multiple_of((u // PB) * BQ + (u % PB) * HALO, HALO)
        for k, v in enumerate(ln_rows(r0, 0, nrows)):
            xs_all[0, k, pl.ds(pl.multiple_of(u * (HALO // 2), HALO // 2), nrows // 2), :] = v

    NF = 3 * NRB
    PF = -(-(NQ - 1) * PB // NF)
    assert NQ == 5 and NRB == 4 and (PB // PF, 2 * PB // PF, 3 * PB // PF) == (2, 5, 8)
    arrivals = {
        0: ([w_copies[WV], w_copies[WAO], x_copy(0)], [w_copies[WMA], x_copy(2)]),
        2: ([x_copy(1)], [w_copies[WDN], w_copies[WMC]]),
        4: ([w_copies[WMA]], [x_copy(3)]),
        5: ([x_copy(2)], [w_copies[WU], w_copies[WG]]),
        8: ([w_copies[WDN], w_copies[WMC], x_copy(3)], [x_copy(4)]),
    }

    def fold(t, c):
        for step, (done, new) in arrivals.items():
            @pl.when(t == step)
            def _():
                for cp in done:
                    cp.wait()
                for cp in new:
                    cp.start()

        j = t // NRB
        left = jnp.where(j == 0, WV, jnp.where(j == 1, W1, WDN))
        right = jnp.where(j == 0, WAO, jnp.where(j == 1, WMA, WMC))
        r = pl.ds(pl.multiple_of((t % NRB) * RB, RB), RB)
        v = _dot(wst[left, r, :], wst[right])
        put_folded(jnp.where(j == 1, VA, jnp.where(j == 2, DC, QK)), r, v)
        wst[jnp.where(j == 0, W1, WQ), r, :] = v.astype(BF16)
        for k in range(PF):
            ln_first(jnp.minimum(PF * t + k, (NQ - 1) * PB - 1), HALO)
        return c
    lax.fori_loop(0, NF, fold, 0)

    lax.fori_loop(2, 6, split_folded, 0)
    w_copies[WU].wait()
    w_copies[WG].wait()

    def split_plain(t, c):
        t0 = t * (HD // 2)
        words = [pltpu.bitcast(wst[WU, pl.ds(pl.multiple_of(h * HD + t0, HD // 2), HD // 2), :], U32)
                 for h in range(2)]
        put_operands(UU, t0, [[_unpack_rows(w, parity) for w in words] for parity in range(2)])
        wg[pl.ds(pl.multiple_of(t0, HD // 2), HD // 2), :] = pltpu.bitcast(
            wst[WG, pl.ds(pl.multiple_of(2 * t0, HD), HD), :], U32)
        return c
    lax.fori_loop(0, 2, split_plain, 0)

    x_copy(NQ - 1).wait()
    x_copy(NQ).start()

    def ln_last(t, c):
        ln_first((NQ - 1) * PB + 5 * t, 5 * HALO)
        return c
    lax.fori_loop(0, PB // 5, ln_last, 0)

    wqk, wva, wdc, wu = (wc.at[j] for j in (QK, VA, DC, UU))
    s_par = (s_even, s_odd)
    a_par = (a_even, a_odd)
    SW = TP // 2

    def block(q):
        return (q // 2) * HB, slice((q % 2) * HD, (q % 2 + 1) * HD)

    def body(n, carry):
        b, i = carry
        b_next = jnp.where(b + 1 < B, b + 1, 0)
        xs = xs_all.at[b]
        slot = n & 1
        r0 = pl.multiple_of(n * BQ, BQ)
        r_next = pl.multiple_of((b_next * NQ + i) * BQ, BQ)
        h0 = pl.multiple_of(i * (HB // 2), HB // 2)

        @pl.when(n + NQ < NB)
        def _():
            x_copy(n + NQ).wait()

        @pl.when(n + NQ + 1 < NB)
        def _():
            x_copy(n + NQ + 1).start()

        @pl.when(n >= 2)
        def _():
            o_copy(n - 2, slot).wait()

        zero_ld = pl.multiple_of((n // NB) * 16, 16)
        zero_st = pl.multiple_of((n // (NB + 1)) * 16, 16)
        pin = functools.partial(_pin, zero=zero_st)

        def project(w, order):
            out = [None] * 7
            for k in order:
                l, r = PAIRS[k]
                out[k] = _dot(_as_bf16(xs[l, pl.ds(h0, HB // 2), :]), _as_bf16(w[r]))
            return _combine(out)

        def plain(planes, row, nrows):
            return jnp.concatenate([xs[l, pl.ds(row, nrows // 2), :] for l in planes], axis=1)

        for l in range(NL):
            cb[G + l, 0:HALO, :] = jnp.where(i == 0, 0.0, cb[G + l, BQ:BQ + HALO, :])
        lower = jnp.concatenate([plain((8, 2), h0, HB), plain((1, 7), h0 + HB // 2, HALO)], axis=0)
        for h, rows in enumerate((plain((1, 7), h0, HB), lower)):
            g = _gate(_gelu2(_dot(_as_bf16(rows), _as_bf16(wg[...]))))
            for l in range(NL):
                cb[G + l, HALO + h * HB:HALO + h * HB + g.shape[0], :] = g[:, l * LANES:(l + 1) * LANES]
        for q, v in enumerate(project(wu, ORDER)):
            for l in range(NL // 2):
                cb[U + (q % 2) * (NL // 2) + l, (q // 2) * HB:(q // 2 + 1) * HB, :] = (
                    v[:, l * LANES:(l + 1) * LANES])
        pin(cb, v)
        q11, q12, q21, q22 = project(wqk, ORDER)
        queries = [v.astype(BF16) for v in
                   (q11 + q22, q21 + q22, q11, q22, q11 + q12, q21 - q11, q12 - q22)]

        def conv_step(l, t0, nrows):
            acc = [None] * (nrows // 8)
            off = HALO - KW // 2
            for s in range(8):
                taps = [(a, 8 * a + s - off) for a in range((KW + off + 7) // 8)
                        if 0 <= 8 * a + s - off < KW]
                w = {a: cb[W + l, 8 * k:8 * k + 8, :] for a, k in taps}
                for j in range(len(acc) + max(a for a, _ in taps)):
                    use = [a for a, _ in taps if 0 <= j - a < len(acc)]
                    if not use:
                        continue
                    gv = cb[G + l, t0 + 8 * j + s:t0 + 8 * j + s + 8, :]
                    for a in use:
                        t = gv * w[a]
                        acc[j - a] = t if acc[j - a] is None else acc[j - a] + t
            cb[Z + l, pl.ds(zero_st + t0, nrows), :] = (
                jnp.concatenate(acc, axis=0) * _gelu2(cb[U + l, t0:t0 + nrows, :]))

        for t0 in range(0, BQ, CONV_ROWS):
            for l in range(NL):
                conv_step(l, t0, min(CONV_ROWS, BQ - t0))

        def keys(j, c):
            return _as_bf16(xs[j, c * BK // 2:(c + 1) * BK // 2, :])

        m = [None, None]
        for c in range(NC):
            prod = [None] * 7
            for k in SCORE_ORDER:
                prod[k] = _dot_nt(queries[k], keys(KEY_OPERAND[k], c))
            s11, s21, s12, s22 = _combine(prod)
            for q, s in enumerate((s11, s12, s21, s22)):
                if (c + 1) * BK > T // 2:
                    col = lax.broadcasted_iota(jnp.int32, (HB, BK), 1)
                    s = jnp.where(col < T // 2 - c * BK, s, -jnp.inf)
                c0 = (q % 2) * SW + (c // 2) * BK
                s_par[c % 2][(q // 2) * HB:(q // 2 + 1) * HB, c0:c0 + BK] = s
                for l in range(BK // LANES):
                    t = s[:, l * LANES:(l + 1) * LANES]
                    m[q // 2] = t if m[q // 2] is None else jnp.maximum(m[q // 2], t)
        row_max = [jnp.max(v, axis=-1, keepdims=True) for v in m]
        scale = [1.0 / jnp.sum(jnp.exp2(v - top), axis=-1, keepdims=True) for v, top in zip(m, row_max)]

        def weights(c):
            p, part = [], [None, None]
            for q in range(4):
                c0 = (q % 2) * SW + (c // 2) * BK
                rows = pl.ds((zero_ld if c == 0 else 0) + (q // 2) * HB, HB)
                e = jnp.exp2(s_par[c % 2][rows, c0:c0 + BK] - row_max[q // 2]) * scale[q // 2]
                for l in range(BK // LANES):
                    t = e[:, l * LANES:(l + 1) * LANES]
                    part[q // 2] = t if part[q // 2] is None else part[q // 2] + t
                p.append(e)
            return [v.astype(BF16) for v in _combos(*p)], jnp.concatenate(part, axis=1)

        def accumulate(c, k, d):
            if c > 0:
                d = d + a_par[(c - 1) % 2][k, 0:HB, :]
            if c + 1 < NC:
                a_par[c % 2][k, 0:HB, :] = d
            return d

        def merge(quads, w, after=None):
            left = _combos(*quads)
            out = [None] * 7
            for step, k in enumerate(MERGE_ORDER):
                l, r = PAIRS[k]
                out[k] = _dot(left[l].astype(BF16), _as_bf16(w[r]))
                if after:
                    after(step + 1, out[k])
            return _combine(out)

        def ln_next():
            for t0 in range(0, HB, LN_ROWS):
                nrows = min(LN_ROWS, HB - t0)
                for j, v in enumerate(ln_rows(r_next, t0, nrows)):
                    xn_buf[j, t0 // 2:(t0 + nrows) // 2, :] = v
                pin(x_buf if t0 + LN_ROWS < HB else xs, xn_buf[0, pl.ds(zero_ld, 8), :])

        def publish(step, v):
            if step < len(PUBLISH) and PUBLISH[step]:
                pin(xn_buf, v)
                for j in PUBLISH[step]:
                    xs_all[b_next, j, pl.ds(h0, HB // 2), :] = xn_buf[j, 0:HB // 2, :]

        nxt = weights(0)

        z = [jnp.concatenate([cb[Z + (q % 2) * (NL // 2) + l, (q // 2) * HB:(q // 2 + 1) * HB, :]
                              for l in range(NL // 2)], axis=1) for q in range(4)]
        for q, v in enumerate(merge(z, wdc)):
            rows, cols = block(q)
            y_buf[q, 0:HB, :] = v + x_buf[pl.ds(r0 + rows, HB), cols].astype(F32)

        for c in range(NC):
            p, part = nxt
            acc = [None] * 7
            for step, k in enumerate(ORDER):
                l, r = PAIRS[k]
                if c == LN_CHUNK and step == 0:
                    ln_next()
                d = _dot(p[l], keys(r, c))
                if step == PIN_STEP and c + 1 < NC:
                    pin(s_par[(c + 1) % 2], d)
                    nxt = weights(c + 1)
                acc[k] = accumulate(c, k, d)
            total = accumulate(c, 7, part)
            if c + 1 < NC:
                pin(a_par[c % 2], total)
        o11, o12, o21, o22 = _combine(acc)
        inv = [1.0 / jnp.sum(v, axis=-1, keepdims=True) for v in (total[:, :LANES], total[:, LANES:])]

        pin(y_buf, acc[ORDER[0]])
        publish(0, acc[ORDER[6]])
        for q, v in enumerate(merge((o11 * inv[0], o12 * inv[0], o21 * inv[1], o22 * inv[1]), wva, publish)):
            rows, cols = block(q)
            o_buf[slot, rows:rows + HB, cols] = (v + y_buf[q, 0:HB, :]).astype(o_buf.dtype)
        o_copy(n, slot).start()
        last = i + 1 == NQ
        return jnp.where(last, b + 1, b), jnp.where(last, 0, i + 1)

    lax.fori_loop(0, NB, body, (jnp.int32(0), jnp.int32(0)))
    o_copy(NB - 2, (NB - 2) % 2).wait()
    o_copy(NB - 1, (NB - 1) % 2).wait()


@jax.jit
def pallas_standalone__conformer_family_branchformer__speech_kernel(
    x: jax.Array,
    w_q: jax.Array,
    w_k: jax.Array,
    w_v: jax.Array,
    w_ao: jax.Array,
    w_up: jax.Array,
    dw: jax.Array,
    w_dn: jax.Array,
    w_merge: jax.Array,
):
    B, T, D = x.shape
    KW = dw.shape[0]
    TP = -(-(T // 2) // BK) * BK
    NL, NQ, HB, HD = D // LANES, T // BQ, BQ // 2, D // 2
    assert T % BQ == 0 and BK == HD == 2 * LANES and KW // 2 < HALO <= TP - T // 2
    vmem, dma = pltpu.VMEM, pltpu.SemaphoreType.DMA
    scratch = [
        vmem((B * T + SPARE, D), BF16),
        vmem((B, 9, TP // 2 + SPARE, HD), U32),
        vmem((10, D, D), BF16),
        vmem((KW, D), BF16),
        vmem((3, NL, D + 8, LANES), F32),
        vmem((4, 7, HD // 2, HD), U32),
        vmem((HD, D), U32),
        vmem((4 * NL, BQ + 2 * HALO + SPARE, LANES), F32),
        vmem((9, HB // 2 + SPARE, HD), U32),
        vmem((BQ + SPARE, TP), F32),
        vmem((BQ + SPARE, TP), F32),
        vmem((8, HB + SPARE, HD), F32),
        vmem((8, HB + SPARE, HD), F32),
        vmem((4, HB + SPARE, HD), F32),
        vmem((2, BQ, D), x.dtype),
        dma((B * NQ,)), dma((10,)), dma((2,)),
    ]
    in_hbm = pl.BlockSpec(memory_space=pl.ANY)
    return pl.pallas_call(
        _kernel,
        out_shape=jax.ShapeDtypeStruct((B * T, D), x.dtype),
        in_specs=[in_hbm] * 9,
        out_specs=in_hbm,
        scratch_shapes=scratch,
        compiler_params=pltpu.CompilerParams(vmem_limit_bytes=110 * 1024 * 1024),
    )(x.reshape(B * T, D), w_q, w_k, w_v, w_ao, w_up, dw, w_dn, w_merge).reshape(B, T, D)
```

```python
import functools
import math

import jax
import jax.numpy as jnp
from jax import lax
from jax.experimental import pallas as pl
from jax.experimental.pallas import tpu as pltpu

F32 = jnp.float32
BF16 = jnp.bfloat16
U32 = jnp.uint32
EPS = 1e-5
LANES = 128
HALO = 16
SPARE = 16

BQ = 800
BK = 256
CONV_ROWS = 24
LN_ROWS = 32
PIN_STEP = 1
LN_CHUNK = 4

PAIRS = ((0, 0), (1, 6), (3, 1), (4, 2), (2, 5), (5, 4), (6, 3))
KEY_OPERAND = (0, 1, 3, 4, 2, 5, 6)
ORDER = (1, 4, 0, 3, 2, 5, 6)
SCORE_ORDER = (0, 1, 4, 3, 2, 5, 6)
MERGE_ORDER = (4, 2, 1, 0, 3, 5, 6)
PUBLISH = ((0, 7), (1,), (2, 3), (4,), (5, 8), (6,))


def _ln(x, eps=EPS):
    d = x.shape[-1]
    m = jnp.sum(x, axis=-1, keepdims=True) * (1.0 / d)
    c = x - m
    v = jnp.sum(c * c, axis=-1, keepdims=True) * (1.0 / d)
    return c * lax.rsqrt(v + eps)


def _gelu2(x):
    c1 = math.sqrt(2.0 / math.pi)
    c2 = c1 * 0.044715
    return x + x * jnp.tanh(x * (c1 + c2 * (x * x)))


def _gate(h2):
    return _ln(h2, 4.0 * EPS)


def _dot(a, b):
    return jnp.dot(a, b, preferred_element_type=F32)


def _dot_nt(a, b):
    return lax.dot_general(a, b, (((1,), (1,)), ((), ())), preferred_element_type=F32)


def _as_bf16(words):
    return pltpu.bitcast(words, BF16)


def _as_words(v):
    return pltpu.bitcast(v.astype(BF16), U32)


def _combos(a11, a12, a21, a22):
    return [a11 + a22, a11, a22, a21 - a22, a12 - a11, a11 + a21, a12 + a22]


def _combine(n):
    return (n[0] - n[4] + n[3] + n[6], n[1] + n[3], n[4] + n[2], n[0] - n[1] + n[2] + n[5])


def _operands(top, bot):
    h = top.shape[1] // 2
    return _combos(top[:, :h], top[:, h:], bot[:, :h], bot[:, h:]) + [top[:, h:], bot[:, :h]]


def _pin(dst, v, zero):
    lead = (0,) * (len(dst.shape) - 2)
    rows = 8 * (4 // jnp.dtype(dst.dtype).itemsize)
    v = pltpu.bitcast(v[v.shape[0] - 8:, :LANES], dst.dtype)
    dst[lead + (pl.ds(dst.shape[-2] - rows + zero, rows), slice(0, LANES))] = v


def _kernel(x_hbm, wq_hbm, wk_hbm, wv_hbm, wao_hbm, wup_hbm, dw_hbm, wdn_hbm, wm_hbm,
            o_hbm,
            x_buf, xs_all, wst, dw_in, wf32, wc, wg, cb, xn_buf,
            s_even, s_odd, a_even, a_odd, y_buf, o_buf,
            x_sem, w_sem, o_sem):
    B, D = xs_all.shape[0], x_hbm.shape[1]
    T = x_hbm.shape[0] // B
    KW = dw_hbm.shape[0]
    TP = s_even.shape[1]
    NQ = T // BQ
    NB = B * NQ
    NL = D // LANES
    NC = TP // BK
    HB = BQ // 2
    HD = D // 2
    G, U, W, Z = (NL * j for j in range(4))

    def x_copy(n):
        r = pl.ds(pl.multiple_of(n * BQ, BQ), BQ)
        return pltpu.make_async_copy(x_hbm.at[r, :], x_buf.at[r, :], x_sem.at[n])

    def o_copy(n, slot):
        r = pl.ds(pl.multiple_of(n * BQ, BQ), BQ)
        return pltpu.make_async_copy(o_buf.at[slot], o_hbm.at[r, :], o_sem.at[slot])

    WQ, WK, WV, WAO, WMA, WDN, WMC, WU, WG, W1 = range(10)
    w_src = [wq_hbm, wk_hbm, wv_hbm, wao_hbm, wm_hbm.at[0:D], wdn_hbm, wm_hbm.at[D:2 * D],
             wup_hbm.at[:, 0:D], wup_hbm.at[:, D:2 * D]]
    w_copies = [pltpu.make_async_copy(src, wst.at[j], w_sem.at[j]) for j, src in enumerate(w_src)]
    dw_copy = pltpu.make_async_copy(dw_hbm, dw_in, w_sem.at[len(w_src)])
    QK, VA, DC, UU = range(4)
    RB = 128
    NRB = D // RB

    def ln_rows(r0, t0, nrows):
        halves = [_ln(x_buf[pl.ds(r0 + h * HB + t0, nrows), :].astype(F32)) for h in range(2)]
        return _operands(*halves)

    for c in (w_copies[WQ], w_copies[WK], dw_copy, w_copies[WV], w_copies[WAO]):
        c.start()
    for b in range(B):
        xs_all[b, :, T // 4:TP // 2, :] = jnp.zeros((9, TP // 2 - T // 4, HD), U32)
    cb[G:G + NL, BQ:BQ + HALO, :] = jnp.zeros((NL, HALO, LANES), F32)
    w_copies[WQ].wait()
    w_copies[WK].wait()
    x_copy(0).start()
    x_copy(1).start()

    def fold_qk(t, c):
        r = pl.ds(pl.multiple_of(t * RB, RB), RB)
        wf32[QK, r, :] = _dot_nt(wst[WQ, r, :], wst[WK]) * (math.log2(math.e) / math.sqrt(D))
        return c
    lax.fori_loop(0, NRB, fold_qk, 0)

    def split(src, j, t0):
        halves = [src[pl.ds(pl.multiple_of(h * HD + t0, HD // 2), HD // 2), :].astype(F32) for h in range(2)]
        for k, v in enumerate(_operands(*halves)[:7]):
            wc[j, k, pl.ds(pl.multiple_of(t0 // 2, HD // 4), HD // 4), :] = _as_words(v)

    def split_folded(t, c):
        split(wf32.at[t // 2], t // 2, (t % 2) * (HD // 2))
        return c
    lax.fori_loop(0, 2, split_folded, 0)

    dw_copy.wait()
    for l in range(NL):
        cb[Z + l, 0:KW, :] = 0.5 * dw_in[:, l * LANES:(l + 1) * LANES].astype(F32)

    def spread_taps(k, c):
        for l in range(NL):
            cb[W + l, pl.ds(pl.multiple_of(8 * k, 8), 8), :] = jnp.broadcast_to(
                cb[Z + l, pl.ds(k, 1), :], (8, LANES))
        return c
    lax.fori_loop(0, KW, spread_taps, 0)

    PB = HB // HALO

    def ln_first(u, nrows):
        r0 = pl.multiple_of((u // PB) * BQ + (u % PB) * HALO, HALO)
        for k, v in enumerate(ln_rows(r0, 0, nrows)):
            xs_all[0, k, pl.ds(pl.multiple_of(u * (HALO // 2), HALO // 2), nrows // 2), :] = _as_words(v)

    NF = 3 * NRB
    PF = -(-(NQ - 1) * PB // NF)
    assert NQ == 5 and NRB == 4 and (PB // PF, 2 * PB // PF, 3 * PB // PF) == (2, 5, 8)
    arrivals = {
        0: ([w_copies[WV], w_copies[WAO], x_copy(0)], [w_copies[WMA], x_copy(2)]),
        2: ([x_copy(1)], [w_copies[WDN], w_copies[WMC]]),
        4: ([w_copies[WMA]], [x_copy(3)]),
        5: ([x_copy(2)], [w_copies[WU], w_copies[WG]]),
        8: ([w_copies[WDN], w_copies[WMC], x_copy(3)], [x_copy(4)]),
    }

    def fold(t, c):
        for step, (done, new) in arrivals.items():
            @pl.when(t == step)
            def _():
                for cp in done:
                    cp.wait()
                for cp in new:
                    cp.start()

        j = t // NRB
        left = jnp.where(j == 0, WV, jnp.where(j == 1, W1, WDN))
        right = jnp.where(j == 0, WAO, jnp.where(j == 1, WMA, WMC))
        r = pl.ds(pl.multiple_of((t % NRB) * RB, RB), RB)
        v = _dot(wst[left, r, :], wst[right])
        wf32[jnp.where(j == 1, VA, jnp.where(j == 2, DC, QK)), r, :] = v
        wst[jnp.where(j == 0, W1, WQ), r, :] = v.astype(BF16)
        for k in range(PF):
            ln_first(jnp.minimum(PF * t + k, (NQ - 1) * PB - 1), HALO)
        return c
    lax.fori_loop(0, NF, fold, 0)

    lax.fori_loop(2, 6, split_folded, 0)
    w_copies[WU].wait()
    w_copies[WG].wait()

    def split_plain(t, c):
        t0 = t * (HD // 2)
        split(wst.at[WU], UU, t0)
        wg[pl.ds(pl.multiple_of(t0, HD // 2), HD // 2), :] = _as_words(
            wst[WG, pl.ds(pl.multiple_of(2 * t0, HD), HD), :])
        return c
    lax.fori_loop(0, 2, split_plain, 0)

    x_copy(NQ - 1).wait()
    x_copy(NQ).start()

    def ln_last(t, c):
        ln_first((NQ - 1) * PB + 5 * t, 5 * HALO)
        return c
    lax.fori_loop(0, PB // 5, ln_last, 0)

    wqk, wva, wdc, wu = (wc.at[j] for j in (QK, VA, DC, UU))
    s_par = (s_even, s_odd)
    a_par = (a_even, a_odd)
    SW = TP // 2

    def block(q):
        return (q // 2) * HB, slice((q % 2) * HD, (q % 2 + 1) * HD)

    def body(n, carry):
        b, i = carry
        b_next = jnp.where(b + 1 < B, b + 1, 0)
        xs = xs_all.at[b]
        slot = n & 1
        r0 = pl.multiple_of(n * BQ, BQ)
        r_next = pl.multiple_of((b_next * NQ + i) * BQ, BQ)
        h0 = pl.multiple_of(i * (HB // 2), HB // 2)

        @pl.when(n + NQ < NB)
        def _():
            x_copy(n + NQ).wait()

        @pl.when(n + NQ + 1 < NB)
        def _():
            x_copy(n + NQ + 1).start()

        @pl.when(n >= 2)
        def _():
            o_copy(n - 2, slot).wait()

        zero_ld = pl.multiple_of((n // NB) * 16, 16)
        zero_st = pl.multiple_of((n // (NB + 1)) * 16, 16)
        pin = functools.partial(_pin, zero=zero_st)

        def project(w, order):
            out = [None] * 7
            for k in order:
                l, r = PAIRS[k]
                out[k] = _dot(_as_bf16(xs[l, pl.ds(h0, HB // 2), :]), _as_bf16(w[r]))
            return _combine(out)

        def plain(planes, row, nrows):
            return jnp.concatenate([xs[l, pl.ds(row, nrows // 2), :] for l in planes], axis=1)

        for l in range(NL):
            cb[G + l, 0:HALO, :] = jnp.where(i == 0, 0.0, cb[G + l, BQ:BQ + HALO, :])
        lower = jnp.concatenate([plain((8, 2), h0, HB), plain((1, 7), h0 + HB // 2, HALO)], axis=0)
        for h, rows in enumerate((plain((1, 7), h0, HB), lower)):
            g = _gate(_gelu2(_dot(_as_bf16(rows), _as_bf16(wg[...]))))
            for l in range(NL):
                cb[G + l, HALO + h * HB:HALO + h * HB + g.shape[0], :] = g[:, l * LANES:(l + 1) * LANES]
        for q, v in enumerate(project(wu, ORDER)):
            for l in range(NL // 2):
                cb[U + (q % 2) * (NL // 2) + l, (q // 2) * HB:(q // 2 + 1) * HB, :] = (
                    v[:, l * LANES:(l + 1) * LANES])
        pin(cb, v)
        q11, q12, q21, q22 = project(wqk, ORDER)
        queries = [v.astype(BF16) for v in
                   (q11 + q22, q21 + q22, q11, q22, q11 + q12, q21 - q11, q12 - q22)]

        def conv_step(l, t0, nrows):
            acc = [None] * (nrows // 8)
            off = HALO - KW // 2
            for s in range(8):
                taps = [(a, 8 * a + s - off) for a in range((KW + off + 7) // 8)
                        if 0 <= 8 * a + s - off < KW]
                w = {a: cb[W + l, 8 * k:8 * k + 8, :] for a, k in taps}
                for j in range(len(acc) + max(a for a, _ in taps)):
                    use = [a for a, _ in taps if 0 <= j - a < len(acc)]
                    if not use:
                        continue
                    gv = cb[G + l, t0 + 8 * j + s:t0 + 8 * j + s + 8, :]
                    for a in use:
                        t = gv * w[a]
                        acc[j - a] = t if acc[j - a] is None else acc[j - a] + t
            cb[Z + l, pl.ds(zero_st + t0, nrows), :] = (
                jnp.concatenate(acc, axis=0) * _gelu2(cb[U + l, t0:t0 + nrows, :]))

        for t0 in range(0, BQ, CONV_ROWS):
            for l in range(NL):
                conv_step(l, t0, min(CONV_ROWS, BQ - t0))

        def keys(j, c):
            return _as_bf16(xs[j, c * BK // 2:(c + 1) * BK // 2, :])

        m = [None, None]
        for c in range(NC):
            prod = [None] * 7
            for k in SCORE_ORDER:
                prod[k] = _dot_nt(queries[k], keys(KEY_OPERAND[k], c))
            s11, s21, s12, s22 = _combine(prod)
            for q, s in enumerate((s11, s12, s21, s22)):
                if (c + 1) * BK > T // 2:
                    col = lax.broadcasted_iota(jnp.int32, (HB, BK), 1)
                    s = jnp.where(col < T // 2 - c * BK, s, -jnp.inf)
                c0 = (q % 2) * SW + (c // 2) * BK
                s_par[c % 2][(q // 2) * HB:(q // 2 + 1) * HB, c0:c0 + BK] = s
                for l in range(BK // LANES):
                    t = s[:, l * LANES:(l + 1) * LANES]
                    m[q // 2] = t if m[q // 2] is None else jnp.maximum(m[q // 2], t)
        row_max = [jnp.max(v, axis=-1, keepdims=True) for v in m]
        scale = [1.0 / jnp.sum(jnp.exp2(v - top), axis=-1, keepdims=True) for v, top in zip(m, row_max)]

        def weights(c):
            p, part = [], [None, None]
            for q in range(4):
                c0 = (q % 2) * SW + (c // 2) * BK
                rows = pl.ds((zero_ld if c == 0 else 0) + (q // 2) * HB, HB)
                e = jnp.exp2(s_par[c % 2][rows, c0:c0 + BK] - row_max[q // 2]) * scale[q // 2]
                for l in range(BK // LANES):
                    t = e[:, l * LANES:(l + 1) * LANES]
                    part[q // 2] = t if part[q // 2] is None else part[q // 2] + t
                p.append(e)
            return [v.astype(BF16) for v in _combos(*p)], jnp.concatenate(part, axis=1)

        def accumulate(c, k, d):
            if c > 0:
                d = d + a_par[(c - 1) % 2][k, 0:HB, :]
            if c + 1 < NC:
                a_par[c % 2][k, 0:HB, :] = d
            return d

        def merge(quads, w, after=None):
            left = _combos(*quads)
            out = [None] * 7
            for step, k in enumerate(MERGE_ORDER):
                l, r = PAIRS[k]
                out[k] = _dot(left[l].astype(BF16), _as_bf16(w[r]))
                if after:
                    after(step + 1, out[k])
            return _combine(out)

        def ln_next():
            for t0 in range(0, HB, LN_ROWS):
                nrows = min(LN_ROWS, HB - t0)
                for j, v in enumerate(ln_rows(r_next, t0, nrows)):
                    xn_buf[j, t0:t0 + nrows, :] = v.astype(BF16)
                pin(x_buf if t0 + LN_ROWS < HB else xs, _as_words(xn_buf[0, pl.ds(zero_ld, 16), :]))

        def publish(step, v):
            if step < len(PUBLISH) and PUBLISH[step]:
                pin(xn_buf, v)
                for j in PUBLISH[step]:
                    xs_all[b_next, j, pl.ds(h0, HB // 2), :] = _as_words(xn_buf[j, 0:HB, :])

        nxt = weights(0)

        z = [jnp.concatenate([cb[Z + (q % 2) * (NL // 2) + l, (q // 2) * HB:(q // 2 + 1) * HB, :]
                              for l in range(NL // 2)], axis=1) for q in range(4)]
        for q, v in enumerate(merge(z, wdc)):
            rows, cols = block(q)
            y_buf[q, 0:HB, :] = v + x_buf[pl.ds(r0 + rows, HB), cols].astype(F32)

        for c in range(NC):
            p, part = nxt
            acc = [None] * 7
            for step, k in enumerate(ORDER):
                l, r = PAIRS[k]
                if c == LN_CHUNK and step == 0:
                    ln_next()
                d = _dot(p[l], keys(r, c))
                if step == PIN_STEP and c + 1 < NC:
                    pin(s_par[(c + 1) % 2], d)
                    nxt = weights(c + 1)
                acc[k] = accumulate(c, k, d)
            total = accumulate(c, 7, part)
            if c + 1 < NC:
                pin(a_par[c % 2], total)
        o11, o12, o21, o22 = _combine(acc)
        inv = [1.0 / jnp.sum(v, axis=-1, keepdims=True) for v in (total[:, :LANES], total[:, LANES:])]

        pin(y_buf, acc[ORDER[0]])
        publish(0, acc[ORDER[6]])
        for q, v in enumerate(merge((o11 * inv[0], o12 * inv[0], o21 * inv[1], o22 * inv[1]), wva, publish)):
            rows, cols = block(q)
            o_buf[slot, rows:rows + HB, cols] = (v + y_buf[q, 0:HB, :]).astype(o_buf.dtype)
        o_copy(n, slot).start()
        last = i + 1 == NQ
        return jnp.where(last, b + 1, b), jnp.where(last, 0, i + 1)

    lax.fori_loop(0, NB, body, (jnp.int32(0), jnp.int32(0)))
    o_copy(NB - 2, (NB - 2) % 2).wait()
    o_copy(NB - 1, (NB - 1) % 2).wait()


@jax.jit
def pallas_standalone__conformer_family_branchformer__speech_kernel(
    x: jax.Array,
    w_q: jax.Array,
    w_k: jax.Array,
    w_v: jax.Array,
    w_ao: jax.Array,
    w_up: jax.Array,
    dw: jax.Array,
    w_dn: jax.Array,
    w_merge: jax.Array,
):
    B, T, D = x.shape
    KW = dw.shape[0]
    TP = -(-(T // 2) // BK) * BK
    NL, NQ, HB, HD = D // LANES, T // BQ, BQ // 2, D // 2
    assert T % BQ == 0 and BK == HD == 2 * LANES and KW // 2 < HALO <= TP - T // 2
    vmem, dma = pltpu.VMEM, pltpu.SemaphoreType.DMA
    scratch = [
        vmem((B * T + SPARE, D), BF16),
        vmem((B, 9, TP // 2 + SPARE, HD), U32),
        vmem((10, D, D), BF16),
        vmem((KW, D), BF16),
        vmem((3, D, D), F32),
        vmem((4, 7, HD // 2, HD), U32),
        vmem((HD, D), U32),
        vmem((4 * NL, BQ + 2 * HALO + SPARE, LANES), F32),
        vmem((9, HB + SPARE, HD), BF16),
        vmem((BQ + SPARE, TP), F32),
        vmem((BQ + SPARE, TP), F32),
        vmem((8, HB + SPARE, HD), F32),
        vmem((8, HB + SPARE, HD), F32),
        vmem((4, HB + SPARE, HD), F32),
        vmem((2, BQ, D), x.dtype),
        dma((B * NQ,)), dma((10,)), dma((2,)),
    ]
    in_hbm = pl.BlockSpec(memory_space=pl.ANY)
    return pl.pallas_call(
        _kernel,
        out_shape=jax.ShapeDtypeStruct((B * T, D), x.dtype),
        in_specs=[in_hbm] * 9,
        out_specs=in_hbm,
        scratch_shapes=scratch,
        compiler_params=pltpu.CompilerParams(vmem_limit_bytes=110 * 1024 * 1024),
    )(x.reshape(B * T, D), w_q, w_k, w_v, w_ao, w_up, dw, w_dn, w_merge).reshape(B, T, D)
```

```python
import functools
import math

import jax
import jax.numpy as jnp
from jax import lax
from jax.experimental import pallas as pl
from jax.experimental.pallas import tpu as pltpu

F32 = jnp.float32
BF16 = jnp.bfloat16
U32 = jnp.uint32
EPS = 1e-5
LANES = 128
HALO = 16
SPARE = 16

BQ = 800
BK = 256
CONV_ROWS = 24
LN_ROWS = 32
PIN_STEP = 1
LN_CHUNK = 4

PAIRS = ((0, 0), (1, 6), (3, 1), (4, 2), (2, 5), (5, 4), (6, 3))
KEY_OPERAND = (0, 1, 3, 4, 2, 5, 6)
ORDER = (1, 4, 0, 3, 2, 5, 6)
SCORE_ORDER = (0, 1, 4, 3, 2, 5, 6)
MERGE_ORDER = (4, 2, 1, 0, 3, 5, 6)
PUBLISH = ((0,), (1,), (2, 3), (4, 5), (6, 7), (8,), ())
PUBLISH_ROWS = 80


def _ln(x, eps=EPS):
    d = x.shape[-1]
    m = jnp.sum(x, axis=-1, keepdims=True) * (1.0 / d)
    c = x - m
    v = jnp.sum(c * c, axis=-1, keepdims=True) * (1.0 / d)
    return c * lax.rsqrt(v + eps)


def _gelu2(x):
    c1 = math.sqrt(2.0 / math.pi)
    c2 = c1 * 0.044715
    return x + x * jnp.tanh(x * (c1 + c2 * (x * x)))


def _gate(h2):
    return _ln(h2, 4.0 * EPS)


def _dot(a, b):
    return jnp.dot(a, b, preferred_element_type=F32)


def _dot_nt(a, b):
    return lax.dot_general(a, b, (((1,), (1,)), ((), ())), preferred_element_type=F32)


def _as_bf16(words):
    return pltpu.bitcast(words, BF16)


def _as_words(v):
    return pltpu.bitcast(v.astype(BF16), U32)


def _combos(a11, a12, a21, a22):
    return [a11 + a22, a11, a22, a21 - a22, a12 - a11, a11 + a21, a12 + a22]


def _combine(n):
    return (n[0] - n[4] + n[3] + n[6], n[1] + n[3], n[4] + n[2], n[0] - n[1] + n[2] + n[5])


def _operands(top, bot):
    h = top.shape[1] // 2
    return _combos(top[:, :h], top[:, h:], bot[:, :h], bot[:, h:]) + [top[:, h:], bot[:, :h]]


def _pin(dst, v, zero):
    lead = (0,) * (len(dst.shape) - 2)
    rows = 8 * (4 // jnp.dtype(dst.dtype).itemsize)
    v = pltpu.bitcast(v[v.shape[0] - 8:, :LANES], dst.dtype)
    dst[lead + (pl.ds(dst.shape[-2] - rows + zero, rows), slice(0, LANES))] = v


def _kernel(x_hbm, wq_hbm, wk_hbm, wv_hbm, wao_hbm, wup_hbm, dw_hbm, wdn_hbm, wm_hbm,
            o_hbm,
            x_buf, xs_all, wst, dw_in, wf32, wc, wg, cb, xn_buf,
            s_even, s_odd, a_even, a_odd, y_buf, o_buf,
            x_sem, w_sem, o_sem):
    B, D = xs_all.shape[0], x_hbm.shape[1]
    T = x_hbm.shape[0] // B
    KW = dw_hbm.shape[0]
    TP = s_even.shape[1]
    NQ = T // BQ
    NB = B * NQ
    NL = D // LANES
    NC = TP // BK
    HB = BQ // 2
    HD = D // 2
    G, U, W, Z = (NL * j for j in range(4))

    def x_copy(n):
        r = pl.ds(pl.multiple_of(n * BQ, BQ), BQ)
        return pltpu.make_async_copy(x_hbm.at[r, :], x_buf.at[r, :], x_sem.at[n])

    def o_copy(n, slot):
        r = pl.ds(pl.multiple_of(n * BQ, BQ), BQ)
        return pltpu.make_async_copy(o_buf.at[slot], o_hbm.at[r, :], o_sem.at[slot])

    WQ, WK, WV, WAO, WMA, WDN, WMC, WU, WG, W1 = range(10)
    w_src = [wq_hbm, wk_hbm, wv_hbm, wao_hbm, wm_hbm.at[0:D], wdn_hbm, wm_hbm.at[D:2 * D],
             wup_hbm.at[:, 0:D], wup_hbm.at[:, D:2 * D]]
    w_copies = [pltpu.make_async_copy(src, wst.at[j], w_sem.at[j]) for j, src in enumerate(w_src)]
    dw_copy = pltpu.make_async_copy(dw_hbm, dw_in, w_sem.at[len(w_src)])
    QK, VA, DC, UU = range(4)
    RB = 128
    NRB = D // RB

    def ln_rows(r0, t0, nrows):
        halves = [_ln(x_buf[pl.ds(r0 + h * HB + t0, nrows), :].astype(F32)) for h in range(2)]
        return _operands(*halves)

    for c in (w_copies[WQ], w_copies[WK], dw_copy, w_copies[WV], w_copies[WAO]):
        c.start()
    for b in range(B):
        xs_all[b, :, T // 4:TP // 2, :] = jnp.zeros((9, TP // 2 - T // 4, HD), U32)
    cb[G:G + NL, BQ:BQ + HALO, :] = jnp.zeros((NL, HALO, LANES), F32)
    w_copies[WQ].wait()
    w_copies[WK].wait()
    x_copy(0).start()
    x_copy(1).start()

    def fold_qk(t, c):
        r = pl.ds(pl.multiple_of(t * RB, RB), RB)
        wf32[QK, r, :] = _dot_nt(wst[WQ, r, :], wst[WK]) * (math.log2(math.e) / math.sqrt(D))
        return c
    lax.fori_loop(0, NRB, fold_qk, 0)

    def split(src, j, t0):
        halves = [src[pl.ds(pl.multiple_of(h * HD + t0, HD // 2), HD // 2), :].astype(F32) for h in range(2)]
        for k, v in enumerate(_operands(*halves)[:7]):
            wc[j, k, pl.ds(pl.multiple_of(t0 // 2, HD // 4), HD // 4), :] = _as_words(v)

    def split_folded(t, c):
        split(wf32.at[t // 2], t // 2, (t % 2) * (HD // 2))
        return c
    lax.fori_loop(0, 2, split_folded, 0)

    dw_copy.wait()
    for l in range(NL):
        cb[Z + l, 0:KW, :] = 0.5 * dw_in[:, l * LANES:(l + 1) * LANES].astype(F32)

    def spread_taps(k, c):
        for l in range(NL):
            cb[W + l, pl.ds(pl.multiple_of(8 * k, 8), 8), :] = jnp.broadcast_to(
                cb[Z + l, pl.ds(k, 1), :], (8, LANES))
        return c
    lax.fori_loop(0, KW, spread_taps, 0)

    PB = HB // HALO

    def ln_first(u, nrows):
        r0 = pl.multiple_of((u // PB) * BQ + (u % PB) * HALO, HALO)
        for k, v in enumerate(ln_rows(r0, 0, nrows)):
            xs_all[0, k, pl.ds(pl.multiple_of(u * (HALO // 2), HALO // 2), nrows // 2), :] = _as_words(v)

    NF = 3 * NRB
    PF = -(-(NQ - 1) * PB // NF)
    assert NQ == 5 and NRB == 4 and (PB // PF, 2 * PB // PF, 3 * PB // PF) == (2, 5, 8)
    arrivals = {
        0: ([w_copies[WV], w_copies[WAO], x_copy(0)], [w_copies[WMA], x_copy(2)]),
        2: ([x_copy(1)], [w_copies[WDN], w_copies[WMC]]),
        4: ([w_copies[WMA]], [x_copy(3)]),
        5: ([x_copy(2)], [w_copies[WU], w_copies[WG]]),
        8: ([w_copies[WDN], w_copies[WMC], x_copy(3)], [x_copy(4)]),
    }

    def fold(t, c):
        for step, (done, new) in arrivals.items():
            @pl.when(t == step)
            def _():
                for cp in done:
                    cp.wait()
                for cp in new:
                    cp.start()

        j = t // NRB
        left = jnp.where(j == 0, WV, jnp.where(j == 1, W1, WDN))
        right = jnp.where(j == 0, WAO, jnp.where(j == 1, WMA, WMC))
        r = pl.ds(pl.multiple_of((t % NRB) * RB, RB), RB)
        v = _dot(wst[left, r, :], wst[right])
        wf32[jnp.where(j == 1, VA, jnp.where(j == 2, DC, QK)), r, :] = v
        wst[jnp.where(j == 0, W1, WQ), r, :] = v.astype(BF16)
        for k in range(PF):
            ln_first(jnp.minimum(PF * t + k, (NQ - 1) * PB - 1), HALO)
        return c
    lax.fori_loop(0, NF, fold, 0)

    lax.fori_loop(2, 6, split_folded, 0)
    w_copies[WU].wait()
    w_copies[WG].wait()

    def split_plain(t, c):
        t0 = t * (HD // 2)
        split(wst.at[WU], UU, t0)
        wg[pl.ds(pl.multiple_of(t0, HD // 2), HD // 2), :] = _as_words(
            wst[WG, pl.ds(pl.multiple_of(2 * t0, HD), HD), :])
        return c
    lax.fori_loop(0, 2, split_plain, 0)

    x_copy(NQ - 1).wait()
    x_copy(NQ).start()

    def ln_last(t, c):
        ln_first((NQ - 1) * PB + 5 * t, 5 * HALO)
        return c
    lax.fori_loop(0, PB // 5, ln_last, 0)

    wqk, wva, wdc, wu = (wc.at[j] for j in (QK, VA, DC, UU))
    s_par = (s_even, s_odd)
    a_par = (a_even, a_odd)
    SW = TP // 2

    def block(q):
        return (q // 2) * HB, slice((q % 2) * HD, (q % 2 + 1) * HD)

    def body(n, carry):
        b, i = carry
        b_next = jnp.where(b + 1 < B, b + 1, 0)
        xs = xs_all.at[b]
        slot = n & 1
        r0 = pl.multiple_of(n * BQ, BQ)
        r_next = pl.multiple_of((b_next * NQ + i) * BQ, BQ)
        h0 = pl.multiple_of(i * (HB // 2), HB // 2)

        @pl.when(n + NQ < NB)
        def _():
            x_copy(n + NQ).wait()

        @pl.when(n + NQ + 1 < NB)
        def _():
            x_copy(n + NQ + 1).start()

        @pl.when(n >= 2)
        def _():
            o_copy(n - 2, slot).wait()

        zero_ld = pl.multiple_of((n // NB) * 16, 16)
        zero_st = pl.multiple_of((n // (NB + 1)) * 16, 16)
        pin = functools.partial(_pin, zero=zero_st)

        def project(w, order):
            out = [None] * 7
            for k in order:
                l, r = PAIRS[k]
                out[k] = _dot(_as_bf16(xs[l, pl.ds(h0, HB // 2), :]), _as_bf16(w[r]))
            return _combine(out)

        def plain(planes, row, nrows):
            return jnp.concatenate([xs[l, pl.ds(row, nrows // 2), :] for l in planes], axis=1)

        for l in range(NL):
            cb[G + l, 0:HALO, :] = jnp.where(i == 0, 0.0, cb[G + l, BQ:BQ + HALO, :])
        lower = jnp.concatenate([plain((8, 2), h0, HB), plain((1, 7), h0 + HB // 2, HALO)], axis=0)
        for h, rows in enumerate((plain((1, 7), h0, HB), lower)):
            g = _gate(_gelu2(_dot(_as_bf16(rows), _as_bf16(wg[...]))))
            for l in range(NL):
                cb[G + l, HALO + h * HB:HALO + h * HB + g.shape[0], :] = g[:, l * LANES:(l + 1) * LANES]
        for q, v in enumerate(project(wu, ORDER)):
            for l in range(NL // 2):
                cb[U + (q % 2) * (NL // 2) + l, (q // 2) * HB:(q // 2 + 1) * HB, :] = (
                    v[:, l * LANES:(l + 1) * LANES])
        pin(cb, v)
        q11, q12, q21, q22 = project(wqk, ORDER)
        queries = [v.astype(BF16) for v in
                   (q11 + q22, q21 + q22, q11, q22, q11 + q12, q21 - q11, q12 - q22)]

        def conv_step(l, t0, nrows):
            acc = [None] * (nrows // 8)
            off = HALO - KW // 2
            for s in range(8):
                taps = [(a, 8 * a + s - off) for a in range((KW + off + 7) // 8)
                        if 0 <= 8 * a + s - off < KW]
                w = {a: cb[W + l, 8 * k:8 * k + 8, :] for a, k in taps}
                for j in range(len(acc) + max(a for a, _ in taps)):
                    use = [a for a, _ in taps if 0 <= j - a < len(acc)]
                    if not use:
                        continue
                    gv = cb[G + l, t0 + 8 * j + s:t0 + 8 * j + s + 8, :]
                    for a in use:
                        t = gv * w[a]
                        acc[j - a] = t if acc[j - a] is None else acc[j - a] + t
            cb[Z + l, pl.ds(zero_st + t0, nrows), :] = (
                jnp.concatenate(acc, axis=0) * _gelu2(cb[U + l, t0:t0 + nrows, :]))

        for t0 in range(0, BQ, CONV_ROWS):
            for l in range(NL):
                conv_step(l, t0, min(CONV_ROWS, BQ - t0))

        def keys(j, c):
            return _as_bf16(xs[j, c * BK // 2:(c + 1) * BK // 2, :])

        m = [None, None]
        for c in range(NC):
            prod = [None] * 7
            for k in SCORE_ORDER:
                prod[k] = _dot_nt(queries[k], keys(KEY_OPERAND[k], c))
            s11, s21, s12, s22 = _combine(prod)
            for q, s in enumerate((s11, s12, s21, s22)):
                if (c + 1) * BK > T // 2:
                    col = lax.broadcasted_iota(jnp.int32, (HB, BK), 1)
                    s = jnp.where(col < T // 2 - c * BK, s, -jnp.inf)
                c0 = (q % 2) * SW + (c // 2) * BK
                s_par[c % 2][(q // 2) * HB:(q // 2 + 1) * HB, c0:c0 + BK] = s
                for l in range(BK // LANES):
                    t = s[:, l * LANES:(l + 1) * LANES]
                    m[q // 2] = t if m[q // 2] is None else jnp.maximum(m[q // 2], t)
        row_max = [jnp.max(v, axis=-1, keepdims=True) for v in m]
        scale = [1.0 / jnp.sum(jnp.exp2(v - top), axis=-1, keepdims=True) for v, top in zip(m, row_max)]

        def weights(c):
            p, part = [], [None, None]
            for q in range(4):
                c0 = (q % 2) * SW + (c // 2) * BK
                rows = pl.ds((zero_ld if c == 0 else 0) + (q // 2) * HB, HB)
                e = jnp.exp2(s_par[c % 2][rows, c0:c0 + BK] - row_max[q // 2]) * scale[q // 2]
                for l in range(BK // LANES):
                    t = e[:, l * LANES:(l + 1) * LANES]
                    part[q // 2] = t if part[q // 2] is None else part[q // 2] + t
                p.append(e)
            return [v.astype(BF16) for v in _combos(*p)], jnp.concatenate(part, axis=1)

        def accumulate(c, k, d):
            if c > 0:
                d = d + a_par[(c - 1) % 2][k, 0:HB, :]
            if c + 1 < NC:
                a_par[c % 2][k, 0:HB, :] = d
            return d

        def merge(quads, w, after=None):
            left = _combos(*quads)
            out = [None] * 7
            for step, k in enumerate(MERGE_ORDER):
                l, r = PAIRS[k]
                out[k] = _dot(left[l].astype(BF16), _as_bf16(w[r]))
                if after:
                    after(step, out[k])
            return _combine(out)

        def ln_next():
            for t0 in range(0, HB, LN_ROWS):
                nrows = min(LN_ROWS, HB - t0)
                for j, v in enumerate(ln_rows(r_next, t0, nrows)):
                    xn_buf[j, t0:t0 + nrows, :] = v.astype(BF16)
                pin(x_buf if t0 + LN_ROWS < HB else xs, _as_words(xn_buf[0, pl.ds(zero_ld, 16), :]))

        def publish(step, v):
            parts = [(j, t0) for j in PUBLISH[step] for t0 in range(0, HB, PUBLISH_ROWS)]
            for k, (j, t0) in enumerate(parts):
                pin(xn_buf, v[:8 * max(1, (k + 1) * (HB // 8) // len(parts))])
                xs_all[b_next, j, pl.ds(h0 + t0 // 2, PUBLISH_ROWS // 2), :] = _as_words(
                    xn_buf[j, t0:t0 + PUBLISH_ROWS, :])

        nxt = weights(0)

        z = [jnp.concatenate([cb[Z + (q % 2) * (NL // 2) + l, (q // 2) * HB:(q // 2 + 1) * HB, :]
                              for l in range(NL // 2)], axis=1) for q in range(4)]
        for q, v in enumerate(merge(z, wdc)):
            rows, cols = block(q)
            y_buf[q, 0:HB, :] = v + x_buf[pl.ds(r0 + rows, HB), cols].astype(F32)

        for c in range(NC):
            p, part = nxt
            acc = [None] * 7
            for step, k in enumerate(ORDER):
                l, r = PAIRS[k]
                if c == LN_CHUNK and step == 0:
                    ln_next()
                d = _dot(p[l], keys(r, c))
                if step == PIN_STEP and c + 1 < NC:
                    pin(s_par[(c + 1) % 2], d)
                    nxt = weights(c + 1)
                acc[k] = accumulate(c, k, d)
            total = accumulate(c, 7, part)
            if c + 1 < NC:
                pin(a_par[c % 2], total)
        o11, o12, o21, o22 = _combine(acc)
        inv = [1.0 / jnp.sum(v, axis=-1, keepdims=True) for v in (total[:, :LANES], total[:, LANES:])]

        pin(y_buf, acc[ORDER[0]])
        for q, v in enumerate(merge((o11 * inv[0], o12 * inv[0], o21 * inv[1], o22 * inv[1]), wva, publish)):
            rows, cols = block(q)
            o_buf[slot, rows:rows + HB, cols] = (v + y_buf[q, 0:HB, :]).astype(o_buf.dtype)
        o_copy(n, slot).start()
        last = i + 1 == NQ
        return jnp.where(last, b + 1, b), jnp.where(last, 0, i + 1)

    lax.fori_loop(0, NB, body, (jnp.int32(0), jnp.int32(0)))
    o_copy(NB - 2, (NB - 2) % 2).wait()
    o_copy(NB - 1, (NB - 1) % 2).wait()


@jax.jit
def pallas_standalone__conformer_family_branchformer__speech_kernel(
    x: jax.Array,
    w_q: jax.Array,
    w_k: jax.Array,
    w_v: jax.Array,
    w_ao: jax.Array,
    w_up: jax.Array,
    dw: jax.Array,
    w_dn: jax.Array,
    w_merge: jax.Array,
):
    B, T, D = x.shape
    KW = dw.shape[0]
    TP = -(-(T // 2) // BK) * BK
    NL, NQ, HB, HD = D // LANES, T // BQ, BQ // 2, D // 2
    assert T % BQ == 0 and BK == HD == 2 * LANES and KW // 2 < HALO <= TP - T // 2
    vmem, dma = pltpu.VMEM, pltpu.SemaphoreType.DMA
    scratch = [
        vmem((B * T + SPARE, D), BF16),
        vmem((B, 9, TP // 2 + SPARE, HD), U32),
        vmem((10, D, D), BF16),
        vmem((KW, D), BF16),
        vmem((3, D, D), F32),
        vmem((4, 7, HD // 2, HD), U32),
        vmem((HD, D), U32),
        vmem((4 * NL, BQ + 2 * HALO + SPARE, LANES), F32),
        vmem((9, HB + SPARE, HD), BF16),
        vmem((BQ + SPARE, TP), F32),
        vmem((BQ + SPARE, TP), F32),
        vmem((8, HB + SPARE, HD), F32),
        vmem((8, HB + SPARE, HD), F32),
        vmem((4, HB + SPARE, HD), F32),
        vmem((2, BQ, D), x.dtype),
        dma((B * NQ,)), dma((10,)), dma((2,)),
    ]
    in_hbm = pl.BlockSpec(memory_space=pl.ANY)
    return pl.pallas_call(
        _kernel,
        out_shape=jax.ShapeDtypeStruct((B * T, D), x.dtype),
        in_specs=[in_hbm] * 9,
        out_specs=in_hbm,
        scratch_shapes=scratch,
        compiler_params=pltpu.CompilerParams(vmem_limit_bytes=110 * 1024 * 1024),
    )(x.reshape(B * T, D), w_q, w_k, w_v, w_ao, w_up, dw, w_dn, w_merge).reshape(B, T, D)
```

```python
import functools
import math

import jax
import jax.numpy as jnp
from jax import lax
from jax.experimental import pallas as pl
from jax.experimental.pallas import tpu as pltpu

F32 = jnp.float32
BF16 = jnp.bfloat16
U32 = jnp.uint32
EPS = 1e-5
LANES = 128
HALO = 16
SPARE = 16

BQ = 800
BK = 256
CONV_ROWS = 24
LN_ROWS = 48
PIN_STEP = 0
LN_CHUNK = 3

PAIRS = ((0, 0), (1, 6), (3, 1), (4, 2), (2, 5), (5, 4), (6, 3))
KEY_OPERAND = (0, 1, 3, 4, 2, 5, 6)
ORDER = (1, 4, 0, 3, 2, 5, 6)
SCORE_ORDER = (0, 4, 1, 3, 2, 6, 5)
MERGE_ORDER = (4, 2, 1, 0, 3, 5, 6)
PUBLISH = ((0,), (1,), (2, 3), (4, 5), (6, 7), (8,), ())
PUBLISH_ROWS = 80


def _ln(x, eps=EPS):
    d = x.shape[-1]
    m = jnp.sum(x, axis=-1, keepdims=True) * (1.0 / d)
    c = x - m
    v = jnp.sum(c * c, axis=-1, keepdims=True) * (1.0 / d)
    return c * lax.rsqrt(v + eps)


def _gelu2(x):
    c1 = math.sqrt(2.0 / math.pi)
    c2 = c1 * 0.044715
    return x + x * jnp.tanh(x * (c1 + c2 * (x * x)))


def _gate(h2):
    return _ln(h2, 4.0 * EPS)


def _dot(a, b):
    return jnp.dot(a, b, preferred_element_type=F32)


def _dot_nt(a, b):
    return lax.dot_general(a, b, (((1,), (1,)), ((), ())), preferred_element_type=F32)


def _as_bf16(words):
    return pltpu.bitcast(words, BF16)


def _as_words(v):
    return pltpu.bitcast(v.astype(BF16), U32)


def _combos(a11, a12, a21, a22):
    return [a11 + a22, a11, a22, a21 - a22, a12 - a11, a11 + a21, a12 + a22]


def _combine(n):
    return (n[0] - n[4] + n[3] + n[6], n[1] + n[3], n[4] + n[2], n[0] - n[1] + n[2] + n[5])


def _operands(top, bot):
    h = top.shape[1] // 2
    return _combos(top[:, :h], top[:, h:], bot[:, :h], bot[:, h:]) + [top[:, h:], bot[:, :h]]


def _pin(dst, v, zero):
    lead = (0,) * (len(dst.shape) - 2)
    rows = 8 * (4 // jnp.dtype(dst.dtype).itemsize)
    v = pltpu.bitcast(v[v.shape[0] - 8:, :LANES], dst.dtype)
    dst[lead + (pl.ds(dst.shape[-2] - rows + zero, rows), slice(0, LANES))] = v


def _kernel(x_hbm, wq_hbm, wk_hbm, wv_hbm, wao_hbm, wup_hbm, dw_hbm, wdn_hbm, wm_hbm,
            o_hbm,
            x_buf, xs_all, wst, dw_in, wf32, wc, wg, cb, xn_buf,
            s_even, s_odd, a_even, a_odd, y_buf, o_buf,
            x_sem, w_sem, o_sem):
    B, D = xs_all.shape[0], x_hbm.shape[1]
    T = x_hbm.shape[0] // B
    KW = dw_hbm.shape[0]
    TP = s_even.shape[1]
    NQ = T // BQ
    NB = B * NQ
    NL = D // LANES
    NC = TP // BK
    HB = BQ // 2
    HD = D // 2
    G, U, W, Z = (NL * j for j in range(4))

    def x_copy(n):
        r = pl.ds(pl.multiple_of(n * BQ, BQ), BQ)
        return pltpu.make_async_copy(x_hbm.at[r, :], x_buf.at[r, :], x_sem.at[n])

    def o_copy(n, slot):
        r = pl.ds(pl.multiple_of(n * BQ, BQ), BQ)
        return pltpu.make_async_copy(o_buf.at[slot], o_hbm.at[r, :], o_sem.at[slot])

    WQ, WK, WV, WAO, WMA, WDN, WMC, WU, WG, W1 = range(10)
    w_src = [wq_hbm, wk_hbm, wv_hbm, wao_hbm, wm_hbm.at[0:D], wdn_hbm, wm_hbm.at[D:2 * D],
             wup_hbm.at[:, 0:D], wup_hbm.at[:, D:2 * D]]
    w_copies = [pltpu.make_async_copy(src, wst.at[j], w_sem.at[j]) for j, src in enumerate(w_src)]
    dw_copy = pltpu.make_async_copy(dw_hbm, dw_in, w_sem.at[len(w_src)])
    QK, VA, DC, UU = range(4)
    RB = 128
    NRB = D // RB

    def ln_rows(r0, t0, nrows):
        halves = [_ln(x_buf[pl.ds(r0 + h * HB + t0, nrows), :].astype(F32)) for h in range(2)]
        return _operands(*halves)

    for c in (w_copies[WQ], w_copies[WK], dw_copy, w_copies[WV], w_copies[WAO]):
        c.start()
    for b in range(B):
        xs_all[b, :, T // 4:TP // 2, :] = jnp.zeros((9, TP // 2 - T // 4, HD), U32)
    cb[G:G + NL, BQ:BQ + HALO, :] = jnp.zeros((NL, HALO, LANES), F32)
    w_copies[WQ].wait()
    w_copies[WK].wait()
    x_copy(0).start()
    x_copy(1).start()

    def fold_qk(t, c):
        r = pl.ds(pl.multiple_of(t * RB, RB), RB)
        wf32[QK, r, :] = _dot_nt(wst[WQ, r, :], wst[WK]) * (math.log2(math.e) / math.sqrt(D))
        return c
    lax.fori_loop(0, NRB, fold_qk, 0)

    def split(src, j, t0):
        halves = [src[pl.ds(pl.multiple_of(h * HD + t0, HD // 2), HD // 2), :].astype(F32) for h in range(2)]
        for k, v in enumerate(_operands(*halves)[:7]):
            wc[j, k, pl.ds(pl.multiple_of(t0 // 2, HD // 4), HD // 4), :] = _as_words(v)

    def split_folded(t, c):
        split(wf32.at[t // 2], t // 2, (t % 2) * (HD // 2))
        return c
    lax.fori_loop(0, 2, split_folded, 0)

    dw_copy.wait()
    for l in range(NL):
        cb[Z + l, 0:KW, :] = 0.5 * dw_in[:, l * LANES:(l + 1) * LANES].astype(F32)

    def spread_taps(k, c):
        for l in range(NL):
            cb[W + l, pl.ds(pl.multiple_of(8 * k, 8), 8), :] = jnp.broadcast_to(
                cb[Z + l, pl.ds(k, 1), :], (8, LANES))
        return c
    lax.fori_loop(0, KW, spread_taps, 0)

    PB = HB // HALO

    def ln_first(u, nrows):
        r0 = pl.multiple_of((u // PB) * BQ + (u % PB) * HALO, HALO)
        for k, v in enumerate(ln_rows(r0, 0, nrows)):
            xs_all[0, k, pl.ds(pl.multiple_of(u * (HALO // 2), HALO // 2), nrows // 2), :] = _as_words(v)

    NF = 3 * NRB
    PF = -(-(NQ - 1) * PB // NF)
    assert NQ == 5 and NRB == 4 and (PB // PF, 2 * PB // PF, 3 * PB // PF) == (2, 5, 8)
    arrivals = {
        0: ([w_copies[WV], w_copies[WAO], x_copy(0)], [w_copies[WMA], x_copy(2)]),
        2: ([x_copy(1)], [w_copies[WDN], w_copies[WMC]]),
        4: ([w_copies[WMA]], [x_copy(3)]),
        5: ([x_copy(2)], [w_copies[WU], w_copies[WG]]),
        8: ([w_copies[WDN], w_copies[WMC], x_copy(3)], [x_copy(4)]),
    }

    def fold(t, c):
        for step, (done, new) in arrivals.items():
            @pl.when(t == step)
            def _():
                for cp in done:
                    cp.wait()
                for cp in new:
                    cp.start()

        j = t // NRB
        left = jnp.where(j == 0, WV, jnp.where(j == 1, W1, WDN))
        right = jnp.where(j == 0, WAO, jnp.where(j == 1, WMA, WMC))
        r = pl.ds(pl.multiple_of((t % NRB) * RB, RB), RB)
        v = _dot(wst[left, r, :], wst[right])
        wf32[jnp.where(j == 1, VA, jnp.where(j == 2, DC, QK)), r, :] = v
        wst[jnp.where(j == 0, W1, WQ), r, :] = v.astype(BF16)
        for k in range(PF):
            ln_first(jnp.minimum(PF * t + k, (NQ - 1) * PB - 1), HALO)
        return c
    lax.fori_loop(0, NF, fold, 0)

    lax.fori_loop(2, 6, split_folded, 0)
    w_copies[WU].wait()
    w_copies[WG].wait()

    def split_plain(t, c):
        t0 = t * (HD // 2)
        split(wst.at[WU], UU, t0)
        wg[pl.ds(pl.multiple_of(t0, HD // 2), HD // 2), :] = _as_words(
            wst[WG, pl.ds(pl.multiple_of(2 * t0, HD), HD), :])
        return c
    lax.fori_loop(0, 2, split_plain, 0)

    x_copy(NQ - 1).wait()
    x_copy(NQ).start()

    def ln_last(t, c):
        ln_first((NQ - 1) * PB + 5 * t, 5 * HALO)
        return c
    lax.fori_loop(0, PB // 5, ln_last, 0)

    wqk, wva, wdc, wu = (wc.at[j] for j in (QK, VA, DC, UU))
    s_par = (s_even, s_odd)
    a_par = (a_even, a_odd)
    SW = TP // 2

    def block(q):
        return (q // 2) * HB, slice((q % 2) * HD, (q % 2 + 1) * HD)

    def body(n, carry):
        b, i = carry
        b_next = jnp.where(b + 1 < B, b + 1, 0)
        xs = xs_all.at[b]
        slot = n & 1
        r0 = pl.multiple_of(n * BQ, BQ)
        r_next = pl.multiple_of((b_next * NQ + i) * BQ, BQ)
        h0 = pl.multiple_of(i * (HB // 2), HB // 2)

        @pl.when(n + NQ < NB)
        def _():
            x_copy(n + NQ).wait()

        @pl.when(n + NQ + 1 < NB)
        def _():
            x_copy(n + NQ + 1).start()

        @pl.when(n >= 2)
        def _():
            o_copy(n - 2, slot).wait()

        zero_ld = pl.multiple_of((n // NB) * 16, 16)
        zero_st = pl.multiple_of((n // (NB + 1)) * 16, 16)
        pin = functools.partial(_pin, zero=zero_st)

        def project(w, order):
            out = [None] * 7
            for k in order:
                l, r = PAIRS[k]
                out[k] = _dot(_as_bf16(xs[l, pl.ds(h0, HB // 2), :]), _as_bf16(w[r]))
            return _combine(out)

        def plain(planes, row, nrows):
            return jnp.concatenate([xs[l, pl.ds(row, nrows // 2), :] for l in planes], axis=1)

        for l in range(NL):
            cb[G + l, 0:HALO, :] = jnp.where(i == 0, 0.0, cb[G + l, BQ:BQ + HALO, :])
        lower = jnp.concatenate([plain((8, 2), h0, HB), plain((1, 7), h0 + HB // 2, HALO)], axis=0)
        for h, rows in enumerate((plain((1, 7), h0, HB), lower)):
            g = _gate(_gelu2(_dot(_as_bf16(rows), _as_bf16(wg[...]))))
            for l in range(NL):
                cb[G + l, HALO + h * HB:HALO + h * HB + g.shape[0], :] = g[:, l * LANES:(l + 1) * LANES]
        for q, v in enumerate(project(wu, ORDER)):
            for l in range(NL // 2):
                cb[U + (q % 2) * (NL // 2) + l, (q // 2) * HB:(q // 2 + 1) * HB, :] = (
                    v[:, l * LANES:(l + 1) * LANES])
        pin(cb, v)
        q11, q12, q21, q22 = project(wqk, ORDER)
        queries = [v.astype(BF16) for v in
                   (q11 + q22, q21 + q22, q11, q22, q11 + q12, q21 - q11, q12 - q22)]

        def conv_step(l, t0, nrows):
            acc = [None] * (nrows // 8)
            off = HALO - KW // 2
            for s in range(8):
                taps = [(a, 8 * a + s - off) for a in range((KW + off + 7) // 8)
                        if 0 <= 8 * a + s - off < KW]
                w = {a: cb[W + l, 8 * k:8 * k + 8, :] for a, k in taps}
                for j in range(len(acc) + max(a for a, _ in taps)):
                    use = [a for a, _ in taps if 0 <= j - a < len(acc)]
                    if not use:
                        continue
                    gv = cb[G + l, t0 + 8 * j + s:t0 + 8 * j + s + 8, :]
                    for a in use:
                        t = gv * w[a]
                        acc[j - a] = t if acc[j - a] is None else acc[j - a] + t
            cb[Z + l, pl.ds(zero_st + t0, nrows), :] = (
                jnp.concatenate(acc, axis=0) * _gelu2(cb[U + l, t0:t0 + nrows, :]))

        for t0 in range(0, BQ, CONV_ROWS):
            for l in range(NL):
                conv_step(l, t0, min(CONV_ROWS, BQ - t0))

        def keys(j, c):
            return _as_bf16(xs[j, c * BK // 2:(c + 1) * BK // 2, :])

        m = [None, None]
        for c in range(NC):
            prod = [None] * 7
            for k in SCORE_ORDER:
                prod[k] = _dot_nt(queries[k], keys(KEY_OPERAND[k], c))
            s11, s21, s12, s22 = _combine(prod)
            for q, s in enumerate((s11, s12, s21, s22)):
                if (c + 1) * BK > T // 2:
                    col = lax.broadcasted_iota(jnp.int32, (HB, BK), 1)
                    s = jnp.where(col < T // 2 - c * BK, s, -jnp.inf)
                c0 = (q % 2) * SW + (c // 2) * BK
                s_par[c % 2][(q // 2) * HB:(q // 2 + 1) * HB, c0:c0 + BK] = s
                for l in range(BK // LANES):
                    t = s[:, l * LANES:(l + 1) * LANES]
                    m[q // 2] = t if m[q // 2] is None else jnp.maximum(m[q // 2], t)
        row_max = [jnp.max(v, axis=-1, keepdims=True) for v in m]
        scale = [1.0 / jnp.sum(jnp.exp2(v - top), axis=-1, keepdims=True) for v, top in zip(m, row_max)]

        def weights(c):
            p, part = [], [None, None]
            for q in range(4):
                c0 = (q % 2) * SW + (c // 2) * BK
                rows = pl.ds((zero_ld if c == 0 else 0) + (q // 2) * HB, HB)
                e = jnp.exp2(s_par[c % 2][rows, c0:c0 + BK] - row_max[q // 2]) * scale[q // 2]
                for l in range(BK // LANES):
                    t = e[:, l * LANES:(l + 1) * LANES]
                    part[q // 2] = t if part[q // 2] is None else part[q // 2] + t
                p.append(e)
            return [v.astype(BF16) for v in _combos(*p)], jnp.concatenate(part, axis=1)

        def accumulate(c, k, d):
            if c > 0:
                d = d + a_par[(c - 1) % 2][k, 0:HB, :]
            if c + 1 < NC:
                a_par[c % 2][k, 0:HB, :] = d
            return d

        def merge(quads, w, after=None):
            left = _combos(*quads)
            out = [None] * 7
            for step, k in enumerate(MERGE_ORDER):
                l, r = PAIRS[k]
                out[k] = _dot(left[l].astype(BF16), _as_bf16(w[r]))
                if after:
                    after(step, out[k])
            return _combine(out)

        def ln_next():
            for t0 in range(0, HB, LN_ROWS):
                nrows = min(LN_ROWS, HB - t0)
                for j, v in enumerate(ln_rows(r_next, t0, nrows)):
                    xn_buf[j, t0:t0 + nrows, :] = v.astype(BF16)
                pin(x_buf if t0 + LN_ROWS < HB else xs, _as_words(xn_buf[0, pl.ds(zero_ld, 16), :]))

        def publish(step, v):
            parts = [(j, t0) for j in PUBLISH[step] for t0 in range(0, HB, PUBLISH_ROWS)]
            for k, (j, t0) in enumerate(parts):
                pin(xn_buf, v[:8 * max(1, (k + 1) * (HB // 8) // len(parts))])
                xs_all[b_next, j, pl.ds(h0 + t0 // 2, PUBLISH_ROWS // 2), :] = _as_words(
                    xn_buf[j, t0:t0 + PUBLISH_ROWS, :])

        nxt = weights(0)

        z = [jnp.concatenate([cb[Z + (q % 2) * (NL // 2) + l, (q // 2) * HB:(q // 2 + 1) * HB, :]
                              for l in range(NL // 2)], axis=1) for q in range(4)]
        for q, v in enumerate(merge(z, wdc)):
            rows, cols = block(q)
            y_buf[q, 0:HB, :] = v + x_buf[pl.ds(r0 + rows, HB), cols].astype(F32)

        for c in range(NC):
            p, part = nxt
            acc = [None] * 7
            for step, k in enumerate(ORDER):
                l, r = PAIRS[k]
                if c == LN_CHUNK and step == 0:
                    ln_next()
                d = _dot(p[l], keys(r, c))
                if step == PIN_STEP and c + 1 < NC:
                    pin(s_par[(c + 1) % 2], d)
                    nxt = weights(c + 1)
                acc[k] = accumulate(c, k, d)
            total = accumulate(c, 7, part)
            if c + 1 < NC:
                pin(a_par[c % 2], total)
        o11, o12, o21, o22 = _combine(acc)
        inv = [1.0 / jnp.sum(v, axis=-1, keepdims=True) for v in (total[:, :LANES], total[:, LANES:])]

        pin(y_buf, acc[ORDER[0]])
        for q, v in enumerate(merge((o11 * inv[0], o12 * inv[0], o21 * inv[1], o22 * inv[1]), wva, publish)):
            rows, cols = block(q)
            o_buf[slot, rows:rows + HB, cols] = (v + y_buf[q, 0:HB, :]).astype(o_buf.dtype)
        o_copy(n, slot).start()
        last = i + 1 == NQ
        return jnp.where(last, b + 1, b), jnp.where(last, 0, i + 1)

    lax.fori_loop(0, NB, body, (jnp.int32(0), jnp.int32(0)))
    o_copy(NB - 2, (NB - 2) % 2).wait()
    o_copy(NB - 1, (NB - 1) % 2).wait()


@jax.jit
def pallas_standalone__conformer_family_branchformer__speech_kernel(
    x: jax.Array,
    w_q: jax.Array,
    w_k: jax.Array,
    w_v: jax.Array,
    w_ao: jax.Array,
    w_up: jax.Array,
    dw: jax.Array,
    w_dn: jax.Array,
    w_merge: jax.Array,
):
    B, T, D = x.shape
    KW = dw.shape[0]
    TP = -(-(T // 2) // BK) * BK
    NL, NQ, HB, HD = D // LANES, T // BQ, BQ // 2, D // 2
    assert T % BQ == 0 and BK == HD == 2 * LANES and KW // 2 < HALO <= TP - T // 2
    vmem, dma = pltpu.VMEM, pltpu.SemaphoreType.DMA
    scratch = [
        vmem((B * T + SPARE, D), BF16),
        vmem((B, 9, TP // 2 + SPARE, HD), U32),
        vmem((10, D, D), BF16),
        vmem((KW, D), BF16),
        vmem((3, D, D), F32),
        vmem((4, 7, HD // 2, HD), U32),
        vmem((HD, D), U32),
        vmem((4 * NL, BQ + 2 * HALO + SPARE, LANES), F32),
        vmem((9, HB + SPARE, HD), BF16),
        vmem((BQ + SPARE, TP), F32),
        vmem((BQ + SPARE, TP), F32),
        vmem((8, HB + SPARE, HD), F32),
        vmem((8, HB + SPARE, HD), F32),
        vmem((4, HB + SPARE, HD), F32),
        vmem((2, BQ, D), x.dtype),
        dma((B * NQ,)), dma((10,)), dma((2,)),
    ]
    in_hbm = pl.BlockSpec(memory_space=pl.ANY)
    return pl.pallas_call(
        _kernel,
        out_shape=jax.ShapeDtypeStruct((B * T, D), x.dtype),
        in_specs=[in_hbm] * 9,
        out_specs=in_hbm,
        scratch_shapes=scratch,
        compiler_params=pltpu.CompilerParams(vmem_limit_bytes=110 * 1024 * 1024),
    )(x.reshape(B * T, D), w_q, w_k, w_v, w_ao, w_up, dw, w_dn, w_merge).reshape(B, T, D)
```
